```python
import jax
import jax.numpy as jnp

def _softmax(x, axis=-1):
    return jax.nn.softmax(x, axis=axis)

def _gelu(x):
    return jax.nn.gelu(x, approximate=True)

def _silu(x):
    return jax.nn.silu(x)

def _sigmoid(x):
    return jax.nn.sigmoid(x)

def _layernorm(x, axis=-1, eps=1e-05):
    m = jnp.mean(x, axis=axis, keepdims=True)
    v = jnp.var(x, axis=axis, keepdims=True)
    return (x - m) / jnp.sqrt(v + eps)

def _scatter_add(tgt, idx, src, axis=0):
    return tgt.at[idx].add(src)

def _segment_sum(src, seg, n):
    return jax.ops.segment_sum(src, seg, n)

class _Rng:

    def __init__(self, key):
        self._k = key

    def _next(self):
        self._k, sub = jax.random.split(self._k)
        return sub

    def normal(self, shape):
        return jax.random.normal(self._next(), shape, dtype=jnp.bfloat16)

    def randint(self, lo, hi, shape):
        return jax.random.randint(self._next(), shape, lo, hi, dtype=jnp.int32)

    def uniform(self, shape, lo=0.0, hi=1.0):
        return jax.random.uniform(self._next(), shape, jnp.bfloat16, lo, hi)

    def permutation(self, n):
        return jax.random.permutation(self._next(), n)
kernel_name = 'interleave_layers__memory_aug_recurrent_mem_tr__glu_gated_swiglu__prompt'

def setup_inputs():
    _rng = _Rng(jax.random.key(int.from_bytes(__import__("os").urandom(4), "little")))
    _w = lambda a: (lambda t: t.astype(jnp.bfloat16) if jnp.issubdtype(t.dtype, jnp.floating) else t)(jnp.asarray(a))

    def _A_setup():
        B, S, Dm = (1, 2048, 576)
        H, Dh = (32, 128)
        M, seg = (8, 32)
        seg = min(seg, S)
        S = S // seg * seg
        return {'x': _w((lambda *s: _rng.normal(s) * 0.05)(B, S, Dm)), 'mem0': _w((lambda *s: _rng.normal(s) * 0.05)(B, M, Dm)), 'Wq': _w((lambda *s: _rng.normal(s) * 0.05)(Dm, H, Dh) * Dm ** (-0.5)), 'Wk': _w((lambda *s: _rng.normal(s) * 0.05)(Dm, H, Dh) * Dm ** (-0.5)), 'Wv': _w((lambda *s: _rng.normal(s) * 0.05)(Dm, H, Dh) * Dm ** (-0.5)), 'Wo': _w((lambda *s: _rng.normal(s) * 0.05)(H, Dh, Dm) * (H * Dh) ** (-0.5)), 'seg_len': seg}
    _A_in = _A_setup()

    def _B_setup():
        B, S, D, F = (1, 2048, 576, 4608)
        return {'x': _w((lambda *s: _rng.normal(s) * 0.05)(B, S, D)), 'w1': _w((lambda *s: _rng.normal(s) * 0.05)(D, F) * (2.0 / D) ** 0.5), 'w3': _w((lambda *s: _rng.normal(s) * 0.05)(D, F) * (2.0 / D) ** 0.5), 'w2': _w((lambda *s: _rng.normal(s) * 0.05)(F, D) * (2.0 / F) ** 0.5)}
    _B_in = _B_setup()
    return {'A_x': _A_in['x'], 'A_mem0': _A_in['mem0'], 'A_Wq': _A_in['Wq'], 'A_Wk': _A_in['Wk'], 'A_Wv': _A_in['Wv'], 'A_Wo': _A_in['Wo'], 'A_seg_len': _A_in['seg_len'], 'B_x': _B_in['x'], 'B_w1': _B_in['w1'], 'B_w3': _B_in['w3'], 'B_w2': _B_in['w2']}

def reference(A_x, A_mem0, A_Wq, A_Wk, A_Wv, A_Wo, A_seg_len, B_x, B_w1, B_w3, B_w2):

    def _A_ref(x, mem0, Wq, Wk, Wv, Wo, seg_len):
        B, S, Dm = x.shape
        H, Dh = (Wq.shape[1], Wq.shape[2])
        M = mem0.shape[1]
        scale = Dh ** (-0.5)
        n_seg = S // seg_len
        L = M + seg_len
        idx = jnp.arange(L)
        mask = (idx[:, None] < M) | (idx[:, None] >= idx[None, :])
        mem = mem0
        outs = []
        for s in range(n_seg):
            xs = x[:, s * seg_len:(s + 1) * seg_len, :].copy()
            h = jnp.concatenate([mem, xs], axis=1)
            q = jnp.einsum('btd,dhe->bhte', h, Wq)
            k = jnp.einsum('btd,dhe->bhte', h, Wk)
            v = jnp.einsum('btd,dhe->bhte', h, Wv)
            scores = jnp.einsum('bhqe,bhke->bhqk', q, k) * scale
            scores = jnp.where(mask[None, None], scores, -1000000000.0)
            p = _softmax(scores, axis=-1)
            o = jnp.einsum('bhqk,bhke->bhqe', p, v)
            o = jnp.einsum('bhte,hed->btd', o, Wo)
            mem = o[:, :M, :].copy()
            outs.append(o[:, M:, :])
        return jnp.concatenate(outs, axis=1)

    def _B_ref(x, w1, w3, w2):
        gate = jnp.einsum('bsd,df->bsf', x, w1)
        up = jnp.einsum('bsd,df->bsf', x, w3)
        h = _silu(gate) * up
        out = jnp.einsum('bsf,fd->bsd', h, w2)
        return out
    x = A_x
    x = x + _A_ref(_layernorm(x, axis=-1), A_mem0, A_Wq, A_Wk, A_Wv, A_Wo, A_seg_len)
    x = x + _B_ref(_layernorm(x, axis=-1), B_w1, B_w3, B_w2)
    x = x + _A_ref(_layernorm(x, axis=-1), A_mem0, A_Wq, A_Wk, A_Wv, A_Wo, A_seg_len)
    x = x + _B_ref(_layernorm(x, axis=-1), B_w1, B_w3, B_w2)
    return x
```

```python
import functools
import math
from typing import NamedTuple

import jax
import jax.numpy as jnp
import jax.experimental.pallas as pl
import jax.experimental.pallas.tpu as pltpu

_EPS = 1e-05
_MASKED = -1000000000.0
_LOG2E = math.log2(math.e)
_T = 128
_BLOCKS = 5
_LAG = 2
_EARLY = 16
_EARLY_ROWS = 64
_SLOTS = 3
_ORDER = ("G0 Q0 K0 V0 S0 G1 A0 Q1 K1 V1 S1 O0 A1 Q2 K2 V2 S2 G2 A2 Q3 K3 V3 O1 S3 G3 A3 "
          "O2 O3 G4 D0 G5 G6 G7 N0 D1 D2 D3")
_ORDER_ATTENTION = "Q0 K0 V0 S0 Q1 A0 K1 V1 S1 Q3 K3 A1 Q2 S3 K2 V3 V2 S2 O0 A3 A2 O1 O3 O2 N0"
_ORDER_FFN = "G0 G1 G2 D0 G3 G4 G5 G6 G7 D1 D2 D3"


class _Product(NamedTuple):
    rows: tuple
    weights: tuple
    tiles: tuple


def _scheme(n_side, edges):
    products = []

    def add(rows, weights, tiles):
        rows = tuple(sorted(rows, key=lambda term: term[1:]))
        if rows[0][0] < 0:
            rows = tuple((-s, half, i) for s, half, i in rows)
            tiles = tuple((-s, half, t) for s, half, t in tiles)
        products.append(_Product(rows, tuple(weights), tuple(tiles)))

    def own_blocks(t, half):
        mine = [((i, v, j), (j, u, i))[half] for u, i, v, j in edges if (u, v)[half] == t]
        for i in range(_BLOCKS):
            if any(i == j for _, _, j in mine):
                continue
            partners = [(p, j) for home, p, j in mine if home == i]
            if not partners:
                add([(1, 0, i)], [(1, t, i)], [(1, 0, t)])
                add([(1, 1, i)], [(1, t, i)], [(1, 1, t)])
                continue
            add([(1, half, i)], [(1, t, i)] + [(1, t, j) for _, j in partners],
                [(1, half, t), (-1, 1 - half, t)])
            add([(1, 0, i), (1, 1, i)], [(1, t, i)] + [(-1, p, i) for p, _ in partners],
                [(1, 1 - half, t)])

    for t in range(n_side):
        own_blocks(t, 0)
        for u, i, v, j in edges:
            if u == t:
                add([(1, 0, j), (-1, 0, i)], [(1, u, j)], [(1, 0, u), (1, 0, v)])
                add([(1, 1, i), (-1, 1, j)], [(1, v, i)], [(1, 1, v), (1, 1, u)])
                add([(1, 0, i), (1, 1, j)], [(1, u, j), (1, v, i)], [(1, 1, u), (1, 0, v)])
    for t in range(n_side, 2 * n_side):
        own_blocks(t, 1)
    return tuple(products)


_TEN = _scheme(5, [(i, i, 5 + j, j) for i in range(5) for j in range(5) if i != j])
_SIX = _scheme(3, [(i, i, 1 + j, j) for i in range(3) for j in range(2, 5) if i != j])
_TWO = _scheme(1, [(0, 0, 1, 2), (0, 1, 1, 3)])
_MIXES = tuple(sorted({p.rows for p in _TEN}))


def _first_half(scheme):
    kept = []
    for n, (rows, weights, tiles) in enumerate(scheme):
        rows = tuple(term for term in rows if term[1] == 0)
        tiles = tuple(term for term in tiles if term[1] == 0)
        if rows and tiles:
            kept.append((n, _Product(rows, weights, tiles)))
    return kept


def _signed_sum(terms):
    (sign, total), *rest = sorted(terms, key=lambda term: -term[0])
    for s, value in rest:
        total = total + value if s == sign else total - value
    return total if sign > 0 else -total


def _accumulate(acc, key, sign, value):
    if key in acc:
        s, total = acc[key]
        if s == sign:
            acc[key] = s, total + value
        else:
            acc[key] = 1, total - value if s > 0 else value - total
    else:
        acc[key] = sign, value


def _dot(a, b):
    return jax.lax.dot_general(a, b, (((1,), (0,)), ((), ())),
                               preferred_element_type=jnp.float32)


def _dot_nt(a, b):
    return jax.lax.dot_general(a, b, (((1,), (1,)), ((), ())),
                               preferred_element_type=jnp.float32)


def _pack(x):
    return pltpu.bitcast(x, jnp.uint32)


def _unpack(words):
    return pltpu.bitcast(words, jnp.bfloat16)


def _cols(n, width=1):
    return slice(n * _T, (n + width) * _T)


def _to_bf16(tiles):
    out = []
    for n in range(0, len(tiles), 2):
        both = jnp.concatenate(tiles[n:n + 2], axis=1).astype(jnp.bfloat16)
        out += [both[:, _cols(c)] for c in range(both.shape[1] // _T)]
    return out


def _kernel(xt_hbm, mem0_hbm, wq_hbm, wk_hbm, wv_hbm, wot_hbm, w1_hbm, w3_hbm, w2t_hbm,
            outt_hbm, mem0_ref, tile_ref, res_ref, mem_ref, mix_ref, early_mix_ref, early_ref,
            early2_ref, qkv_ref, qkv2_ref, gate_ref, gate2_ref, out_ref, wo2_ref, down6_ref,
            qkv_stage, gate_stage, out_stage, qkv_sem, gate_sem, out_sem, tile_sem, mem_sem,
            *, seg):
    d_model, n_tok = xt_hbm.shape
    n_mem = mem0_ref.shape[0]
    d_head = wq_hbm.shape[2]
    n_seg = n_tok // seg
    n_io = n_tok // _T
    last = d_model - (_BLOCKS - 1) * _T
    n_qkv, n_gate, n_out = qkv_ref.shape[0], gate_ref.shape[0], out_ref.shape[0]
    n_full = n_qkv // 3
    score_scale = d_head ** -0.5 * _LOG2E

    def clear_padding(x):
        lane = jax.lax.broadcasted_iota(jnp.int32, x.shape, 1)
        return jnp.where(lane < last, x, 0.0)

    def layernorm(blocks):
        mean = jnp.sum(sum(blocks[1:], blocks[0]), axis=-1, keepdims=True) / d_model
        d = [x - mean for x in blocks]
        d[-1] = clear_padding(d[-1])
        var = jnp.sum(sum([x * x for x in d[1:]], d[0] * d[0]), axis=-1, keepdims=True) / d_model
        inv = jax.lax.rsqrt(var + _EPS)
        return [x * inv for x in d]

    def rows_of(s):
        return pl.ds(pl.multiple_of(s * seg, seg), seg)

    def load(s):
        return [res_ref[rows_of(s), _cols(i)] for i in range(_BLOCKS)]

    def store(s, blocks):
        for i, x in enumerate(blocks):
            res_ref[rows_of(s), _cols(i)] = x

    def mixes(halves):
        return {rows: _signed_sum([(s, halves[half][i]) for s, half, i in rows])
                for rows in _MIXES if all(half < len(halves) for _, half, _ in rows)}

    def products(scheme, n_halves):
        return list(enumerate(scheme)) if n_halves == 2 else _first_half(scheme)

    def widen(mix, w_ref, scheme, n_halves):
        acc = {}
        for n, (rows, weights, tiles) in products(scheme, n_halves):
            short = any(all(term[2] == _BLOCKS - 1 for term in terms) for terms in (rows, weights))
            depth = last if short else _T
            value = _dot(mix(rows)[:, :depth], _unpack(w_ref[:depth // 2, _cols(n)]))
            for s, half, t in tiles:
                _accumulate(acc, (t, half), s, value)
        return [[_signed_sum([acc[t, half]]) for half in range(n_halves)]
                for t in range(len(acc) // n_halves)]

    def narrow(acc, wide, w_ref, scheme):
        by_rows = {}
        for n, product in products(scheme, len(wide[0])):
            by_rows.setdefault(product.rows, []).append((n, product.tiles))
        for rows in sorted(by_rows, key=lambda rows: sorted({i for _, _, i in rows})):
            total = {}
            for n, tiles in by_rows[rows]:
                sign = max(s for s, _, _ in tiles)
                lhs = _signed_sum([(s * sign, wide[t][half]) for s, half, t in tiles])
                _accumulate(total, 0, sign, _dot(lhs, _unpack(w_ref[:, _cols(n)])))
            for s, half, i in rows:
                _accumulate(acc, (half, i), s * total[0][0], total[0][1])

    def blocks_of(acc, half):
        blocks = [_signed_sum([acc[half, i]]) for i in range(_BLOCKS)]
        return blocks[:-1] + [clear_padding(blocks[-1])]

    def masks(n_layers):
        span = n_mem + seg
        i, j = (jax.lax.broadcasted_iota(jnp.int32, (n_layers * span,) * 2, a) for a in (0, 1))
        if n_layers == 1:
            return (i < n_mem) | (i >= j), _MASKED * _LOG2E
        same = (i >= span) == (j >= span)
        visible = (i < n_mem) | ((i >= span) & (i < span + n_mem)) | (i >= j)
        return same & visible, jnp.where(same, _MASKED * _LOG2E, -jnp.inf).astype(jnp.float32)

    def step(order, attend=(), feed=(), partner=None):
        n_layers = len(attend)
        if attend:
            visible, fill = masks(n_layers)
            x = [load(s) for s in attend]
            mem = [[mem_ref[n, :, _cols(i)] for i in range(_BLOCKS)] for n in range(n_layers)]
            h = [layernorm(x[0])]
            if n_layers == 1:
                halves = [[jnp.concatenate(parts, axis=0) for parts in zip(mem[0], h[0])]]
            else:
                h.append(layernorm([block[:seg - _EARLY] for block in x[1]]))
                cut = seg - _EARLY // 2
                halves = [[jnp.concatenate([m, a[:cut]], axis=0) for m, a in zip(mem[0], h[0])],
                          [jnp.concatenate([m, a[cut:], b], axis=0)
                           for m, a, b in zip(mem[1], h[0], h[1])]]
                known = pl.ds(pl.multiple_of(attend[0] * (_EARLY // 2), _EARLY // 2), _EARLY // 2)
            mix = mixes(halves)
        qkv, probs, heads, hidden, mixed, fed = {}, {}, {}, [], {}, {}

        def project(which, g):
            full = g < n_full
            tiles = widen(mix.get, qkv_ref.at[3 * g + which] if full else qkv2_ref.at[which],
                          _TEN if full else _TWO, n_layers)
            if n_layers == 1:
                tiles = [halves[0] for halves in tiles]
                return tiles if which == 0 else _to_bf16(tiles)
            moved = n_mem + _EARLY // 2
            tiles = [jnp.concatenate([a, b[n_mem:moved], b[:n_mem], b[moved:]], axis=0)
                     for a, b in tiles]
            ref = early_ref.at[3 * g + which] if full else early2_ref.at[which]
            early = [_unpack(ref[known, _cols(t)]) for t in range(len(tiles))]
            if which == 0:
                early = [e.astype(jnp.float32) for e in early]
            else:
                tiles = _to_bf16(tiles)
            return [jnp.concatenate(parts, axis=0) for parts in zip(tiles, early)]

        for name in order.split():
            stage, g = name[0], int(name[1:])
            if stage in "QKV":
                qkv[name] = project("QKV".index(stage), g)
            elif stage == "S":
                probs[g] = []
                for q, k in zip(qkv[f"Q{g}"], qkv[f"K{g}"]):
                    s = jnp.where(visible, _dot_nt(q, k) * score_scale, fill)
                    p = jnp.exp2(s - jnp.max(s, axis=-1, keepdims=True))
                    probs[g].append((p, 1.0 / jnp.sum(p, axis=-1, keepdims=True)))
            elif stage == "A":
                heads[g] = [jnp.split(_dot(p, v) * inv, n_layers, axis=0)
                            for (p, inv), v in zip(probs[g], qkv[f"V{g}"])]
            elif stage == "O":
                full = g < n_full
                narrow(mixed, heads[g], out_ref.at[g] if full else wo2_ref, _TEN if full else _TWO)
            elif stage == "N":
                for n, s in enumerate(attend):
                    out = blocks_of(mixed, n)
                    x[n] = [a + o[n_mem:] for a, o in zip(x[n], out)]
                    store(s, x[n])
                    for i, o in enumerate(out):
                        mem_ref[n, :, _cols(i)] = o[:n_mem]
                if partner is not None:
                    x.insert(0, load(partner))
                following = mixes([layernorm(blocks) for blocks in x])
                for rows, value in following.items():
                    mix_ref[_MIXES.index(rows)] = value
            elif stage == "G":
                full = g < n_gate
                tiles = widen(lambda rows: mix_ref[_MIXES.index(rows)],
                              gate_ref.at[g] if full else gate2_ref, _TEN if full else _TWO, 2)
                n_side = len(tiles) // 2
                hidden += [[gate * jax.nn.sigmoid(gate) * up for gate, up in zip(*pair)]
                           for pair in zip(tiles[:n_side], tiles[n_side:])]
            elif stage == "D":
                full = g < n_full
                narrow(fed, hidden[10 * g:10 * g + 10],
                       out_ref.at[n_full + g] if full else down6_ref, _TEN if full else _SIX)
        for n, s in enumerate(feed):
            store(s, [a + o for a, o in zip(load(s), blocks_of(fed, n))])

    def qkv_copies(w_hbm, first, count, slot, offset=0):
        return [pltpu.make_async_copy(w_hbm.bitcast(jnp.uint32).at[:, first + p, :],
                                      qkv_stage.at[slot, offset + p], qkv_sem.at[slot])
                for p in range(count)]

    def column_copy(w_hbm, first, count, stage, sem, slot, offset=0):
        cols = pl.ds(pl.multiple_of(first * _T, _T), count * _T)
        return pltpu.make_async_copy(w_hbm.bitcast(jnp.uint32).at[:, cols],
                                     stage.at[slot, :, _cols(offset, count)], sem.at[slot])

    def wo_copies(first, count, slot):
        return [pltpu.make_async_copy(wot_hbm.bitcast(jnp.uint32).at[first + t],
                                      out_stage.at[slot, :, _cols(t)], out_sem.at[slot])
                for t in range(count)]

    def when(condition, act, copies):
        @pl.when(condition)
        def _():
            for c in copies():
                getattr(c, act)()

    def move_qkv(act, n):
        slot = n % _SLOTS
        for which, w in enumerate((wq_hbm, wk_hbm, wv_hbm)):
            when((n < n_qkv) & (n % 3 == which), act,
                 functools.partial(qkv_copies, w, 5 * (n // 3), 5, slot))
        when(n == n_qkv, act, lambda: [
            c for which, w in enumerate((wq_hbm, wk_hbm, wv_hbm))
            for c in qkv_copies(w, 5 * n_full, 1, slot, which)])

    def move_gate(act, n):
        slot = n % _SLOTS
        for active, count in (((n >= 0) & (n < n_gate), 5), (n == n_gate, 1)):
            when(active, act, lambda count=count: [
                column_copy(w, 5 * n, count, gate_stage, gate_sem, slot, side * count)
                for side, w in enumerate((w1_hbm, w3_hbm))])

    def move_out(act, n):
        slot = n % _SLOTS
        when((n >= 0) & (n < n_full), act, lambda: wo_copies(10 * n, 10, slot))
        when((n >= n_full) & (n < n_out), act,
             lambda: [column_copy(w2t_hbm, 10 * (n - n_full), 10, out_stage, out_sem, slot)])
        when(n == n_out, act, lambda: wo_copies(10 * n_full, 2, slot) + [
            column_copy(w2t_hbm, 10 * n_full, 6, out_stage, out_sem, slot, 2)])

    def block_rows(i, packing=1):
        return slice(i * _T // packing, min((i + 1) * _T, d_model) // packing)

    def padded(x):
        if x.shape[0] == _T:
            return x
        return jnp.concatenate([x, jnp.zeros((_T - x.shape[0], _T), x.dtype)], axis=0)

    def head_tile(slot, first):
        def tile(t, i):
            words = qkv_stage[slot, first + t // 2, block_rows(i), :]
            words = words & jnp.uint32(0xFFFF0000) if t % 2 else words << 16
            return padded(pltpu.bitcast(words, jnp.float32))
        return tile

    def column_tile(stage, slot, first=0, transposed=False):
        def tile(t, i):
            w = _unpack(stage[slot, block_rows(i, 2), _cols(first + t)])
            return padded(w).T if transposed else padded(w)
        return functools.cache(tile)

    def combine(tile, w_ref, scheme):
        sums = []
        for n, (_, weights, _) in enumerate(scheme):
            terms = [(s, tile(t, i)) for s, t, i in weights]
            if len(terms) == 1 and terms[0][1].dtype == jnp.bfloat16:
                w_ref[:, _cols(n)] = _pack(terms[0][1])
                continue
            sums.append((n, _signed_sum([(s, w.astype(jnp.float32)) for s, w in terms])))
            if len(sums) == 2:
                for (m, _), w in zip(sums, _to_bf16([w for _, w in sums])):
                    w_ref[:, _cols(m)] = _pack(w)
                sums = []
        assert not sums

    def project_early(w_ref, dst_ref, scheme):
        total = early_mix_ref.shape[1]
        for start in range(0, total, _EARLY_ROWS // 2):
            words = slice(start, min(start + _EARLY_ROWS // 2, total))
            tiles = widen(lambda rows: _unpack(early_mix_ref[_MIXES.index(rows), words, :]),
                          w_ref, scheme, 2)
            tiles = [jnp.concatenate([half[r:r + _EARLY] for r in range(0, a.shape[0], _EARLY)
                                      for half in (a, b)], axis=0) for a, b in tiles]
            for t, value in enumerate(_to_bf16(tiles)):
                dst_ref[2 * words.start:2 * words.stop, _cols(t)] = _pack(value)

    def x_copy(i):
        cols = pl.ds(pl.multiple_of(i * _T, _T), _T)
        return pltpu.make_async_copy(xt_hbm.at[:, cols], tile_ref.at[i], tile_sem.at[i])

    def out_copy(i):
        return pltpu.make_async_copy(tile_ref.at[i], outt_hbm.at[:, _cols(i)], tile_sem.at[i])

    def transpose_out(i):
        rows = pl.ds(pl.multiple_of(i * _T, _T), _T)
        tile_ref[i] = res_ref[rows, :].T[:d_model].astype(tile_ref.dtype)

    mem_copy = pltpu.make_async_copy(mem0_hbm, mem0_ref, mem_sem)
    for i in range(n_io):
        x_copy(i).start()
    mem_copy.start()
    move_qkv("start", 0)
    move_qkv("start", 1)

    @pl.loop(0, n_io)
    def _load_tile(i):
        x_copy(i).wait()
        blocks = [padded(tile_ref[i, block_rows(b), :].astype(jnp.float32)).T
                  for b in range(_BLOCKS)]
        for b, x in enumerate(blocks):
            res_ref[pl.ds(pl.multiple_of(i * _T, _T), _T), _cols(b)] = x
        halves = [layernorm([
            jnp.concatenate([x[(s + 1) * seg - _EARLY:(s + 1) * seg]
                             for s in range(half, _T // seg, 2)], axis=0) for x in blocks])
                  for half in range(2)]
        words = _EARLY // 2
        for n, value in enumerate(_to_bf16(list(mixes(halves).values()))):
            value = _pack(value)
            for pair in range(_T // seg // 2):
                at = jnp.maximum(i * (_T // seg // 2) + pair - _LAG // 2, 0) * words
                early_mix_ref[n, pl.ds(pl.multiple_of(at, words), words), :] = (
                    value[pair * words:(pair + 1) * words])

    move_qkv("wait", 0)
    combine(head_tile(0, 0), qkv_ref.at[0], _TEN)

    def load_group(n, _, *, heads, gate, out):
        n_g, n_o = n - (n_qkv - n_gate), n - (n_qkv - n_out)
        move_qkv("start", n + 2)
        move_gate("start", n_g + 1)
        move_out("start", n_o + 1)
        move_qkv("wait", n + 1)
        move_gate("wait", n_g)
        move_out("wait", n_o)
        project_early(qkv_ref.at[n], early_ref.at[n], _TEN)
        if heads:
            combine(head_tile((n + 1) % _SLOTS, 0), qkv_ref.at[n + 1], _TEN)
        if gate:
            combine(column_tile(gate_stage, n_g % _SLOTS), gate_ref.at[n_g], _TEN)
        if out:
            combine(column_tile(out_stage, n_o % _SLOTS, 0, True), out_ref.at[n_o], _TEN)

    bounds = (0, n_qkv - n_gate, n_qkv - n_out, n_qkv - 1)
    for n, (lo, hi) in enumerate(zip(bounds, bounds[1:])):
        jax.lax.fori_loop(
            lo, hi, functools.partial(load_group, heads=True, gate=n > 0, out=n > 1), None)
    load_group(n_qkv - 1, None, heads=False, gate=True, out=True)
    for which in range(3):
        combine(head_tile(n_qkv % _SLOTS, which), qkv2_ref.at[which], _TWO)
    move_gate("wait", n_gate)
    move_out("wait", n_out)
    for which in range(3):
        project_early(qkv2_ref.at[which], early2_ref.at[which], _TWO)
    combine(column_tile(gate_stage, n_gate % _SLOTS), gate2_ref, _TWO)
    combine(column_tile(out_stage, n_out % _SLOTS, 0, True), wo2_ref, _TWO)
    combine(column_tile(out_stage, n_out % _SLOTS, 2, True), down6_ref, _SIX)

    mem_copy.wait()
    mem0 = jnp.concatenate([mem0_ref[...].astype(jnp.float32),
                            jnp.zeros((n_mem, _BLOCKS * _T - d_model), jnp.float32)], axis=1)
    mem_ref[0] = mem0
    pl.loop(0, _LAG)(lambda s: step(_ORDER_ATTENTION, attend=[s], partner=0))
    step(_ORDER_FFN, feed=[0, 1])
    mem_ref[1] = mem_ref[0]
    mem_ref[0] = mem0
    step(_ORDER_ATTENTION, attend=[0, _LAG])

    @pl.loop(1, n_seg - _LAG)
    def _double_step(b):
        transpose_out(jnp.maximum(b - 5, 0) * seg // _T)
        step(_ORDER, attend=[b, b + _LAG], feed=[b - 1, b + _LAG - 1])

    for i in range(n_io - 1):
        out_copy(i).start()
    step(_ORDER_FFN, feed=[n_seg - _LAG - 1, n_seg - 1])
    pl.loop(n_seg - _LAG, n_seg)(
        lambda s: step(_ORDER_ATTENTION, attend=[s], partner=n_seg - 2))
    step(_ORDER_FFN, feed=[n_seg - 2, n_seg - 1])
    transpose_out(n_io - 1)
    out_copy(n_io - 1).start()
    for i in range(n_io):
        out_copy(i).wait()


@functools.partial(jax.jit, static_argnames=("A_seg_len",))
def pallas_interleave_layers__memory_aug_recurrent_mem_tr__glu_gated_swiglu__prompt_kernel(
    A_x: jax.Array,
    A_mem0: jax.Array,
    A_Wq: jax.Array,
    A_Wk: jax.Array,
    A_Wv: jax.Array,
    A_Wo: jax.Array,
    A_seg_len: int,
    B_x: jax.Array,
    B_w1: jax.Array,
    B_w3: jax.Array,
    B_w2: jax.Array,
):
    del B_x
    _, n_tok, d_model = A_x.shape
    n_mem = A_mem0.shape[1]
    _, n_heads, d_head = A_Wq.shape
    d_ff = B_w1.shape[1]
    assert A_x.shape[0] == 1 and 4 * A_seg_len == _T and n_mem == 8
    assert (d_model, n_heads, d_head, d_ff) == (576, 32, _T, 36 * _T)
    early_words = (n_tok // A_seg_len - _LAG) * _EARLY // 2
    hbm = pl.BlockSpec(memory_space=pltpu.HBM)

    def weights(scheme, *groups):
        return pltpu.VMEM((*groups, _T // 2, len(scheme) * _T), jnp.uint32)

    out_t = pl.pallas_call(
        functools.partial(_kernel, seg=A_seg_len),
        out_shape=jax.ShapeDtypeStruct((d_model, n_tok), A_x.dtype),
        in_specs=[hbm] * 9,
        out_specs=hbm,
        scratch_shapes=[
            pltpu.VMEM((n_mem, d_model), A_mem0.dtype),
            pltpu.VMEM((n_tok // _T, d_model, _T), A_x.dtype),
            pltpu.VMEM((n_tok, _BLOCKS * _T), jnp.float32),
            pltpu.VMEM((2, n_mem, _BLOCKS * _T), jnp.float32),
            pltpu.VMEM((len(_MIXES), A_seg_len, _T), jnp.float32),
            pltpu.VMEM((len(_MIXES), early_words // 2, _T), jnp.uint32),
            pltpu.VMEM((9, early_words, 10 * _T), jnp.uint32),
            pltpu.VMEM((3, early_words, 2 * _T), jnp.uint32),
            weights(_TEN, 9), weights(_TWO, 3), weights(_TEN, 7), weights(_TWO),
            weights(_TEN, 6), weights(_TWO), weights(_SIX),
            pltpu.VMEM((_SLOTS, 5, d_model, _T), jnp.uint32),
            pltpu.VMEM((_SLOTS, d_model // 2, 10 * _T), jnp.uint32),
            pltpu.VMEM((_SLOTS, d_model // 2, 10 * _T), jnp.uint32),
            pltpu.SemaphoreType.DMA((_SLOTS,)),
            pltpu.SemaphoreType.DMA((_SLOTS,)),
            pltpu.SemaphoreType.DMA((_SLOTS,)),
            pltpu.SemaphoreType.DMA((n_tok // _T,)),
            pltpu.SemaphoreType.DMA,
        ],
        compiler_params=pltpu.CompilerParams(vmem_limit_bytes=120 * 1024 * 1024),
    )(A_x.reshape(n_tok, d_model).T, A_mem0.reshape(n_mem, d_model), A_Wq, A_Wk, A_Wv,
      A_Wo.transpose(0, 2, 1), B_w1, B_w3, B_w2.T)
    return out_t.T.reshape(A_x.shape)
```

```python
import functools
import itertools
import math
from typing import NamedTuple

import jax
import jax.numpy as jnp
import jax.experimental.pallas as pl
import jax.experimental.pallas.tpu as pltpu

_EPS = 1e-05
_MASKED = -1000000000.0
_LOG2E = math.log2(math.e)
_T = 128
_FULL = 4
_UNIT = 16
_LAG = 2
_EARLY = 16
_EARLY_ROWS = 64
_ORDER = "G0 Q0 K0+T0 Q1+S6 K1+S6 V0+S6 V1+S7+A6 G1+S7+A10 O0+A8 G2+A8 O1 G3+N0 G4 D0 D1 D2"
_ORDER_ATTENTION = "Q0 K0 Q1+S8 K1+S8 V0+S16 V1+A16 O0+A16 O1 N0"
_ORDER_FFN = "G0 G1 G2 G3 G4 D0 D1 D2"
_LEAD = 0.1
_DEV = ""
_FLAGS = None


class _Product(NamedTuple):
    rows: tuple
    weights: tuple
    tiles: tuple


class _Scheme(NamedTuple):
    piece: tuple
    helper: tuple
    shared: tuple
    main: tuple


def _pair_up(blocks, left, right, edges):
    products = []
    edges = [(u, blocks[u][i], v, blocks[v][j]) for u, i, v, j in edges]
    assert all(i in blocks[v] and j in blocks[u] for u, i, v, j in edges)

    def add(rows, weights, tiles):
        rows = tuple(sorted(rows, key=lambda term: term[1:]))
        if rows[0][0] < 0:
            rows = tuple((-s, half, i) for s, half, i in rows)
            tiles = tuple((-s, half, t) for s, half, t in tiles)
        products.append(_Product(rows, tuple(weights), tuple(tiles)))

    def own_blocks(t, half):
        mine = [((i, v, j), (j, u, i))[half] for u, i, v, j in edges if (u, v)[half] == t]
        for i in blocks[t]:
            if any(i == j for _, _, j in mine):
                continue
            partners = [(p, j) for home, p, j in mine if home == i]
            if not partners:
                add([(1, 0, i)], [(1, t, i)], [(1, 0, t)])
                add([(1, 1, i)], [(1, t, i)], [(1, 1, t)])
                continue
            add([(1, half, i)], [(1, t, i)] + [(1, t, j) for _, j in partners],
                [(1, half, t), (-1, 1 - half, t)])
            add([(1, 0, i), (1, 1, i)], [(1, t, i)] + [(-1, p, i) for p, _ in partners],
                [(1, 1 - half, t)])

    for t in left:
        own_blocks(t, 0)
        for u, i, v, j in edges:
            if u == t:
                add([(1, 0, j), (-1, 0, i)], [(1, u, j)], [(1, 0, u), (1, 0, v)])
                add([(1, 1, i), (-1, 1, j)], [(1, v, i)], [(1, 1, v), (1, 1, u)])
                add([(1, 0, i), (1, 1, j)], [(1, u, j), (1, v, i)], [(1, 1, u), (1, 0, v)])
    for t in right:
        own_blocks(t, 1)
    return products


def _scheme(n):
    if n == 4:
        piece = [0, 0, 1, 1]
        groups = [([u], [u + 1], [(u, 0, u + 1, 2), (u, 1, u + 1, 3)]) for u in (0, 2)]
    else:
        piece = [2 * (t // 8) + ((t % 4 == t // 8) == (t % 8 >= 4)) for t in range(n)]
        groups = [(range(g, g + 4), range(g + 4, g + 8),
                   [(g + i, i, g + 4 + j, j) for i in range(4) for j in range(4) if i != j])
                  for g in range(0, n, 8)]
    helper = [n + piece[:t].count(piece[t]) for t in range(n)]
    helpers = range(n, max(helper) + 1)
    blocks = [[_FULL + p if i == p // 2 else i for i in range(_FULL)] for p in piece]
    blocks += [range(max(piece) // 2 + 1)] * len(helpers)
    shared = [p for u in helpers[::2] for p in _pair_up(
        blocks, [u], [u + 1], [(u, 0, u + 1, 1)] if len(blocks[u]) == 2 else [])]
    return _Scheme(tuple(piece), tuple(helper), tuple(shared),
                   tuple(p for group in groups for p in _pair_up(blocks, *group)))


_SIXTEEN, _EIGHT, _FOUR = _scheme(_UNIT), _scheme(8), _scheme(4)


def _numbered(scheme, n_halves):
    kept = [], []
    for n, (rows, weights, tiles) in enumerate(scheme.shared + scheme.main):
        rows = tuple(term for term in rows if term[1] < n_halves)
        tiles = tuple(term for term in tiles if term[1] < n_halves)
        if rows and tiles:
            kept[n >= len(scheme.shared)].append((n, _Product(rows, weights, tiles)))
    return kept


def _count(scheme, n_halves=2):
    return sum(map(len, _numbered(scheme, n_halves)))


def _plain(block):
    return block if block < _FULL else (block - _FULL) // 2


def _signed_sum(terms):
    (sign, total), *rest = sorted(terms, key=lambda term: -term[0])
    for s, value in rest:
        total = total + value if s == sign else total - value
    return total if sign > 0 else -total


def _accumulate(acc, key, sign, value):
    if key in acc:
        s, total = acc[key]
        if s == sign:
            acc[key] = s, total + value
        else:
            acc[key] = 1, total - value if s > 0 else value - total
    else:
        acc[key] = sign, value


def _interleave(main, count=0, others=()):
    due = sorted((count * (_LEAD + (1 - _LEAD) * (k + m / len(others)) / n), m, k)
                 for m, (_, n) in enumerate(others) for k in range(n))
    for done, _ in enumerate(main):
        while due and due[0][0] <= done:
            next(others[due.pop(0)[1]][0])
    for other, _ in others:
        for _ in other:
            pass


def _dot(a, b):
    return jax.lax.dot_general(a, b, (((1,), (0,)), ((), ())),
                               preferred_element_type=jnp.float32)


def _dot_nt(a, b):
    return jax.lax.dot_general(a, b, (((1,), (1,)), ((), ())),
                               preferred_element_type=jnp.float32)


def _pack(x):
    return pltpu.bitcast(x, jnp.uint32)


def _unpack(words):
    return pltpu.bitcast(words, jnp.bfloat16)


def _cols(n, width=1):
    return slice(n * _T, (n + width) * _T)


def _to_bf16(tiles):
    out = []
    for n in range(0, len(tiles), 2):
        both = jnp.concatenate(tiles[n:n + 2], axis=1).astype(jnp.bfloat16)
        out += [both[:, _cols(c)] for c in range(both.shape[1] // _T)]
    return out


def _halves(low, high):
    lane = jax.lax.broadcasted_iota(jnp.int32, low.shape, 1)
    return jnp.where(lane < _T // 2, low, high)


def _layernorm(blocks):
    def mean(terms):
        total = sum(terms[:-1], 0.5 * terms[-1])
        return jnp.sum(total, axis=-1, keepdims=True) * (1 / ((_FULL + 0.5) * _T))

    center = mean(blocks)
    d = [x - center for x in blocks]
    inv = jax.lax.rsqrt(mean([x * x for x in d]) + _EPS)
    return [x * inv for x in d]


def _mixer(halves):
    @functools.cache
    def block(half, i):
        x, rest = halves[half][_plain(i)], halves[half][_FULL]
        if i < _FULL:
            return x
        return _halves(x, rest) if (i - _FULL) % 2 else _halves(rest, x)

    return functools.cache(lambda rows: _signed_sum([(s, block(half, i)) for s, half, i in rows]))


def _widen(mix, w_ref, scheme, n_halves):
    acc = {}
    for products in _numbered(scheme, n_halves):
        acc = {(t, half): acc[h, half] for t, h in enumerate(scheme.helper)
               for half in range(n_halves) if acc}
        for n, (rows, _, tiles) in products:
            value = _dot(mix(rows), _unpack(w_ref[:, _cols(n)]))
            for s, half, t in tiles:
                _accumulate(acc, (t, half), s, value)
            yield
    return [[_signed_sum([acc[t, half]]) for half in range(n_halves)]
            for t in range(len(scheme.piece))]


def _narrow(acc, wide, w_ref, scheme):
    n_halves = len(wide[0])
    wide = wide + [
        [_signed_sum([(1, x[half]) for x, h in zip(wide, scheme.helper) if h == helper])
         for half in range(n_halves)] for helper in range(len(wide), max(scheme.helper) + 1)]
    by_rows = {}
    for n, product in sum(_numbered(scheme, n_halves)[::-1], []):
        by_rows.setdefault(product.rows, []).append((n, product.tiles))
    for rows in sorted(by_rows, key=lambda rows: sorted({i for _, _, i in rows})[::-1])[::-1]:
        total = {}
        for n, tiles in by_rows[rows]:
            sign = max(s for s, _, _ in tiles)
            lhs = _signed_sum([(s * sign, wide[t][half]) for s, half, t in tiles])
            _accumulate(total, 0, sign, _dot(lhs, _unpack(w_ref[:, _cols(n)])))
            yield
        for s, half, i in rows:
            _accumulate(acc, (half, i), s * total[0][0], total[0][1])


def _narrowed(acc, half):
    blocks = [_signed_sum([acc[half, i]]) for i in range(2 * _FULL)]
    folded = list(zip(blocks[_FULL::2], blocks[_FULL + 1::2]))
    rest = _signed_sum([(1, _halves(low, high)) for low, high in folded])
    rest += jnp.concatenate([rest[:, _T // 2:], rest[:, :_T // 2]], axis=1)
    return ([x + _halves(high, low) for x, (low, high) in zip(blocks, folded)]
            + blocks[len(folded):_FULL] + [rest])


def _combine(part, w_ref, scheme, transposed=False):
    donor = {(h, p): t for t, (h, p) in enumerate(zip(scheme.helper, scheme.piece))}

    def folded(t, p):
        if t >= len(scheme.piece):
            return part(donor[t, p], p)
        if p == scheme.piece[t]:
            return part(t, 2 * _FULL)
        if (scheme.helper[t], p) in donor:
            return (part(t, p).astype(jnp.float32)
                    - folded(scheme.helper[t], p).astype(jnp.float32))
        return part(t, p)

    @functools.cache
    def tile(t, i):
        parts = [folded(t, 2 * _plain(i) + side) for side in range(2)]
        if parts[0].dtype != parts[1].dtype:
            parts = [w.astype(jnp.float32) for w in parts]
        return jnp.concatenate(parts, axis=0)

    def store(n, w):
        w_ref[:, _cols(n)] = _pack(w.T if transposed else w)

    sums = {}
    for n, (_, weights, _) in enumerate(scheme.shared + scheme.main):
        terms = [(s, tile(t, i)) for s, t, i in weights]
        if len(terms) == 1 and terms[0][1].dtype == jnp.bfloat16:
            store(n, terms[0][1])
        else:
            sums[n] = _signed_sum([(s, w.astype(jnp.float32)) for s, w in terms])
        if len(sums) == 2:
            for m, w in zip(sums, _to_bf16(list(sums.values()))):
                store(m, w)
            sums = {}
        yield
    assert not sums


def _kernel(xt_hbm, mem0_hbm, wq_hbm, wk_hbm, wv_hbm, wot_hbm, w1_hbm, w3_hbm, w2t_hbm,
            outt_hbm, mem0_ref, tile_ref, res_ref, mem_ref, norm_ref, early_norm_ref, early_ref,
            qkv_ref, gate_ref, gate8_ref, out_ref, down4_ref,
            qkv_stage, gate_stage, out_stage, qkv_sem, gate_sem, out_sem, tile_sem, mem_sem,
            *, seg):
    d_model, n_tok = xt_hbm.shape
    n_mem = mem0_ref.shape[0]
    d_head = wq_hbm.shape[2]
    n_seg = n_tok // seg
    n_io = n_tok // _T
    n_qkv, n_gate, n_out = qkv_ref.shape[0], gate_ref.shape[0], out_ref.shape[0]
    n_wo = n_qkv // 3
    span = n_mem + seg
    score_scale = d_head ** -0.5 * _LOG2E

    def blocks_at(ref, *index):
        return [ref[(*index, _cols(i))] for i in range(_FULL + 1)]

    def set_blocks(ref, index, blocks):
        for i, x in enumerate(blocks):
            ref[(*index, _cols(i))] = x

    def rows_of(s):
        return pl.ds(pl.multiple_of(s * seg, seg), seg)

    def step(order, attend=(), feed=(), partner=None, finished=None):
        n_layers = len(attend)
        qkv, probs, heads, hidden, mixed, fed = [[], [], []], [], [], [], {}, {}
        if attend:
            i, j = (jax.lax.broadcasted_iota(jnp.int32, (n_layers * span, _T), a) for a in (0, 1))
            same = ((i >= span) == (j >= span)) & (j < 2 * span)
            visible = same & ((i < n_mem) | ((i >= span) & (i < span + n_mem)) | (i >= j))
            fill = jnp.where(same, _MASKED * _LOG2E, -jnp.inf).astype(jnp.float32)
            mem = [blocks_at(mem_ref, n, slice(None)) for n in range(n_layers)]
            h = _layernorm(blocks_at(res_ref, rows_of(attend[0])))
            if n_layers == 1:
                attend_mix = _mixer([[jnp.concatenate(parts, axis=0) for parts in zip(mem[0], h)]])
            else:
                ahead = _layernorm(
                    [x[:seg - _EARLY] for x in blocks_at(res_ref, rows_of(attend[1]))])
                cut = seg - _EARLY // 2
                attend_mix = _mixer([
                    [jnp.concatenate([m, a[:cut]], axis=0) for m, a in zip(mem[0], h)],
                    [jnp.concatenate([m, a[cut:], b], axis=0) for m, a, b in zip(mem[1], h, ahead)]])
        if feed:
            feed_mix = _mixer([blocks_at(norm_ref, n, slice(None)) for n in range(2)])

        def project(which, g):
            tiles = yield from _widen(attend_mix, qkv_ref.at[3 * g + which], _SIXTEEN, n_layers)
            if n_layers == 1:
                tiles = [halves[0] for halves in tiles]
                qkv[which] += tiles if which == 0 else _to_bf16(
                    [jnp.concatenate([x, jnp.zeros((n_mem, _T), x.dtype)], axis=0) for x in tiles])
                return
            moved = n_mem + _EARLY // 2
            tiles = [jnp.concatenate([a, b[n_mem:moved], b[:n_mem], b[moved:]], axis=0)
                     for a, b in tiles]
            known = pl.ds(pl.multiple_of(attend[0] * (_EARLY // 2), _EARLY // 2), _EARLY // 2)
            early = [_unpack(early_ref[3 * g + which, known, _cols(t)]) for t in range(_UNIT)]
            if which == 0:
                early = [e.astype(jnp.float32) for e in early]
            else:
                tiles = _to_bf16(tiles)
            qkv[which] += [jnp.concatenate(parts, axis=0) for parts in zip(tiles, early)]

        def score(count):
            for t in range(len(probs), len(probs) + count):
                s = _dot_nt(qkv[0][t], qkv[1][t])
                s = jnp.concatenate([s, jnp.zeros((s.shape[0], _T - s.shape[1]), s.dtype)], axis=1)
                s = jnp.where(visible, s * score_scale, fill)
                p = jnp.exp2(s - jnp.max(s, axis=-1, keepdims=True))
                probs.append(
                    (p, pltpu.reciprocal(jnp.sum(p, axis=-1, keepdims=True), approx=True)))
                yield

        def average(count):
            for t in range(len(heads), len(heads) + count):
                (p, inv), v = probs[t], qkv[2][t]
                both = _dot(p[:, :v.shape[0]], v) * inv
                heads.append([both[n * span:(n + 1) * span] for n in range(n_layers)])
                yield

        def hand_over():
            x = [] if partner is None else [blocks_at(res_ref, rows_of(partner))]
            for n, s in enumerate(attend):
                out = _narrowed(mixed, n)
                x.append([a + o[n_mem:] for a, o in zip(blocks_at(res_ref, rows_of(s)), out)])
                set_blocks(res_ref, [rows_of(s)], x[-1])
                set_blocks(mem_ref, [n, slice(None)], [o[:n_mem] for o in out])
            for n, blocks in enumerate(x):
                set_blocks(norm_ref, [n, slice(None)], _layernorm(blocks))
                yield

        def gated(w_ref, scheme):
            tiles = yield from _widen(feed_mix, w_ref, scheme, 2)
            for pair in zip(tiles[::2], tiles[1::2]):
                halved = [(0.5 * gate, up) for gate, up in zip(*pair)]
                hidden.append([(g * jnp.tanh(g) + g) * up for g, up in halved])

        def begin(name):
            stage, g = name[0], int(name[1:])
            tiles = slice(g * _UNIT, (g + 1) * _UNIT)
            if stage in "QKV":
                return project("QKV".index(stage), g), _count(_SIXTEEN, n_layers)
            if stage in "SA":
                return (score if stage == "S" else average)(g), g
            if stage == "N":
                return hand_over(), 2
            if stage == "T":
                return transpose_out(finished), _FULL + 1
            if stage == "O":
                return (_narrow(mixed, heads[tiles], out_ref.at[g], _SIXTEEN),
                        _count(_SIXTEEN, n_layers))
            if stage == "G":
                unit = (gate_ref.at[g], _SIXTEEN) if g < n_gate else (gate8_ref, _EIGHT)
                return gated(*unit), _count(unit[1])
            unit = (out_ref.at[n_wo + g], _SIXTEEN) if n_wo + g < n_out else (down4_ref, _FOUR)
            return _narrow(fed, hidden[tiles], *unit), _count(unit[1])

        for names in order.split():
            main, *others = [begin(name) for name in names.split("+")]
            _interleave(*main, others)
        for n, s in enumerate(feed):
            set_blocks(res_ref, [rows_of(s)], [
                a + o for a, o in zip(blocks_at(res_ref, rows_of(s)), _narrowed(fed, n))])

    def when(condition, act, copies):
        @pl.when(condition)
        def _():
            for c in copies():
                act(c)

    def start(copy):
        copy.start()

    def wait(copy):
        copy.wait()

    def column_copy(w_hbm, first, count, stage, sem, offset=0):
        cols = pl.ds(pl.multiple_of(first * _T, _T), count * _T)
        return pltpu.make_async_copy(w_hbm.bitcast(jnp.uint32).at[:, cols],
                                     stage.at[:, _cols(offset, count)], sem)

    def move_qkv(act, n):
        for which, w in enumerate((wq_hbm, wk_hbm, wv_hbm)):
            when((n < n_qkv) & (n % 3 == which), act, lambda w=w: [
                pltpu.make_async_copy(w.bitcast(jnp.uint32).at[:, n // 3 * (_UNIT // 2) + p, :],
                                      qkv_stage.at[n % 2, p], qkv_sem.at[n % 2])
                for p in range(_UNIT // 2)])

    def move_others(act, n):
        gate, out = (gate_stage.at[n % 2], gate_sem.at[n % 2]), (out_stage.at[n % 2], out_sem.at[n % 2])
        for active, count in ((n < n_gate, _UNIT // 2), (n == n_gate, 4)):
            when(active, act, lambda count=count: [
                column_copy(w, n * (_UNIT // 2), count, *gate, side * (_UNIT // 2))
                for side, w in enumerate((w1_hbm, w3_hbm))])
        when(n < n_wo, act, lambda: [
            pltpu.make_async_copy(wot_hbm.bitcast(jnp.uint32).at[n * _UNIT + t],
                                  out[0].at[:, _cols(t)], out[1]) for t in range(_UNIT)])
        for active, count in (((n >= n_wo) & (n < n_out), _UNIT), (n == n_out, 4)):
            when(active, act,
                 lambda count=count: [column_copy(w2t_hbm, (n - n_wo) * _UNIT, count, *out)])

    def combine_qkv(n):
        def part(t, p):
            words = qkv_stage[n % 2, t // 2, pl.ds(p * _T // 2, _T // 2), :]
            words = words & jnp.uint32(0xFFFF0000) if t % 2 else words << 16
            return pltpu.bitcast(words, jnp.float32)

        return _combine(part, qkv_ref.at[n], _SIXTEEN)

    def combine_others(n, gate, out):
        def part(stage, column, t, p):
            return _unpack(stage[n % 2, pl.ds(p * _T // 4, _T // 4), _cols(column(t))])

        yield from _combine(
            functools.partial(part, gate_stage, lambda t: t % 2 * (_UNIT // 2) + t // 2), *gate)
        yield from _combine(functools.partial(part, out_stage, lambda t: t), *out, True)

    def project_early(n):
        total = early_norm_ref.shape[1]
        for first in range(0, total, _EARLY_ROWS):
            rows = slice(first, min(first + _EARLY_ROWS, total))
            tiles = yield from _widen(
                _mixer([blocks_at(early_norm_ref, half, rows) for half in range(2)]),
                qkv_ref.at[n], _SIXTEEN, 2)
            tiles = [jnp.concatenate([half[r:r + _EARLY] for r in range(0, a.shape[0], _EARLY)
                                      for half in (a, b)], axis=0) for a, b in tiles]
            for t in range(0, _UNIT, 2):
                early_ref[n, rows, _cols(t, 2)] = _pack(
                    jnp.concatenate(tiles[t:t + 2], axis=1).astype(jnp.bfloat16))

    def x_copy(i):
        cols = pl.ds(pl.multiple_of(i * _T, _T), _T)
        return pltpu.make_async_copy(xt_hbm.at[:, cols], tile_ref.at[i], tile_sem.at[i])

    def out_copy(i):
        return pltpu.make_async_copy(tile_ref.at[i], outt_hbm.at[:, _cols(i)], tile_sem.at[i])

    def transpose_out(i):
        for b, x in enumerate(blocks_at(res_ref, pl.ds(pl.multiple_of(i * _T, _T), _T))):
            depth = min(_T, d_model - b * _T)
            tile_ref[i, pl.ds(b * _T, depth), :] = x.T[:depth].astype(tile_ref.dtype)
            yield

    def double_step(b):
        step(_ORDER, attend=[b, b + _LAG], feed=[b - 1, b + _LAG - 1],
             finished=jnp.maximum(b - 5, 0) * seg // _T)

    if _DEV == "main":
        pl.loop(1, n_seg - _LAG)(double_step)
        out_copy(0).start()
        out_copy(0).wait()
        return

    mem_copy = pltpu.make_async_copy(mem0_hbm, mem0_ref, mem_sem)
    for i in range(n_io):
        x_copy(i).start()
    mem_copy.start()
    move_qkv(start, 0)

    @pl.loop(0, n_io)
    def _load_tile(i):
        x_copy(i).wait()
        x = tile_ref[i].astype(jnp.float32)
        x = jnp.concatenate([x, x[_FULL * _T:]], axis=0)
        blocks = [x[b * _T:(b + 1) * _T].T for b in range(_FULL + 1)]
        set_blocks(res_ref, [pl.ds(pl.multiple_of(i * _T, _T), _T)], blocks)
        normed = _layernorm([
            jnp.concatenate([x[s - _EARLY:s] for s in range(seg, _T + 1, seg)], axis=0)
            for x in blocks])
        for s in range(_T // seg):
            at = jnp.maximum(i * (_T // seg) + s - _LAG, 0) // 2 * _EARLY
            set_blocks(early_norm_ref, [s % 2, pl.ds(pl.multiple_of(at, _EARLY), _EARLY)],
                       [x[s * _EARLY:(s + 1) * _EARLY] for x in normed])

    move_qkv(start, 1)
    move_qkv(wait, 0)
    _interleave(combine_qkv(0))
    n_early = pl.cdiv(early_norm_ref.shape[1], _EARLY_ROWS) * _count(_SIXTEEN)
    move_qkv(start, 2)
    move_others(start, 0)
    move_qkv(wait, 1)
    _interleave(project_early(0), n_early, [(combine_qkv(1), _count(_SIXTEEN))])

    @pl.loop(1, n_qkv - 1)
    def _load_units(n):
        move_qkv(start, n + 2)
        move_others(start, n)
        move_qkv(wait, n + 1)
        move_others(wait, n - 1)
        work = itertools.chain(combine_qkv(n + 1), combine_others(
            n - 1, (gate_ref.at[n - 1], _SIXTEEN), (out_ref.at[n - 1], _SIXTEEN)))
        _interleave(project_early(n), n_early, [(work, 3 * _count(_SIXTEEN))])

    move_others(wait, n_gate)
    work = combine_others(n_gate, (gate8_ref, _EIGHT), (down4_ref, _FOUR))
    _interleave(project_early(n_qkv - 1), n_early, [(work, _count(_EIGHT) + _count(_FOUR))])

    mem_copy.wait()
    mem0 = mem0_ref[...].astype(jnp.float32)
    mem_ref[0] = mem0 = jnp.concatenate([mem0, mem0[:, _FULL * _T:]], axis=1)
    pl.loop(0, _LAG)(lambda s: step(_ORDER_ATTENTION, attend=[s], partner=0))
    step(_ORDER_FFN, feed=[0, 1])
    mem_ref[1] = mem_ref[0]
    mem_ref[0] = mem0
    step(_ORDER_ATTENTION, attend=[0, _LAG])
    pl.loop(1, n_seg - _LAG)(double_step)
    for i in range(n_io - 1):
        out_copy(i).start()
    step(_ORDER_FFN, feed=[n_seg - _LAG - 1, n_seg - 1])
    pl.loop(n_seg - _LAG, n_seg)(
        lambda s: step(_ORDER_ATTENTION, attend=[s], partner=n_seg - 2))
    step(_ORDER_FFN, feed=[n_seg - 2, n_seg - 1])
    _interleave(transpose_out(n_io - 1))
    out_copy(n_io - 1).start()
    for i in range(n_io):
        out_copy(i).wait()


@functools.partial(jax.jit, static_argnames=("A_seg_len",))
def pallas_interleave_layers__memory_aug_recurrent_mem_tr__glu_gated_swiglu__prompt_kernel(
    A_x: jax.Array,
    A_mem0: jax.Array,
    A_Wq: jax.Array,
    A_Wk: jax.Array,
    A_Wv: jax.Array,
    A_Wo: jax.Array,
    A_seg_len: int,
    B_x: jax.Array,
    B_w1: jax.Array,
    B_w3: jax.Array,
    B_w2: jax.Array,
):
    del B_x
    _, n_tok, d_model = A_x.shape
    n_mem = A_mem0.shape[1]
    _, n_heads, d_head = A_Wq.shape
    d_ff = B_w1.shape[1]
    assert A_x.shape[0] == 1 and 4 * A_seg_len == _T and n_mem == 8
    assert (d_model, n_heads, d_head, d_ff) == (576, 2 * _UNIT, _T, 36 * _T)
    early_rows = (n_tok // A_seg_len - _LAG) * _EARLY
    width = (_FULL + 1) * _T
    hbm = pl.BlockSpec(memory_space=pltpu.HBM)

    def weights(scheme, *units):
        return pltpu.VMEM((*units, _T // 2, _count(scheme) * _T), jnp.uint32)

    out_t = pl.pallas_call(
        functools.partial(_kernel, seg=A_seg_len),
        out_shape=jax.ShapeDtypeStruct((d_model, n_tok), A_x.dtype),
        in_specs=[hbm] * 9,
        out_specs=hbm,
        scratch_shapes=[
            pltpu.VMEM((n_mem, d_model), A_mem0.dtype),
            pltpu.VMEM((n_tok // _T, d_model, _T), A_x.dtype),
            pltpu.VMEM((n_tok, width), jnp.float32),
            pltpu.VMEM((2, n_mem, width), jnp.float32),
            pltpu.VMEM((2, A_seg_len, width), jnp.float32),
            pltpu.VMEM((2, early_rows // 2, width), jnp.float32),
            pltpu.VMEM((6, early_rows // 2, _UNIT * _T), jnp.uint32),
            weights(_SIXTEEN, 6), weights(_SIXTEEN, 4), weights(_EIGHT),
            weights(_SIXTEEN, 4), weights(_FOUR),
            pltpu.VMEM((2, _UNIT // 2, d_model, _T), jnp.uint32),
            pltpu.VMEM((2, d_model // 2, _UNIT * _T), jnp.uint32),
            pltpu.VMEM((2, d_model // 2, _UNIT * _T), jnp.uint32),
            pltpu.SemaphoreType.DMA((2,)),
            pltpu.SemaphoreType.DMA((2,)),
            pltpu.SemaphoreType.DMA((2,)),
            pltpu.SemaphoreType.DMA((n_tok // _T,)),
            pltpu.SemaphoreType.DMA,
        ],
        compiler_params=pltpu.CompilerParams(vmem_limit_bytes=120 * 1024 * 1024, flags=_FLAGS),
    )(A_x.reshape(n_tok, d_model).T, A_mem0.reshape(n_mem, d_model), A_Wq, A_Wk, A_Wv,
      A_Wo.transpose(0, 2, 1), B_w1, B_w3, B_w2.T)
    return out_t.T.reshape(A_x.shape)
```

```python
import functools
import itertools
import math
from typing import NamedTuple

import jax
import jax.numpy as jnp
import jax.experimental.pallas as pl
import jax.experimental.pallas.tpu as pltpu

_EPS = 1e-05
_MASKED = -1000000000.0
_LOG2E = math.log2(math.e)
_T = 128
_FULL = 4
_UNIT = 16
_LAG = 2
_EARLY = 16
_EARLY_ROWS = (48,) * 9 + (32,) * 2
_ORDER = "G0 Q0 K0+T0 Q1+S6 K1+S6 V0+S6 V1+S7+A6 G1+S7+A10 O0+A8 G2+A8 O1 G3+N0 G4 D0 D1 D2"
_ORDER_ATTENTION = "Q0 K0 Q1+S8 K1+S8 V0+S16 V1+A16 O0+A16 O1 N0"
_ORDER_FFN = "G0 G1 G2 G3 G4 D0 D1 D2"
_LEAD = 0.1
_DEV = ""
_FORTY = False
_PACK = (False, True, True)
_FLAGS = None


class _Product(NamedTuple):
    rows: tuple
    weights: tuple
    tiles: tuple


class _Scheme(NamedTuple):
    piece: tuple
    helper: tuple
    shared: tuple
    main: tuple


def _pair_up(blocks, left, right, edges):
    products = []
    edges = [(u, blocks[u][i], v, blocks[v][j]) for u, i, v, j in edges]
    assert all(i in blocks[v] and j in blocks[u] for u, i, v, j in edges)

    def add(rows, weights, tiles):
        rows = tuple(sorted(rows, key=lambda term: term[1:]))
        if rows[0][0] < 0:
            rows = tuple((-s, half, i) for s, half, i in rows)
            tiles = tuple((-s, half, t) for s, half, t in tiles)
        products.append(_Product(rows, tuple(weights), tuple(tiles)))

    def own_blocks(t, half):
        mine = [((i, v, j), (j, u, i))[half] for u, i, v, j in edges if (u, v)[half] == t]
        for i in blocks[t]:
            if any(i == j for _, _, j in mine):
                continue
            partners = [(p, j) for home, p, j in mine if home == i]
            if not partners:
                add([(1, 0, i)], [(1, t, i)], [(1, 0, t)])
                add([(1, 1, i)], [(1, t, i)], [(1, 1, t)])
                continue
            add([(1, half, i)], [(1, t, i)] + [(1, t, j) for _, j in partners],
                [(1, half, t), (-1, 1 - half, t)])
            add([(1, 0, i), (1, 1, i)], [(1, t, i)] + [(-1, p, i) for p, _ in partners],
                [(1, 1 - half, t)])

    for t in left:
        own_blocks(t, 0)
        for u, i, v, j in edges:
            if u == t:
                add([(1, 0, j), (-1, 0, i)], [(1, u, j)], [(1, 0, u), (1, 0, v)])
                add([(1, 1, i), (-1, 1, j)], [(1, v, i)], [(1, 1, v), (1, 1, u)])
                add([(1, 0, i), (1, 1, j)], [(1, u, j), (1, v, i)], [(1, 1, u), (1, 0, v)])
    for t in right:
        own_blocks(t, 1)
    return products


def _scheme(n):
    if n == 4:
        piece = [0, 0, 1, 1]
        groups = [([u], [u + 1], [(u, 0, u + 1, 2), (u, 1, u + 1, 3)]) for u in (0, 2)]
    else:
        piece = [2 * (t // 8) + ((t % 4 == t // 8) == (t % 8 >= 4)) for t in range(n)]
        groups = [(range(g, g + 4), range(g + 4, g + 8),
                   [(g + i, i, g + 4 + j, j) for i in range(4) for j in range(4) if i != j])
                  for g in range(0, n, 8)]
    helper = [n + piece[:t].count(piece[t]) for t in range(n)]
    helpers = range(n, max(helper) + 1)
    blocks = [[_FULL + p if i == p // 2 else i for i in range(_FULL)] for p in piece]
    blocks += [range(max(piece) // 2 + 1)] * len(helpers)
    shared = [p for u in helpers[::2] for p in _pair_up(
        blocks, [u], [u + 1], [(u, 0, u + 1, 1)] if len(blocks[u]) == 2 else [])]
    return _Scheme(tuple(piece), tuple(helper), tuple(shared),
                   tuple(p for group in groups for p in _pair_up(blocks, *group)))


_SIXTEEN, _EIGHT, _FOUR = _scheme(_UNIT), _scheme(8), _scheme(4)


def _numbered(scheme, n_halves):
    kept = [], []
    for n, (rows, weights, tiles) in enumerate(scheme.shared + scheme.main):
        rows = tuple(term for term in rows if term[1] < n_halves)
        tiles = tuple(term for term in tiles if term[1] < n_halves)
        if rows and tiles:
            kept[n >= len(scheme.shared)].append((n, _Product(rows, weights, tiles)))
    return kept


def _count(scheme, n_halves=2):
    return sum(map(len, _numbered(scheme, n_halves)))


def _plain(block):
    return block if block < _FULL else (block - _FULL) // 2


def _signed_sum(terms):
    (sign, total), *rest = sorted(terms, key=lambda term: -term[0])
    for s, value in rest:
        total = total + value if s == sign else total - value
    return total if sign > 0 else -total


def _accumulate(acc, key, sign, value):
    if key in acc:
        s, total = acc[key]
        if s == sign:
            acc[key] = s, total + value
        else:
            acc[key] = 1, total - value if s > 0 else value - total
    else:
        acc[key] = sign, value


def _interleave(main, count=0, others=()):
    due = sorted((count * (_LEAD + (1 - _LEAD) * (k + m / len(others)) / n), m, k)
                 for m, (_, n) in enumerate(others) for k in range(n))
    for done, _ in enumerate(main):
        while due and due[0][0] <= done:
            next(others[due.pop(0)[1]][0])
    for other, _ in others:
        for _ in other:
            pass


def _dot(a, b):
    return jax.lax.dot_general(a, b, (((1,), (0,)), ((), ())),
                               preferred_element_type=jnp.float32)


def _dot_nt(a, b):
    return jax.lax.dot_general(a, b, (((1,), (1,)), ((), ())),
                               preferred_element_type=jnp.float32)


def _pack(x):
    return pltpu.bitcast(x, jnp.uint32)


def _unpack(words):
    return pltpu.bitcast(words, jnp.bfloat16)


def _cols(n, width=1):
    return slice(n * _T, (n + width) * _T)


def _halves(low, high):
    lane = jax.lax.broadcasted_iota(jnp.int32, low.shape, 1)
    return jnp.where(lane < _T // 2, low, high)


def _layernorm(blocks):
    def mean(terms):
        total = sum(terms[:-1], 0.5 * terms[-1])
        return jnp.sum(total, axis=-1, keepdims=True) * (1 / ((_FULL + 0.5) * _T))

    center = mean(blocks)
    d = [x - center for x in blocks]
    inv = jax.lax.rsqrt(mean([x * x for x in d]) + _EPS)
    return [x * inv for x in d]


def _mixer(halves):
    @functools.cache
    def block(half, i):
        x, rest = halves[half][_plain(i)], halves[half][_FULL]
        if i < _FULL:
            return x
        return _halves(x, rest) if (i - _FULL) % 2 else _halves(rest, x)

    return functools.cache(lambda rows: _signed_sum([(s, block(half, i)) for s, half, i in rows]))


def _widen(mix, weights, scheme, n_halves):
    acc = {}
    for products in _numbered(scheme, n_halves):
        acc = {(t, half): acc[h, half] for t, h in enumerate(scheme.helper)
               for half in range(n_halves) if acc}
        for n, (rows, _, tiles) in products:
            value = _dot(mix(rows), weights[:, _cols(n)])
            for s, half, t in tiles:
                _accumulate(acc, (t, half), s, value)
            yield
    return [[_signed_sum([acc[t, half]]) for half in range(n_halves)]
            for t in range(len(scheme.piece))]


def _narrow(acc, wide, w_ref, scheme):
    n_halves, weights = len(wide[0]), _unpack(w_ref[...])
    wide = wide + [
        [_signed_sum([(1, x[half]) for x, h in zip(wide, scheme.helper) if h == helper])
         for half in range(n_halves)] for helper in range(len(wide), max(scheme.helper) + 1)]
    by_rows = {}
    for n, product in sum(_numbered(scheme, n_halves)[::-1], []):
        by_rows.setdefault(product.rows, []).append((n, product.tiles))
    for rows in sorted(by_rows, key=lambda rows: sorted({i for _, _, i in rows})[::-1])[::-1]:
        total = {}
        for n, tiles in by_rows[rows]:
            sign = max(s for s, _, _ in tiles)
            lhs = _signed_sum([(s * sign, wide[t][half]) for s, half, t in tiles])
            _accumulate(total, 0, sign, _dot(lhs, weights[:, _cols(n)]))
            yield
        for s, half, i in rows:
            _accumulate(acc, (half, i), s * total[0][0], total[0][1])


def _narrowed(acc, half):
    blocks = [_signed_sum([acc[half, i]]) for i in range(2 * _FULL)]
    folded = list(zip(blocks[_FULL::2], blocks[_FULL + 1::2]))
    rest = _signed_sum([(1, _halves(low, high)) for low, high in folded])
    rest += jnp.concatenate([rest[:, _T // 2:], rest[:, :_T // 2]], axis=1)
    return ([x + _halves(high, low) for x, (low, high) in zip(blocks, folded)]
            + blocks[len(folded):_FULL] + [rest])


def _combine(part, w_ref, scheme, transposed=False):
    donor = {(h, p): t for t, (h, p) in enumerate(zip(scheme.helper, scheme.piece))}
    products = scheme.shared + scheme.main
    uses = {}
    for single in (True, False):
        for n, product in enumerate(products):
            if single == (len(product.weights) == 1):
                for s, t, i in product.weights:
                    uses.setdefault((t, i), []).append((s, n))

    def folded(t, p):
        if t >= len(scheme.piece):
            return part(donor[t, p], p)
        if p == scheme.piece[t]:
            return part(t, 2 * _FULL)
        if (scheme.helper[t], p) in donor:
            return (part(t, p).astype(jnp.float32)
                    - folded(scheme.helper[t], p).astype(jnp.float32))
        return part(t, p)

    tokens = []
    for side in range(2):
        acc, missing, stored = {}, [len(product.weights) for product in products], []
        for t, i in sorted(uses, key=lambda source: uses[source][0][1]):
            w = folded(t, 2 * _plain(i) + side)
            exact = w.astype(jnp.float32)
            for s, n in uses[t, i]:
                _accumulate(acc, n, s, exact if len(products[n].weights) > 1 else w)
                missing[n] -= 1
                if not missing[n]:
                    at = pl.ds(side * _T // 4, _T // 4), _cols(n)
                    w_ref[at] = _pack(_signed_sum([acc.pop(n)]).astype(jnp.bfloat16))
                    stored.append(w_ref[at])
        stored = [functools.reduce(jnp.bitwise_or, stored[n:n + 4])
                  for n in range(0, len(stored), 4)]
        tokens += [words[r:r + 8] for r in range(0, _T // 4, 8) for words in stored]
    for n in range(len(products) if transposed else 0):
        w_ref[:, _cols(n)] = words = _pack(_unpack(w_ref[:, _cols(n)]).T)
        tokens += [words[:8], words[-8:]]
    return tokens


def _kernel(xt_hbm, mem0_hbm, wq_hbm, wk_hbm, wv_hbm, wot_hbm, w1_hbm, w3_hbm, w2t_hbm,
            outt_hbm, mem0_ref, tile_ref, res_ref, mem_ref, norm_ref, early_norm_ref, early_refs,
            qkv_refs, gate_ref, gate8_ref, out_ref, down4_ref,
            qkv_stage, gate_stage, out_stage, qkv_sem, gate_sem, out_sem, tile_sem, mem_sem,
            *, seg):
    d_model, n_tok = xt_hbm.shape
    n_mem = mem0_ref.shape[0]
    d_head = wq_hbm.shape[2]
    n_seg = n_tok // seg
    n_io = n_tok // _T
    n_qkv, n_gate, n_out = len(qkv_refs), len(gate_ref), len(out_ref)
    n_wo = n_qkv // 3
    span = n_mem + seg
    score_scale = d_head ** -0.5 * _LOG2E

    def blocks_at(ref, *index):
        return [ref[(*index, _cols(i))] for i in range(_FULL + 1)]

    def set_blocks(ref, index, blocks):
        for i, x in enumerate(blocks):
            ref[(*index, _cols(i))] = x

    def rows_of(s):
        return pl.ds(pl.multiple_of(s * seg, seg), seg)

    def step(order, attend=(), feed=(), partner=None, finished=None):
        n_layers = len(attend)
        qkv, probs, heads, hidden, mixed, fed = [[], [], []], [], [], [], {}, {}
        if attend:
            i, j = (jax.lax.broadcasted_iota(jnp.int32, (n_layers * span, _T), a) for a in (0, 1))
            same = ((i >= span) == (j >= span)) & (j < 2 * span)
            visible = same & ((i < n_mem) | ((i >= span) & (i < span + n_mem)) | (i >= j))
            fill = jnp.where(same, _MASKED * _LOG2E, -jnp.inf).astype(jnp.float32)
            mem = [blocks_at(mem_ref, n, slice(None)) for n in range(n_layers)]
            h = _layernorm(blocks_at(res_ref, rows_of(attend[0])))
            if n_layers == 1:
                attend_mix = _mixer([[jnp.concatenate(parts, axis=0) for parts in zip(mem[0], h)]])
            elif _FORTY:
                attend_mix = _mixer([
                    [jnp.concatenate(parts, axis=0) for parts in zip(m, x)]
                    for m, x in zip(mem, (h, _layernorm(blocks_at(res_ref, rows_of(attend[1])))))])
            else:
                ahead = _layernorm(
                    [x[:seg - _EARLY] for x in blocks_at(res_ref, rows_of(attend[1]))])
                cut = seg - _EARLY // 2
                attend_mix = _mixer([
                    [jnp.concatenate([m, a[:cut]], axis=0) for m, a in zip(mem[0], h)],
                    [jnp.concatenate([m, a[cut:], b], axis=0) for m, a, b in zip(mem[1], h, ahead)]])
        if feed:
            feed_mix = _mixer([blocks_at(norm_ref, n, slice(None)) for n in range(2)])

        def project(which, g):
            tiles = yield from _widen(
                attend_mix, _unpack(qkv_refs[3 * g + which][...]), _SIXTEEN, n_layers)
            if n_layers == 1 or _FORTY:
                tiles = [jnp.concatenate(halves, axis=0) for halves in tiles]
            else:
                moved = n_mem + _EARLY // 2
                known = pl.ds(pl.multiple_of(attend[0] * (_EARLY // 2), _EARLY // 2), _EARLY // 2)
                early = _unpack(early_refs[3 * g + which][known, :]).astype(jnp.float32)
                tiles = [jnp.concatenate(
                    [a, b[n_mem:moved], b[:n_mem], b[moved:], early[:, _cols(t)]], axis=0)
                         for t, (a, b) in enumerate(tiles)]
            qkv[which] += [x.astype(jnp.bfloat16) if _PACK[which] and n_layers == 2 else x for x in tiles]

        def score(count):
            for t in range(len(probs), len(probs) + count):
                s = _dot_nt(qkv[0][t], qkv[1][t])
                s = jnp.concatenate([s, jnp.zeros((s.shape[0], _T - s.shape[1]), s.dtype)], axis=1)
                s = jnp.where(visible, s * score_scale, fill)
                p = jnp.exp2(s - jnp.max(s, axis=-1, keepdims=True))
                probs.append(
                    (p, pltpu.reciprocal(jnp.sum(p, axis=-1, keepdims=True), approx=True)))
                yield

        def average(count):
            for t in range(len(heads), len(heads) + count):
                (p, inv), v = probs[t], qkv[2][t]
                both = _dot(p[:, :v.shape[0]], v) * inv
                heads.append([both[n * span:(n + 1) * span] for n in range(n_layers)])
                yield

        def hand_over():
            x = [] if partner is None else [blocks_at(res_ref, rows_of(partner))]
            for n, s in enumerate(attend):
                out = _narrowed(mixed, n)
                x.append([a + o[n_mem:] for a, o in zip(blocks_at(res_ref, rows_of(s)), out)])
                set_blocks(res_ref, [rows_of(s)], x[-1])
                set_blocks(mem_ref, [n, slice(None)], [o[:n_mem] for o in out])
            for n, blocks in enumerate(x):
                set_blocks(norm_ref, [n, slice(None)], _layernorm(blocks))
                yield

        def gated(w_ref, scheme):
            tiles = yield from _widen(feed_mix, _unpack(w_ref[...]), scheme, 2)
            for pair in zip(tiles[::2], tiles[1::2]):
                halved = [(0.5 * gate, up) for gate, up in zip(*pair)]
                hidden.append([(g * jnp.tanh(g) + g) * up for g, up in halved])

        def begin(name):
            stage, g = name[0], int(name[1:])
            tiles = slice(g * _UNIT, (g + 1) * _UNIT)
            if stage in "QKV":
                return project("QKV".index(stage), g), _count(_SIXTEEN, n_layers)
            if stage in "SA":
                return (score if stage == "S" else average)(g), g
            if stage == "N":
                return hand_over(), 2
            if stage == "T":
                return transpose_out(finished), _FULL + 1
            if stage == "O":
                return (_narrow(mixed, heads[tiles], out_ref[g], _SIXTEEN),
                        _count(_SIXTEEN, n_layers))
            if stage == "G":
                unit = (gate_ref[g], _SIXTEEN) if g < n_gate else (gate8_ref, _EIGHT)
                return gated(*unit), _count(unit[1])
            unit = (out_ref[n_wo + g], _SIXTEEN) if n_wo + g < n_out else (down4_ref, _FOUR)
            return _narrow(fed, hidden[tiles], *unit), _count(unit[1])

        for names in order.split():
            main, *others = [begin(name) for name in names.split("+")]
            _interleave(*main, others)
        for n, s in enumerate(feed):
            set_blocks(res_ref, [rows_of(s)], [
                a + o for a, o in zip(blocks_at(res_ref, rows_of(s)), _narrowed(fed, n))])

    def when(condition, act, copies):
        @pl.when(condition)
        def _():
            for c in copies():
                act(c)

    def start(copy):
        copy.start()

    def wait(copy):
        copy.wait()

    def column_copy(w_hbm, first, count, stage, sem, offset=0):
        cols = pl.ds(pl.multiple_of(first * _T, _T), count * _T)
        return pltpu.make_async_copy(w_hbm.bitcast(jnp.uint32).at[:, cols],
                                     stage.at[:, _cols(offset, count)], sem)

    def move_qkv(act, n):
        for which, w in enumerate((wq_hbm, wk_hbm, wv_hbm)):
            when((n < n_qkv) & (n % 3 == which), act, lambda w=w: [
                pltpu.make_async_copy(w.bitcast(jnp.uint32).at[:, n // 3 * (_UNIT // 2) + p, :],
                                      qkv_stage.at[n % 2, p], qkv_sem.at[n % 2])
                for p in range(_UNIT // 2)])

    def move_others(act, n):
        gate, out = (gate_stage.at[n % 2], gate_sem.at[n % 2]), (out_stage.at[n % 2], out_sem.at[n % 2])
        for active, count in ((n < n_gate, _UNIT // 2), (n == n_gate, 4)):
            when(active, act, lambda count=count: [
                column_copy(w, n * (_UNIT // 2), count, *gate, side * (_UNIT // 2))
                for side, w in enumerate((w1_hbm, w3_hbm))])
        when(n < n_wo, act, lambda: [
            pltpu.make_async_copy(wot_hbm.bitcast(jnp.uint32).at[n * _UNIT + t],
                                  out[0].at[:, _cols(t)], out[1]) for t in range(_UNIT)])
        for active, count in (((n >= n_wo) & (n < n_out), _UNIT), (n == n_out, 4)):
            when(active, act,
                 lambda count=count: [column_copy(w2t_hbm, (n - n_wo) * _UNIT, count, *out)])

    def combine_qkv(n):
        def part(t, p):
            words = qkv_stage[n % 2, t // 2, pl.ds(p * _T // 2, _T // 2), :]
            words = words & jnp.uint32(0xFFFF0000) if t % 2 else words << 16
            return pltpu.bitcast(words, jnp.float32)

        return _combine(part, qkv_refs[n], _SIXTEEN)

    def combine_others(n, gate, out):
        def part(stage, column, t, p):
            return _unpack(stage[n % 2, pl.ds(p * _T // 4, _T // 4), _cols(column(t))])

        return (_combine(functools.partial(part, out_stage, lambda t: t), *out, True) + _combine(
            functools.partial(part, gate_stage, lambda t: t % 2 * (_UNIT // 2) + t // 2), *gate))

    def project_early(n, tokens):
        n_products = len(_EARLY_ROWS) * _count(_SIXTEEN)
        due = {n_products * (k + 2) // (len(tokens) + 2): token for k, token in enumerate(tokens)}
        done = itertools.count()
        weights = _unpack(qkv_refs[n][...])
        for first, count in zip(itertools.accumulate((0,) + _EARLY_ROWS), _EARLY_ROWS):
            mix = _mixer([blocks_at(early_norm_ref, half, pl.ds(first, count)) for half in (0, 1)])

            def paced(key, mix=mix):
                x, token = mix(key), due.get(next(done))
                if token is None:
                    return x
                return jnp.concatenate(
                    [x[:-8], jnp.where(loaded, x[-8:], pltpu.bitcast(token, jnp.float32))], axis=0)

            tiles = yield from _widen(paced, weights, _SIXTEEN, 2)
            for t, (a, b) in enumerate(tiles):
                for r in range(0, a.shape[0], _EARLY):
                    for half, x in enumerate((a, b)):
                        words = pl.ds(first + r + half * _EARLY // 2, _EARLY // 2)
                        early_refs[n][words, _cols(t)] = _pack(
                            x[r:r + _EARLY].astype(jnp.bfloat16))

    def x_copy(i):
        cols = pl.ds(pl.multiple_of(i * _T, _T), _T)
        return pltpu.make_async_copy(xt_hbm.at[:, cols], tile_ref.at[i], tile_sem.at[i])

    def out_copy(i):
        return pltpu.make_async_copy(tile_ref.at[i], outt_hbm.at[:, _cols(i)], tile_sem.at[i])

    def transpose_out(i):
        for b, x in enumerate(blocks_at(res_ref, pl.ds(pl.multiple_of(i * _T, _T), _T))):
            depth = min(_T, d_model - b * _T)
            tile_ref[i, pl.ds(b * _T, depth), :] = x.T[:depth].astype(tile_ref.dtype)
            yield

    def double_step(b):
        step(_ORDER, attend=[b, b + _LAG], feed=[b - 1, b + _LAG - 1],
             finished=jnp.maximum(b - 5, 0) * seg // _T)

    if _DEV == "main":
        pl.loop(1, n_seg - _LAG)(double_step)
        out_copy(0).start()
        out_copy(0).wait()
        return

    mem_copy = pltpu.make_async_copy(mem0_hbm, mem0_ref, mem_sem)
    for i in range(n_io):
        x_copy(i).start()
    mem_copy.start()
    move_qkv(start, 0)

    def load_tile(i, _):
        x_copy(i).wait()
        x = tile_ref[i].astype(jnp.float32)
        x = jnp.concatenate([x, x[_FULL * _T:]], axis=0)
        blocks = [x[b * _T:(b + 1) * _T].T for b in range(_FULL + 1)]
        set_blocks(res_ref, [pl.ds(pl.multiple_of(i * _T, _T), _T)], blocks)
        normed = _layernorm([
            jnp.concatenate([x[s - _EARLY:s] for s in range(seg, _T + 1, seg)], axis=0)
            for x in blocks])
        for s in range(_T // seg):
            at = jnp.maximum(i * (_T // seg) + s - _LAG, 0) // 2 * _EARLY
            set_blocks(early_norm_ref, [s % 2, pl.ds(pl.multiple_of(at, _EARLY), _EARLY)],
                       [x[s * _EARLY:(s + 1) * _EARLY] for x in normed])

        return i

    loaded = jax.lax.fori_loop(0, n_io, load_tile, 0) > 0
    move_qkv(start, 1)
    move_qkv(wait, 0)
    combine_qkv(0)
    for n in range(n_qkv if _DEV != "pro" else 2):
        move_qkv(start, n + 2)
        move_others(start, n)
        move_qkv(wait, n + 1)
        tokens = []
        if n > 0:
            move_others(wait, n - 1)
            tokens += combine_others(n - 1, *(
                ((gate_ref[n - 1], _SIXTEEN), (out_ref[n - 1], _SIXTEEN)) if n <= n_gate
                else ((gate8_ref, _EIGHT), (down4_ref, _FOUR))))
        if n + 1 < n_qkv:
            tokens += combine_qkv(n + 1)
        _interleave(project_early(n, tokens))
    if _DEV == "pro":
        @pl.loop(0, 2)
        def _(i):
            tile_ref[0, :128] = _unpack(sum(r[:64, pl.ds(pl.multiple_of(i * 128, 128), 128)] for r in (gate_ref[0], out_ref[0], *qkv_refs[:3], *early_refs[:2])))
        out_copy(0).start()
        out_copy(0).wait()
        return

    mem_copy.wait()
    mem0 = mem0_ref[...].astype(jnp.float32)
    mem_ref[0] = mem0 = jnp.concatenate([mem0, mem0[:, _FULL * _T:]], axis=1)
    pl.loop(0, _LAG)(lambda s: step(_ORDER_ATTENTION, attend=[s], partner=0))
    step(_ORDER_FFN, feed=[0, 1])
    mem_ref[1] = mem_ref[0]
    mem_ref[0] = mem0
    step(_ORDER_ATTENTION, attend=[0, _LAG])
    pl.loop(1, n_seg - _LAG)(double_step)
    for i in range(n_io - 1):
        out_copy(i).start()
    step(_ORDER_FFN, feed=[n_seg - _LAG - 1, n_seg - 1])
    pl.loop(n_seg - _LAG, n_seg)(
        lambda s: step(_ORDER_ATTENTION, attend=[s], partner=n_seg - 2))
    step(_ORDER_FFN, feed=[n_seg - 2, n_seg - 1])
    _interleave(transpose_out(n_io - 1))
    out_copy(n_io - 1).start()
    for i in range(n_io):
        out_copy(i).wait()


@functools.partial(jax.jit, static_argnames=("A_seg_len",))
def pallas_interleave_layers__memory_aug_recurrent_mem_tr__glu_gated_swiglu__prompt_kernel(
    A_x: jax.Array,
    A_mem0: jax.Array,
    A_Wq: jax.Array,
    A_Wk: jax.Array,
    A_Wv: jax.Array,
    A_Wo: jax.Array,
    A_seg_len: int,
    B_x: jax.Array,
    B_w1: jax.Array,
    B_w3: jax.Array,
    B_w2: jax.Array,
):
    del B_x
    _, n_tok, d_model = A_x.shape
    n_mem = A_mem0.shape[1]
    _, n_heads, d_head = A_Wq.shape
    d_ff = B_w1.shape[1]
    assert A_x.shape[0] == 1 and 4 * A_seg_len == _T and n_mem == 8
    assert (d_model, n_heads, d_head, d_ff) == (576, 2 * _UNIT, _T, 36 * _T)
    early_rows = (n_tok // A_seg_len - _LAG) * _EARLY
    width = (_FULL + 1) * _T
    hbm = pl.BlockSpec(memory_space=pltpu.HBM)

    def weights(scheme, *units):
        return pltpu.VMEM((*units, _T // 2, _count(scheme) * _T), jnp.uint32)

    out_t = pl.pallas_call(
        functools.partial(_kernel, seg=A_seg_len),
        out_shape=jax.ShapeDtypeStruct((d_model, n_tok), A_x.dtype),
        in_specs=[hbm] * 9,
        out_specs=hbm,
        scratch_shapes=[
            pltpu.VMEM((n_mem, d_model), A_mem0.dtype),
            pltpu.VMEM((n_tok // _T, d_model, _T), A_x.dtype),
            pltpu.VMEM((n_tok, width), jnp.float32),
            pltpu.VMEM((2, n_mem, width), jnp.float32),
            pltpu.VMEM((2, A_seg_len, width), jnp.float32),
            pltpu.VMEM((2, early_rows // 2, width), jnp.float32),
            [pltpu.VMEM((early_rows // 2, _UNIT * _T), jnp.uint32)] * 6,
            [weights(_SIXTEEN)] * 6, [weights(_SIXTEEN)] * 4, weights(_EIGHT),
            [weights(_SIXTEEN)] * 4, weights(_FOUR),
            pltpu.VMEM((2, _UNIT // 2, d_model, _T), jnp.uint32),
            pltpu.VMEM((2, d_model // 2, _UNIT * _T), jnp.uint32),
            pltpu.VMEM((2, d_model // 2, _UNIT * _T), jnp.uint32),
            pltpu.SemaphoreType.DMA((2,)),
            pltpu.SemaphoreType.DMA((2,)),
            pltpu.SemaphoreType.DMA((2,)),
            pltpu.SemaphoreType.DMA((n_tok // _T,)),
            pltpu.SemaphoreType.DMA,
        ],
        compiler_params=pltpu.CompilerParams(vmem_limit_bytes=120 * 1024 * 1024, flags=_FLAGS,
                                             disable_bounds_checks=True),
    )(A_x.reshape(n_tok, d_model).T, A_mem0.reshape(n_mem, d_model), A_Wq, A_Wk, A_Wv,
      A_Wo.transpose(0, 2, 1), B_w1, B_w3, B_w2.T)
    return out_t.T.reshape(A_x.shape)
```

```python
import functools
import itertools
import math
from typing import NamedTuple

import jax
import jax.numpy as jnp
import jax.experimental.pallas as pl
import jax.experimental.pallas.tpu as pltpu

_EPS = 1e-05
_MASKED = -1000000000.0
_LOG2E = math.log2(math.e)
_T = 128
_FULL = 4
_UNIT = 16
_LAG = 2
_EARLY = 16
_EARLY_ROWS = (48,) * 9 + (32,) * 2
_FIRST_TILES, _FIRST_PASSES = 5, 2
_ARRIVALS = {0: "Q0", 7: "K0", 11: "V0", 17: "Q1 O0", 27: "K1 O1 V1", 42: "D0 D1 D2 G0",
             59: "G1 G2 G3 G4"}
_DEPARTURES = {0: "K0", 2: "V0", 7: "Q1 O0", 11: "K1", 17: "O1 V1 D0", 27: "D1 D2 G0 G1",
               42: "G2 G3 G4"}
_ORDER = "G0 K0 Q0 K1+S6 Q1+S6 V0+S6+T0 G1+S7+A6 V1+S7+A10 O0+A12 G2+A4 O1 G3+N0 G4 D0 D1 D2 F0"
_ORDER_TAIL = "G0 G1 G2 G3 G4 Q0 K0 Q1+S8 K1+S8 V0+S8 V1+S8+A16 D0 D1 D2 F0 O0+A16 O1 N0"
_ORDER_LAST = "Q0 K0 Q1+S8 K1+S8 V0+S16 V1+A16 O0+A16 O1 N0"
_ORDER_FIRST = "Q0 K0 Q1+S8 K1+S8 V0+S16 V1+A16 O0+A16 O1 X0+N0"
_ORDER_BOTH = "Q0 K0 Q1+S8 K1+S8 V0+S16 V1+A16 O0+A16 O1 X0+N0"
_ORDER_FFN = "G0 G1 G2 G3 G4 D0 D1 D2 F0"
_LEAD = 0.1
_DEV = ""
_CS = 1
_BW = False
_BP = False
_CA = 1
_PACK = (True, True, True)
_FLAGS = None


class _Product(NamedTuple):
    rows: tuple
    weights: tuple
    tiles: tuple


class _Scheme(NamedTuple):
    piece: tuple
    helper: tuple
    shared: tuple
    main: tuple


def _pair_up(blocks, left, right, edges):
    products = []
    edges = [(u, blocks[u][i], v, blocks[v][j]) for u, i, v, j in edges]
    assert all(i in blocks[v] and j in blocks[u] for u, i, v, j in edges)

    def add(rows, weights, tiles):
        rows = tuple(sorted(rows, key=lambda term: term[1:]))
        if rows[0][0] < 0:
            rows = tuple((-s, half, i) for s, half, i in rows)
            tiles = tuple((-s, half, t) for s, half, t in tiles)
        products.append(_Product(rows, tuple(weights), tuple(tiles)))

    def own_blocks(t, half):
        mine = [((i, v, j), (j, u, i))[half] for u, i, v, j in edges if (u, v)[half] == t]
        for i in blocks[t]:
            if any(i == j for _, _, j in mine):
                continue
            partners = [(p, j) for home, p, j in mine if home == i]
            if not partners:
                add([(1, 0, i)], [(1, t, i)], [(1, 0, t)])
                add([(1, 1, i)], [(1, t, i)], [(1, 1, t)])
                continue
            add([(1, half, i)], [(1, t, i)] + [(1, t, j) for _, j in partners],
                [(1, half, t), (-1, 1 - half, t)])
            add([(1, 0, i), (1, 1, i)], [(1, t, i)] + [(-1, p, i) for p, _ in partners],
                [(1, 1 - half, t)])

    for t in left:
        own_blocks(t, 0)
        for u, i, v, j in edges:
            if u == t:
                add([(1, 0, j), (-1, 0, i)], [(1, u, j)], [(1, 0, u), (1, 0, v)])
                add([(1, 1, i), (-1, 1, j)], [(1, v, i)], [(1, 1, v), (1, 1, u)])
                add([(1, 0, i), (1, 1, j)], [(1, u, j), (1, v, i)], [(1, 1, u), (1, 0, v)])
    for t in right:
        own_blocks(t, 1)
    return products


def _scheme(n):
    if n == 4:
        piece = [0, 0, 1, 1]
        groups = [([u], [u + 1], [(u, 0, u + 1, 2), (u, 1, u + 1, 3)]) for u in (0, 2)]
    else:
        piece = [2 * (t // 8) + ((t % 4 == t // 8) == (t % 8 >= 4)) for t in range(n)]
        groups = [(range(g, g + 4), range(g + 4, g + 8),
                   [(g + i, i, g + 4 + j, j) for i in range(4) for j in range(4) if i != j])
                  for g in range(0, n, 8)]
    helper = [n + piece[:t].count(piece[t]) for t in range(n)]
    helpers = range(n, max(helper) + 1)
    blocks = [[_FULL + p if i == p // 2 else i for i in range(_FULL)] for p in piece]
    blocks += [range(max(piece) // 2 + 1)] * len(helpers)
    shared = [p for u in helpers[::2] for p in _pair_up(
        blocks, [u], [u + 1], [(u, 0, u + 1, 1)] if len(blocks[u]) == 2 else [])]
    return _Scheme(tuple(piece), tuple(helper), tuple(shared),
                   tuple(p for group in groups for p in _pair_up(blocks, *group)))


_SIXTEEN, _EIGHT, _FOUR = _scheme(_UNIT), _scheme(8), _scheme(4)


def _numbered(scheme, n_halves):
    kept = [], []
    for n, (rows, weights, tiles) in enumerate(scheme.shared + scheme.main):
        rows = tuple(term for term in rows if term[1] < n_halves)
        tiles = tuple(term for term in tiles if term[1] < n_halves)
        if rows and tiles:
            kept[n >= len(scheme.shared)].append((n, _Product(rows, weights, tiles)))
    return kept


def _count(scheme, n_halves=2):
    return sum(map(len, _numbered(scheme, n_halves)))


def _plain(block):
    return block if block < _FULL else (block - _FULL) // 2


def _signed_sum(terms):
    (sign, total), *rest = sorted(terms, key=lambda term: -term[0])
    for s, value in rest:
        total = total + value if s == sign else total - value
    return total if sign > 0 else -total


def _accumulate(acc, key, sign, value):
    if key in acc:
        s, total = acc[key]
        if s == sign:
            acc[key] = s, total + value
        else:
            acc[key] = 1, total - value if s > 0 else value - total
    else:
        acc[key] = sign, value


def _interleave(main, count=0, others=()):
    due = sorted((count * (_LEAD + (1 - _LEAD) * (k + m / len(others)) / n), m, k)
                 for m, (_, n) in enumerate(others) for k in range(n))
    for done, _ in enumerate(main):
        while due and due[0][0] <= done:
            next(others[due.pop(0)[1]][0])
    for other, _ in others:
        for _ in other:
            pass


def _dot(a, b):
    return jax.lax.dot_general(a, b, (((1,), (0,)), ((), ())),
                               preferred_element_type=jnp.float32)


def _dot_nt(a, b):
    return jax.lax.dot_general(a, b, (((1,), (1,)), ((), ())),
                               preferred_element_type=jnp.float32)


def _pack(x):
    return pltpu.bitcast(x, jnp.uint32)


def _unpack(words):
    return pltpu.bitcast(words, jnp.bfloat16)


def _cols(n, width=1):
    return slice(n * _T, (n + width) * _T)


def _operand(x, on=True):
    return x.astype(jnp.bfloat16) if on and x.shape[0] % 16 == 0 else x


def _halves(low, high):
    lane = jax.lax.broadcasted_iota(jnp.int32, low.shape, 1)
    return jnp.where(lane < _T // 2, low, high)


def _layernorm(blocks):
    def mean(terms):
        total = sum(terms[:-1], 0.5 * terms[-1])
        return jnp.sum(total, axis=-1, keepdims=True) * (1 / ((_FULL + 0.5) * _T))

    center = mean(blocks)
    d = [x - center for x in blocks]
    inv = jax.lax.rsqrt(mean([x * x for x in d]) + _EPS)
    return [x * inv for x in d]


def _mixer(halves, packed=True):
    @functools.cache
    def block(half, i):
        x, rest = halves[half][_plain(i)], halves[half][_FULL]
        if i < _FULL:
            return x
        return _halves(x, rest) if (i - _FULL) % 2 else _halves(rest, x)

    return functools.cache(
        lambda rows: _operand(_signed_sum([(s, block(half, i)) for s, half, i in rows]), _BW and packed))


def _widen(mix, w_ref, scheme, n_halves, paced):
    acc, weights = {}, _unpack(w_ref[...])
    for products in _numbered(scheme, n_halves):
        acc = {(t, half): acc[h, half] for t, h in enumerate(scheme.helper)
               for half in range(n_halves) if acc}
        for n, (rows, _, tiles) in products:
            value = _dot(paced(mix(rows)), weights[:, _cols(n)])
            for s, half, t in tiles:
                _accumulate(acc, (t, half), s, value)
            yield
    return [[_signed_sum([acc[t, half]]) for half in range(n_halves)]
            for t in range(len(scheme.piece))]


def _narrow(acc, wide, w_ref, scheme, paced):
    n_halves, weights = len(wide[0]), _unpack(w_ref[...])
    wide = wide + [
        [_signed_sum([(1, x[half]) for x, h in zip(wide, scheme.helper) if h == helper])
         for half in range(n_halves)] for helper in range(len(wide), max(scheme.helper) + 1)]
    by_rows = {}
    for n, product in sum(_numbered(scheme, n_halves)[::-1], []):
        by_rows.setdefault(product.rows, []).append((n, product.tiles))
    for rows in sorted(by_rows, key=lambda rows: sorted({i for _, _, i in rows})[::-1])[::-1]:
        total = {}
        for n, tiles in by_rows[rows]:
            sign = max(s for s, _, _ in tiles)
            lhs = _signed_sum([(s * sign, wide[t][half]) for s, half, t in tiles])
            _accumulate(total, 0, sign, _dot(paced(lhs), weights[:, _cols(n)]))
            yield
        for s, half, i in rows:
            _accumulate(acc, (half, i), s * total[0][0], total[0][1])


def _narrowed(acc, half):
    blocks = [_signed_sum([acc[half, i]]) for i in range(2 * _FULL)]
    folded = list(zip(blocks[_FULL::2], blocks[_FULL + 1::2]))
    rest = _signed_sum([(1, _halves(low, high)) for low, high in folded])
    rest += jnp.concatenate([rest[:, _T // 2:], rest[:, :_T // 2]], axis=1)
    return ([x + _halves(high, low) for x, (low, high) in zip(blocks, folded)]
            + blocks[len(folded):_FULL] + [rest])


def _combine(part, w_ref, scheme, transposed=False):
    donor = {(h, p): t for t, (h, p) in enumerate(zip(scheme.helper, scheme.piece))}
    products = scheme.shared + scheme.main
    uses = {}
    for single in (True, False):
        for n, product in enumerate(products):
            if single == (len(product.weights) == 1):
                for s, t, i in product.weights:
                    uses.setdefault((t, i), []).append((s, n))

    def folded(t, p):
        if t >= len(scheme.piece):
            return part(donor[t, p], p)
        if p == scheme.piece[t]:
            return part(t, 2 * _FULL)
        if (scheme.helper[t], p) in donor:
            return (part(t, p).astype(jnp.float32)
                    - folded(scheme.helper[t], p).astype(jnp.float32))
        return part(t, p)

    tokens = []
    for side in range(2):
        acc, missing, stored = {}, [len(product.weights) for product in products], []
        for t, i in sorted(uses, key=lambda source: uses[source][0][1]):
            w = folded(t, 2 * _plain(i) + side)
            exact = w.astype(jnp.float32)
            for s, n in uses[t, i]:
                _accumulate(acc, n, s, exact if len(products[n].weights) > 1 else w)
                missing[n] -= 1
                if not missing[n]:
                    at = pl.ds(side * _T // 4, _T // 4), _cols(n)
                    w_ref[at] = _pack(_signed_sum([acc.pop(n)]).astype(jnp.bfloat16))
                    stored.append(w_ref[at])
        stored = [functools.reduce(jnp.bitwise_or, stored[n:n + 4])
                  for n in range(0, len(stored), 4)]
        tokens += [words[r:r + 8] for r in range(0, _T // 4, 8) for words in stored]
    for n in range(len(products) if transposed else 0):
        w_ref[:, _cols(n)] = words = _pack(_unpack(w_ref[:, _cols(n)]).T)
        tokens.append(words[-8:])
    return tokens


def _kernel(xt_hbm, mem0_hbm, wq_hbm, wk_hbm, wv_hbm, wot_hbm, w1_hbm, w3_hbm, w2t_hbm,
            outt_hbm, mem0_ref, tile_ref, res_ref, mem_ref, norm_ref, early_norm_ref, early_refs,
            qkv_refs, wo_refs, gate_refs, down_refs,
            head_stages, column_stages, weight_sem, tile_sem, mem_sem,
            *, seg):
    d_model, n_tok = xt_hbm.shape
    n_mem = mem0_ref.shape[0]
    d_head = wq_hbm.shape[2]
    n_seg = n_tok // seg
    n_io = n_tok // _T
    span = n_mem + seg
    score_scale = d_head ** -0.5 * _LOG2E

    def blocks_at(ref, *index):
        return [ref[(*index, _cols(i))] for i in range(_FULL + 1)]

    def set_blocks(ref, index, blocks):
        for i, x in enumerate(blocks):
            ref[(*index, _cols(i))] = x

    def rows_of(s):
        return pl.ds(pl.multiple_of(s * seg, seg), seg)

    def unit(name):
        stage, g = name[0], int(name[1:])
        if stage in "QKV":
            return qkv_refs[3 * g + "QKV".index(stage)], _SIXTEEN
        return ({"O": wo_refs, "G": gate_refs, "D": down_refs}[stage][g],
                {"G4": _EIGHT, "D2": _FOUR}.get(name, _SIXTEEN))

    def step(order, attend=(), feed=(), partner=None, finished=None):
        n_layers = len(attend)
        qkv, probs, heads, hidden, mixed, fed = [[], [], []], [], [], [], {}, {}
        if attend:
            i, j = (jax.lax.broadcasted_iota(jnp.int32, (n_layers * span, _T), a) for a in (0, 1))
            same = ((i >= span) == (j >= span)) & (j < 2 * span)
            visible = same & ((i < n_mem) | ((i >= span) & (i < span + n_mem)) | (i >= j))
            fill = jnp.where(same, _MASKED * _LOG2E, -jnp.inf).astype(jnp.float32)
            mem = [blocks_at(mem_ref, n, slice(None)) for n in range(n_layers)]
            h = _layernorm(blocks_at(res_ref, rows_of(attend[0])))
            if n_layers == 1:
                attend_mix = _mixer([[jnp.concatenate(parts, axis=0) for parts in zip(mem[0], h)]])
            else:
                ahead = _layernorm(
                    [x[:seg - _EARLY] for x in blocks_at(res_ref, rows_of(attend[1]))])
                cut = seg - _EARLY // 2
                attend_mix = _mixer([
                    [jnp.concatenate([m, a[:cut]], axis=0) for m, a in zip(mem[0], h)],
                    [jnp.concatenate([m, a[cut:], b], axis=0) for m, a, b in zip(mem[1], h, ahead)]])
        if feed:
            feed_mix = _mixer([blocks_at(norm_ref, n, slice(None)) for n in range(2)])

        def project(which, g):
            tiles = yield from _widen(
                attend_mix, qkv_refs[3 * g + which], _SIXTEEN, n_layers, paced)
            if n_layers == 1:
                tiles = [jnp.concatenate(halves, axis=0) for halves in tiles]
            else:
                moved = n_mem + _EARLY // 2
                known = pl.ds(pl.multiple_of(attend[0] * (_EARLY // 2), _EARLY // 2), _EARLY // 2)
                early = _unpack(early_refs[3 * g + which][known, :]).astype(jnp.float32)
                tiles = [jnp.concatenate(
                    [a, b[n_mem:moved], b[:n_mem], b[moved:], early[:, _cols(t)]], axis=0)
                         for t, (a, b) in enumerate(tiles)]
            qkv[which] += [x.astype(jnp.bfloat16) if _PACK[which] and n_layers == 2 else x for x in tiles]

        def score(count):
            for t in range(len(probs), len(probs) + count * _CS):
                s = _dot_nt(qkv[0][t], qkv[1][t])
                s = jnp.concatenate([s, jnp.zeros((s.shape[0], _T - s.shape[1]), s.dtype)], axis=1)
                s = jnp.where(visible, s * score_scale, fill)
                p = jnp.exp2(s - jnp.max(s, axis=-1, keepdims=True))
                probs.append(
                    (_operand(p[:, :n_layers * span], _BP), pltpu.reciprocal(jnp.sum(p, axis=-1, keepdims=True), approx=True)))
                if len(probs) % _CS == 0:
                    yield

        def average(count):
            for t in range(len(heads), len(heads) + count * _CA):
                (p, inv), v = probs[t], qkv[2][t]
                both = _dot(p, v) * inv
                heads.append([both[n * span:(n + 1) * span] for n in range(n_layers)])
                if len(heads) % _CA == 0:
                    yield

        def hand_over():
            x = [] if partner is None else [blocks_at(res_ref, rows_of(partner))]
            for n, s in enumerate(attend):
                out = _narrowed(mixed, n)
                x.append([a + o[n_mem:] for a, o in zip(blocks_at(res_ref, rows_of(s)), out)])
                set_blocks(res_ref, [rows_of(s)], x[-1])
                set_blocks(mem_ref, [n, slice(None)], [o[:n_mem] for o in out])
            for n, blocks in enumerate(x):
                set_blocks(norm_ref, [n, slice(None)], _layernorm(blocks))
                yield

        def gated(w_ref, scheme):
            tiles = yield from _widen(feed_mix, w_ref, scheme, 2, paced)
            for pair in zip(tiles[::2], tiles[1::2]):
                halved = [(0.5 * gate, up) for gate, up in zip(*pair)]
                hidden.append([(g * jnp.tanh(g) + g) * up for g, up in halved])

        def add_fed():
            for n, s in enumerate(feed):
                set_blocks(res_ref, [rows_of(s)], [
                    a + o for a, o in zip(blocks_at(res_ref, rows_of(s)), _narrowed(fed, n))])
            yield

        def begin(name):
            stage, g = name[0], int(name[1:])
            tiles = slice(g * _UNIT, (g + 1) * _UNIT)
            if stage in "QKV":
                return project("QKV".index(stage), g), _count(_SIXTEEN, n_layers)
            if stage in "SA":
                return (score if stage == "S" else average)(g), g
            if stage == "X":
                return next(early_passes), _count(_SIXTEEN)
            if stage in "NF":
                return (hand_over if stage == "N" else add_fed)(), 1
            if stage == "T":
                return transpose_out(finished), _FULL + 1
            w_ref, scheme = unit(name)
            if stage == "O":
                return _narrow(mixed, heads[tiles], w_ref, scheme, paced), _count(scheme, n_layers)
            if stage == "G":
                return gated(w_ref, scheme), _count(scheme)
            return _narrow(fed, hidden[tiles], w_ref, scheme, paced), _count(scheme)

        for names in order.split():
            main, *others = [begin(name) for name in names.split("+")]
            _interleave(*main, others)

    arriving = " ".join(_ARRIVALS.values()).split()

    def staging(name):
        alike = [other for other in arriving if (other[0] in "QKV") == (name[0] in "QKV")]
        buffers = head_stages if name[0] in "QKV" else column_stages
        return buffers[alike.index(name) % len(buffers)]

    def weight_copies(name):
        stage, g, count = name[0], int(name[1:]), len(unit(name)[1].piece)
        if stage in "QKV":
            w = (wq_hbm, wk_hbm, wv_hbm)["QKV".index(stage)].bitcast(jnp.uint32)
            pairs = [(w.at[:, g * _UNIT // 2 + p, :], staging(name).at[p])
                     for p in range(count // 2)]
        elif stage == "O":
            pairs = [(wot_hbm.bitcast(jnp.uint32).at[g * _UNIT + t], staging(name).at[:, _cols(t)])
                     for t in range(count)]
        else:
            sources = (w1_hbm, w3_hbm) if stage == "G" else (w2t_hbm,)
            width, count = _UNIT // len(sources), count // len(sources)
            pairs = [(w.bitcast(jnp.uint32).at[:, _cols(g * width, count)],
                      staging(name).at[:, _cols(side * width, count)])
                     for side, w in enumerate(sources)]
        return [pltpu.make_async_copy(*pair, weight_sem.at[arriving.index(name)])
                for pair in pairs]

    def combined(name):
        def part(t, p):
            if name[0] in "QKV":
                words = staging(name)[t // 2, pl.ds(p * _T // 2, _T // 2), :]
                words = words & jnp.uint32(0xFFFF0000) if t % 2 else words << 16
                return pltpu.bitcast(words, jnp.float32)
            column = t % 2 * (_UNIT // 2) + t // 2 if name[0] == "G" else t
            return _unpack(staging(name)[pl.ds(p * _T // 4, _T // 4), _cols(column)])

        return _combine(part, *unit(name), transposed=name[0] in "OD")

    def x_copy(i):
        cols = pl.ds(pl.multiple_of(i * _T, _T), _T)
        return pltpu.make_async_copy(xt_hbm.at[:, cols], tile_ref.at[i], tile_sem.at[i])

    def transpose_in(i):
        x = tile_ref[i].astype(jnp.float32)
        x = jnp.concatenate([x, x[_FULL * _T:]], axis=0)
        blocks = [x[b * _T:(b + 1) * _T].T for b in range(_FULL + 1)]
        set_blocks(res_ref, [pl.ds(pl.multiple_of(i * _T, _T), _T)], blocks)
        normed = _layernorm([
            jnp.concatenate([x[s - _EARLY:s] for s in range(seg, _T + 1, seg)], axis=0)
            for x in blocks])
        for s in range(_T // seg):
            at = (i * (_T // seg // 2) + s // 2) * _EARLY
            set_blocks(early_norm_ref, [s % 2, pl.ds(pl.multiple_of(at, _EARLY), _EARLY)],
                       [x[s * _EARLY:(s + 1) * _EARLY] for x in normed])

    due = []

    def paced(x):
        for r in range(0, x.shape[0] if due else 0, 8):
            token = due.pop() if due else None
            if token is not None:
                waiting = jnp.where(loaded, x[r:r + 8], pltpu.bitcast(token, jnp.float32))
                x = jnp.concatenate([y for y in (x[:r] if r else None, waiting,
                                                 x[r + 8:] if r + 8 < x.shape[0] else None)
                                     if y is not None], axis=0)
        return x

    early_rows = _EARLY_ROWS * len(qkv_refs)
    n_plain = len(early_rows) - (_LAG * _ORDER_FIRST + "X" + _ORDER_BOTH).count("X")

    def early_pass(c):
        n, chunk = divmod(c, len(_EARLY_ROWS))
        first = sum(_EARLY_ROWS[:chunk])
        if c == _FIRST_PASSES:
            for i in range(_FIRST_TILES, n_io):
                x_copy(i).wait()
        if c in _ARRIVALS:
            following = min([later for later in _ARRIVALS if later > c], default=None)
            for name in _ARRIVALS[c].split():
                for copy in weight_copies(name):
                    copy.wait()
        for name in _DEPARTURES.get(c, "").split():
            for copy in weight_copies(name):
                copy.start()
        if c in _ARRIVALS:
            tokens = sum(map(combined, _ARRIVALS[c].split()), [])
            slots = sum(early_rows[c:following or n_plain + _LAG]) * _count(_SIXTEEN) // 8
            if not following:
                slots += _LAG * len(qkv_refs + wo_refs) * _count(_SIXTEEN, 1) * span // 8
            at = {slots * (k + 1) // (len(tokens) + 1): token for k, token in enumerate(tokens)}
            due[:] = [at.get(k) for k in reversed(range(slots if c else 0))]
        rows = pl.ds(first + _LAG // 2 * _EARLY, early_rows[c])
        for i in range(_FIRST_TILES, n_io) if c == _FIRST_PASSES else []:
            transpose_in(i)
        mix = _mixer([blocks_at(early_norm_ref, half, rows) for half in range(2)], False)
        tiles = yield from _widen(mix, qkv_refs[n], _SIXTEEN, 2, paced)
        for t, halves in enumerate(tiles):
            for r in range(0, rows.size, _EARLY):
                for half, x in enumerate(halves):
                    words = pl.ds(first + r + half * _EARLY // 2, _EARLY // 2)
                    early_refs[n][words, _cols(t)] = _pack(x[r:r + _EARLY].astype(jnp.bfloat16))

    def out_copy(i):
        return pltpu.make_async_copy(tile_ref.at[i], outt_hbm.at[:, _cols(i)], tile_sem.at[i])

    def transpose_out(i):
        for b, x in enumerate(blocks_at(res_ref, pl.ds(pl.multiple_of(i * _T, _T), _T))):
            depth = min(_T, d_model - b * _T)
            tile_ref[i, pl.ds(b * _T, depth), :] = x.T[:depth].astype(tile_ref.dtype)
            yield

    def double_step(b):
        step(_ORDER, attend=[b, b + _LAG], feed=[b - 1, b + _LAG - 1],
             finished=jnp.maximum(b - 5, 0) * seg // _T)

    def last_steps():
        step(_ORDER_TAIL, attend=[n_seg - 2], feed=[n_seg - 3, n_seg - 1])
        step(_ORDER_LAST, attend=[n_seg - 1], partner=n_seg - 2)
        step(_ORDER_FFN, feed=[n_seg - 2, n_seg - 1])
        _interleave(transpose_out(n_io - 1))

    if _DEV in ("main", "tail"):
        pl.loop(1, n_seg - _LAG)(double_step if _DEV == "main" else lambda i: last_steps())
        out_copy(n_io - 1).start()
        out_copy(n_io - 1).wait()
        return

    mem_copy = pltpu.make_async_copy(mem0_hbm, mem0_ref, mem_sem)
    for copy in [mem_copy] + [x_copy(i) for i in range(_FIRST_TILES)] + weight_copies(arriving[0]):
        copy.start()

    def load_tile(i, _):
        x_copy(i).wait()
        transpose_in(i)
        return i

    loaded = jax.lax.fori_loop(0, _FIRST_TILES, load_tile, 0) > 0
    for i in range(_FIRST_TILES, n_io):
        x_copy(i).start()
    mem_copy.wait()
    mem0 = mem0_ref[...].astype(jnp.float32)
    mem_ref[0] = mem_ref[1] = jnp.concatenate([mem0, mem0[:, _FULL * _T:]], axis=1)
    early_passes = map(early_pass, range(len(early_rows)))
    for _ in range(n_plain):
        _interleave(next(early_passes))
    for s in range(_LAG):
        step(_ORDER_FIRST, attend=[s], partner=0)
    step(_ORDER_FFN, feed=[0, 1])
    _interleave(next(early_passes))
    mem_ref[0], mem_ref[1] = mem_ref[1], mem_ref[0]
    step(_ORDER_BOTH, attend=[0, _LAG])
    pl.loop(1, n_seg - _LAG)(double_step)
    for i in range(n_io - 1):
        out_copy(i).start()
    last_steps()
    out_copy(n_io - 1).start()
    for i in range(n_io):
        out_copy(i).wait()


@functools.partial(jax.jit, static_argnames=("A_seg_len",))
def pallas_interleave_layers__memory_aug_recurrent_mem_tr__glu_gated_swiglu__prompt_kernel(
    A_x: jax.Array,
    A_mem0: jax.Array,
    A_Wq: jax.Array,
    A_Wk: jax.Array,
    A_Wv: jax.Array,
    A_Wo: jax.Array,
    A_seg_len: int,
    B_x: jax.Array,
    B_w1: jax.Array,
    B_w3: jax.Array,
    B_w2: jax.Array,
):
    del B_x
    _, n_tok, d_model = A_x.shape
    n_mem = A_mem0.shape[1]
    _, n_heads, d_head = A_Wq.shape
    d_ff = B_w1.shape[1]
    assert A_x.shape[0] == 1 and 4 * A_seg_len == _T and n_mem == 8
    assert (d_model, n_heads, d_head, d_ff) == (576, 2 * _UNIT, _T, 36 * _T)
    early_rows = (n_tok // A_seg_len - _LAG) * _EARLY
    width = (_FULL + 1) * _T
    hbm = pl.BlockSpec(memory_space=pltpu.HBM)

    def weights(scheme, *units):
        return pltpu.VMEM((*units, _T // 2, _count(scheme) * _T), jnp.uint32)

    out_t = pl.pallas_call(
        functools.partial(_kernel, seg=A_seg_len),
        out_shape=jax.ShapeDtypeStruct((d_model, n_tok), A_x.dtype),
        in_specs=[hbm] * 9,
        out_specs=hbm,
        scratch_shapes=[
            pltpu.VMEM((n_mem, d_model), A_mem0.dtype),
            pltpu.VMEM((n_tok // _T, d_model, _T), A_x.dtype),
            pltpu.VMEM((n_tok, width), jnp.float32),
            pltpu.VMEM((2, n_mem, width), jnp.float32),
            pltpu.VMEM((2, A_seg_len, width), jnp.float32),
            pltpu.VMEM((2, n_tok // A_seg_len * _EARLY // 2, width), jnp.float32),
            [pltpu.VMEM((early_rows // 2, _UNIT * _T), jnp.uint32)] * 6,
            [weights(_SIXTEEN)] * 6,
            [weights(_SIXTEEN)] * 2,
            [weights(_SIXTEEN)] * 4 + [weights(_EIGHT)],
            [weights(_SIXTEEN)] * 2 + [weights(_FOUR)],
            [pltpu.VMEM((_UNIT // 2, d_model, _T), jnp.uint32)] * 3,
            [pltpu.VMEM((d_model // 2, _UNIT * _T), jnp.uint32)] * 8,
            pltpu.SemaphoreType.DMA((16,)),
            pltpu.SemaphoreType.DMA((n_tok // _T,)),
            pltpu.SemaphoreType.DMA,
        ],
        compiler_params=pltpu.CompilerParams(vmem_limit_bytes=124 * 1024 * 1024, flags=_FLAGS,
                                             disable_bounds_checks=True),
    )(A_x.reshape(n_tok, d_model).T, A_mem0.reshape(n_mem, d_model), A_Wq, A_Wk, A_Wv,
      A_Wo.transpose(0, 2, 1), B_w1, B_w3, B_w2.T)
    return out_t.T.reshape(A_x.shape)
```

```python
import functools
import math
from typing import NamedTuple

import jax
import jax.numpy as jnp
import jax.experimental.pallas as pl
import jax.experimental.pallas.tpu as pltpu

_EPS = 1e-05
_MASKED = -1000000000.0
_LOG2E = math.log2(math.e)
_T = 128
_FULL = 4
_UNIT = 16
_LAG = 2
_EARLY = 16
_EARLY_ROWS = (48,) * 9 + (32,) * 2
_FIRST_TILES = 5
_TILES_ARRIVE = 2
_UNIT_ARRIVES = 7
_ORDER = ("G0 Q0 K0 K1+S6 Q1+S3+T0 V0+S5 G1+S11+A6 V1+S7+A10 O0+A15 G2+A1 O1 G3+N0 G4 "
          "D1 D0 D2 F0")
_ORDER_HEAD = "Q0 K0 Q1+S8 K1+S8 V0+S16 V1+A16 O0+A16 O1 X0+N0"
_ORDER_TAIL = "G0 G1 G2 G3 G4 Q0 K0 Q1+S8 K1+S8 V0+S8 V1+S8+A16 D0 D1 D2 F0 O0+A16 O1 N0"
_ORDER_LAST = "Q0 K0 Q1+S8 K1+S8 V0+S16 V1+A16 O0+A16 O1 N0"
_ORDER_FFN = "G0 G1 G2 G3 G4 D0 D1 D2 F0"
_LEAD = 0.1


class _Product(NamedTuple):
    rows: tuple
    weights: tuple
    tiles: tuple


class _Scheme(NamedTuple):
    piece: tuple
    helper: tuple
    shared: tuple
    main: tuple


def _pair_up(blocks, left, right, edges):
    products = []
    edges = [(u, blocks[u][i], v, blocks[v][j]) for u, i, v, j in edges]
    assert all(i in blocks[v] and j in blocks[u] for u, i, v, j in edges)

    def add(rows, weights, tiles):
        rows = tuple(sorted(rows, key=lambda term: term[1:]))
        if rows[0][0] < 0:
            rows = tuple((-s, half, i) for s, half, i in rows)
            tiles = tuple((-s, half, t) for s, half, t in tiles)
        products.append(_Product(rows, tuple(weights), tuple(tiles)))

    def unpaired_blocks(t, half):
        mine = [((i, v, j), (j, u, i))[half] for u, i, v, j in edges if (u, v)[half] == t]
        for i in blocks[t]:
            if any(i == j for _, _, j in mine):
                continue
            partners = [(p, j) for own, p, j in mine if own == i]
            if not partners:
                add([(1, 0, i)], [(1, t, i)], [(1, 0, t)])
                add([(1, 1, i)], [(1, t, i)], [(1, 1, t)])
                continue
            add([(1, half, i)], [(1, t, i)] + [(1, t, j) for _, j in partners],
                [(1, half, t), (-1, 1 - half, t)])
            add([(1, 0, i), (1, 1, i)], [(1, t, i)] + [(-1, p, i) for p, _ in partners],
                [(1, 1 - half, t)])

    for t in left:
        unpaired_blocks(t, 0)
        for u, i, v, j in edges:
            if u == t:
                add([(1, 1, i), (-1, 1, j)], [(1, v, i)], [(1, 1, v), (1, 1, u)])
                add([(1, 0, j), (-1, 0, i)], [(1, u, j)], [(1, 0, u), (1, 0, v)])
                add([(1, 0, i), (1, 1, j)], [(1, u, j), (1, v, i)], [(1, 1, u), (1, 0, v)])
    for t in right:
        unpaired_blocks(t, 1)
    return products


def _scheme(n):
    if n == 4:
        piece = [0, 0, 1, 1]
        groups = [([u], [u + 1], [(u, 0, u + 1, 2), (u, 1, u + 1, 3)]) for u in (0, 2)]
    else:
        piece = [2 * (t // 8) + ((t % 4 == t // 8) == (t % 8 >= 4)) for t in range(n)]
        groups = [(range(g, g + 4), range(g + 4, g + 8),
                   [(g + i, i, g + 4 + j, j) for i in range(4) for j in range(4) if i != j])
                  for g in range(0, n, 8)]
    helper = [n + piece[:t].count(piece[t]) for t in range(n)]
    helpers = range(n, max(helper) + 1)
    blocks = [[_FULL + p if i == p // 2 else i for i in range(_FULL)] for p in piece]
    blocks += [range(max(piece) // 2 + 1)] * len(helpers)
    shared = [p for u in helpers[::2] for p in _pair_up(
        blocks, [u], [u + 1], [(u, 0, u + 1, 1)] if len(blocks[u]) == 2 else [])]
    return _Scheme(tuple(piece), tuple(helper), tuple(shared),
                   tuple(p for group in groups for p in _pair_up(blocks, *group)))


_WHOLE, _GATE_REST, _DOWN_REST = _scheme(_UNIT), _scheme(8), _scheme(4)


def _numbered(scheme, n_halves):
    kept = [], []
    for n, (rows, weights, tiles) in enumerate(scheme.shared + scheme.main):
        rows = tuple(term for term in rows if term[1] < n_halves)
        tiles = tuple(term for term in tiles if term[1] < n_halves)
        if rows and tiles:
            kept[n >= len(scheme.shared)].append((n, _Product(rows, weights, tiles)))
    return kept


def _count(scheme, n_halves=2):
    return sum(map(len, _numbered(scheme, n_halves)))


def _plain(block):
    return block if block < _FULL else (block - _FULL) // 2


def _signed_sum(terms):
    (sign, total), *rest = sorted(terms, key=lambda term: -term[0])
    for s, value in rest:
        total = total + value if s == sign else total - value
    return total if sign > 0 else -total


def _accumulate(acc, key, sign, value):
    if key in acc:
        s, total = acc[key]
        if s == sign:
            acc[key] = s, total + value
        else:
            acc[key] = 1, total - value if s > 0 else value - total
    else:
        acc[key] = sign, value


def _interleave(main, count=0, others=()):
    due = sorted((count * (_LEAD + (1 - _LEAD) * (k + m / len(others)) / n), m, k)
                 for m, (_, n) in enumerate(others) for k in range(n))
    for done, _ in enumerate(main):
        while due and due[0][0] <= done:
            next(others[due.pop(0)[1]][0])
    for other, _ in others:
        for _ in other:
            pass


def _dot(a, b, axis=0):
    return jax.lax.dot_general(a, b, (((1,), (axis,)), ((), ())),
                               preferred_element_type=jnp.float32)


def _pack(x):
    return pltpu.bitcast(x, jnp.uint32)


def _unpack(words):
    return pltpu.bitcast(words, jnp.bfloat16)


def _cols(n, width=1):
    return slice(n * _T, (n + width) * _T)


def _stack(*parts):
    return jnp.concatenate(parts, axis=0)


def _splice(low, high):
    lane = jax.lax.broadcasted_iota(jnp.int32, low.shape, 1)
    return jnp.where(lane < _T // 2, low, high)


def _layernorm(blocks):
    def mean(terms):
        total = sum(terms[:-1], 0.5 * terms[-1])
        return jnp.sum(total, axis=-1, keepdims=True) * (1 / ((_FULL + 0.5) * _T))

    center = mean(blocks)
    d = [x - center for x in blocks]
    inv = jax.lax.rsqrt(mean([x * x for x in d]) + _EPS)
    return [x * inv for x in d]


def _mixer(halves, dtype=jnp.float32):
    @functools.cache
    def block(half, i):
        x, rest = halves[half][_plain(i)], halves[half][_FULL]
        if i < _FULL:
            return x
        return _splice(x, rest) if (i - _FULL) % 2 else _splice(rest, x)

    return functools.cache(
        lambda rows: _signed_sum([(s, block(half, i)) for s, half, i in rows]).astype(dtype))


def _weights(w_ref):
    w = _unpack(w_ref[...])
    return functools.cache(lambda n: w[:, _cols(n)])


def _widen(mix, n_halves, weights, scheme):
    acc = {}
    for products in _numbered(scheme, n_halves):
        if acc:
            acc = {(t, half): acc[h, half] for t, h in enumerate(scheme.helper)
                   for half in range(n_halves)}
        for n, (rows, _, tiles) in products:
            value = _dot(mix(rows), weights(n))
            for s, half, t in tiles:
                _accumulate(acc, (t, half), s, value)
            yield
    return [[_signed_sum([acc[t, half]]) for half in range(n_halves)]
            for t in range(len(scheme.piece))]


def _narrow(acc, wide, weights, scheme):
    n_halves = len(wide[0])
    wide = wide + [
        [_signed_sum([(1, x[half]) for x, h in zip(wide, scheme.helper) if h == helper])
         for half in range(n_halves)] for helper in range(len(wide), max(scheme.helper) + 1)]
    by_rows = {}
    for n, product in sum(_numbered(scheme, n_halves)[::-1], []):
        by_rows.setdefault(product.rows, []).append((n, product.tiles))
    for rows in sorted(by_rows, key=lambda rows: sorted({-i for _, _, i in rows})):
        total = {}
        for n, tiles in by_rows[rows]:
            sign = max(s for s, _, _ in tiles)
            lhs = _signed_sum([(s * sign, wide[t][half]) for s, half, t in tiles])
            _accumulate(total, rows, sign, _dot(lhs, weights(n)))
            yield
        for s, half, i in rows:
            _accumulate(acc, (half, i), s * total[rows][0], total[rows][1])


def _narrowed(acc, half):
    blocks = [_signed_sum([acc[half, i]]) for i in range(2 * _FULL)]
    folded = list(zip(blocks[_FULL::2], blocks[_FULL + 1::2]))
    rest = _signed_sum([(1, _splice(low, high)) for low, high in folded])
    rest += jnp.concatenate([rest[:, _T // 2:], rest[:, :_T // 2]], axis=1)
    return ([x + _splice(high, low) for x, (low, high) in zip(blocks, folded)]
            + blocks[len(folded):_FULL] + [rest])


def _combine(part, w_ref, scheme, transposed=False):
    donor = {(h, p): t for t, (h, p) in enumerate(zip(scheme.helper, scheme.piece))}
    products = scheme.shared + scheme.main
    uses = {}
    for n in sorted(range(len(products)), key=lambda n: len(products[n].weights) > 1):
        for s, t, i in products[n].weights:
            uses.setdefault((t, i), []).append((s, n))

    def folded(t, p):
        if t >= len(scheme.piece):
            return part(donor[t, p], p)
        if p == scheme.piece[t]:
            return part(t, 2 * _FULL)
        if (scheme.helper[t], p) in donor:
            return (part(t, p).astype(jnp.float32)
                    - folded(scheme.helper[t], p).astype(jnp.float32))
        return part(t, p)

    acc, missing, stored = {}, [len(product.weights) for product in products], []
    for t, i in sorted(uses, key=lambda source: uses[source][0][1]):
        w = _stack(*[folded(t, 2 * _plain(i) + side) for side in range(2)])
        exact = w.astype(jnp.float32)
        for s, n in uses[t, i]:
            _accumulate(acc, n, s, exact if len(products[n].weights) > 1 else w)
            missing[n] -= 1
            if not missing[n]:
                w_ref[:, _cols(n)] = _pack(_signed_sum([acc.pop(n)]).astype(jnp.bfloat16))
                stored.append(w_ref[:, _cols(n)])
    stored = [functools.reduce(jnp.bitwise_or, stored[n:n + 4]) for n in range(0, len(stored), 4)]
    stored = [pltpu.bitcast(words, jnp.float32) for words in stored]
    tokens = [words[r:r + 8] for r in range(0, _T // 2, 8) for words in stored]
    for n in range(len(products) if transposed else 0):
        w_ref[:, _cols(n)] = words = _pack(_unpack(w_ref[:, _cols(n)]).T)
        tokens.append(pltpu.bitcast(words[-8:], jnp.float32))
    return tokens


def _kernel(xt_hbm, mem0_hbm, wq_hbm, wk_hbm, wv_hbm, wot_hbm, w1_hbm, w3_hbm, w2t_hbm,
            outt_hbm, tile_ref, res_ref, norm_ref, early_norm_ref, early_ref, qkv_ref, gate_ref,
            back_ref, gate_rest_ref, down_rest_ref, qkv_stage, gate_stage, back_stage, mem_ref,
            mem0_ref, qkv_sem, other_sem, tile_sem, mem_sem, *, seg):
    d_model, n_tok = xt_hbm.shape
    n_mem = mem0_hbm.shape[0]
    n_seg = n_tok // seg
    n_io = n_tok // _T
    span = n_mem + seg
    score_scale = wq_hbm.shape[2] ** -0.5 * _LOG2E
    n_qkv, n_gate = early_ref.shape[0], gate_ref.shape[0]
    n_wo = n_qkv // 3

    def blocks_at(ref, *index):
        return [ref[(*index, _cols(i))] for i in range(_FULL + 1)]

    def set_blocks(ref, index, blocks):
        for i, x in enumerate(blocks):
            ref[(*index, _cols(i))] = x

    def part_of(i, size):
        return pl.ds(pl.multiple_of(i * size, size), size)

    def step(order, attend=(), feed=(), partner=None, finished=None, filler=None):
        n_layers = len(attend)
        operand = jnp.bfloat16 if n_layers == 2 else jnp.float32
        qkv, probs, heads, hidden, mixed, fed = {"Q": [], "K": [], "V": []}, [], [], [], {}, {}
        if attend:
            query, key = (jax.lax.broadcasted_iota(jnp.int32, (span, _T), a) for a in (0, 1))
            own_keys = [(key >= n * span) & (key < (n + 1) * span) for n in range(n_layers)]
            visible = (query < n_mem) | (query >= jnp.where(key < span, key, key - span))
            mem = [blocks_at(mem_ref, n, slice(None)) for n in range(n_layers)]
            h = _layernorm(blocks_at(res_ref, part_of(attend[0], seg)))
            if n_layers == 1:
                attend_mix = _mixer([list(map(_stack, mem[0], h))])
            else:
                ahead = _layernorm(
                    [x[:seg - _EARLY] for x in blocks_at(res_ref, part_of(attend[1], seg))])
                cut = seg - _EARLY // 2
                known = part_of(attend[0] % 2 * (sum(_EARLY_ROWS) // _EARLY) + attend[0] // 2,
                                _EARLY // 2)
                attend_mix = _mixer(
                    [[_stack(m, a[:cut]) for m, a in zip(mem[0], h)],
                     [_stack(m, a[cut:], b) for m, a, b in zip(mem[1], h, ahead)]], operand)
        if feed:
            feed_mix = _mixer([blocks_at(norm_ref, n, slice(None)) for n in range(2)])

        def project(stage, n):
            tiles = yield from _widen(attend_mix, n_layers, _weights(qkv_ref.at[n]), _WHOLE)
            if n_layers == 1:
                qkv[stage] += [halves[0] for halves in tiles]
                return
            moved = n_mem + _EARLY // 2
            early = _unpack(early_ref[n, known, :]).astype(jnp.float32)
            for t, (a, b) in enumerate(tiles):
                x = _stack(a, b[n_mem:moved], b[:n_mem], b[moved:], early[:, _cols(t)])
                if stage == "V":
                    x = _stack(x, jnp.zeros((_T - 2 * span, _T), x.dtype))
                qkv[stage].append(x if stage == "Q" else x.astype(operand))

        def score(count):
            for t in range(len(probs), len(probs) + count):
                s = _dot(qkv["Q"][t], qkv["K"][t], axis=1)
                if n_layers == 2:
                    s = jnp.where(own_keys[1][:, :2 * span], s[span:], s[:span])
                s = jnp.concatenate(
                    [s * score_scale, jnp.zeros((span, _T - s.shape[1]), s.dtype)], axis=1)
                s = jnp.where(visible, s, _MASKED * _LOG2E)
                top = [jnp.max(jnp.where(own, s, -jnp.inf), axis=-1, keepdims=True)
                       for own in own_keys]
                p = jnp.exp2(s - jnp.where(own_keys[-1], top[-1], top[0]))
                p = _stack(*[jnp.where(own, p, 0.0) for own in own_keys])
                probs.append((p.astype(operand), pltpu.reciprocal(
                    jnp.sum(p, axis=-1, keepdims=True), approx=True)))
                yield

        def average(count):
            for t in range(len(heads), len(heads) + count):
                (p, inv), v = probs[t], qkv["V"][t]
                both = _dot(p[:, :v.shape[0]], v) * inv
                heads.append([both[n * span:(n + 1) * span] for n in range(n_layers)])
                yield

        def add_attended():
            x = [] if partner is None else [blocks_at(res_ref, part_of(partner, seg))]
            before = [blocks_at(res_ref, part_of(s, seg)) for s in attend]
            for n, s in enumerate(attend):
                out = _narrowed(mixed, n)
                x.append([a + o[n_mem:] for a, o in zip(before[n], out)])
                set_blocks(res_ref, [part_of(s, seg)], x[-1])
                set_blocks(mem_ref, [n, slice(None)], [o[:n_mem] for o in out])
            for n, blocks in enumerate(x):
                set_blocks(norm_ref, [n, slice(None)], _layernorm(blocks))
                yield

        def gated(w_ref, scheme):
            tiles = yield from _widen(feed_mix, 2, _weights(w_ref), scheme)
            for pair in zip(tiles[::2], tiles[1::2]):
                halved = [(0.5 * gate, up) for gate, up in zip(*pair)]
                hidden.append([(g * jnp.tanh(g) + g) * up for g, up in halved])

        def add_fed():
            before = [blocks_at(res_ref, part_of(s, seg)) for s in feed]
            for n, s in enumerate(feed):
                set_blocks(res_ref, [part_of(s, seg)],
                           [a + o for a, o in zip(before[n], _narrowed(fed, n))])
            yield

        def begin(name):
            stage, number = name[0], int(name[1:])
            if stage in "SA":
                return (score if stage == "S" else average)(number), number
            if stage in "NF":
                return (add_attended if stage == "N" else add_fed)(), 1
            if stage == "T":
                return transpose_out(finished), _FULL + 1
            if stage == "X":
                return filler, _count(_WHOLE)
            if stage in "QKV":
                return project(stage, 3 * number + "QKV".index(stage)), _count(_WHOLE, n_layers)
            if stage == "G":
                unit = ((gate_ref.at[number], _WHOLE) if number < n_gate
                        else (gate_rest_ref, _GATE_REST))
                return gated(*unit), _count(unit[1])
            acc, wide, n = (mixed, heads, number) if stage == "O" else (fed, hidden, n_wo + number)
            w_ref, scheme = (back_ref.at[n], _WHOLE) if n < n_gate else (down_rest_ref, _DOWN_REST)
            wide = wide[number * _UNIT:(number + 1) * _UNIT]
            return _narrow(acc, wide, _weights(w_ref), scheme), _count(scheme, len(wide[0]))

        for names in order.split():
            main, *others = map(begin, names.split("+"))
            _interleave(*main, others)

    def start(copy):
        copy.start()

    def wait(copy):
        copy.wait()

    def when(condition, act, copies):
        @pl.when(condition)
        def _():
            for copy in copies():
                act(copy)

    def move_qkv(act, n, pairs=range(_UNIT // 2)):
        for which, w in enumerate((wq_hbm, wk_hbm, wv_hbm)):
            when((n < n_qkv) & (n % 3 == which), act, lambda w=w: [
                pltpu.make_async_copy(w.bitcast(jnp.uint32).at[:, n // 3 * (_UNIT // 2) + p, :],
                                      qkv_stage.at[n % 2, p], qkv_sem.at[n % 2]) for p in pairs])

    def move_others(act, n):
        def columns(w_hbm, first, count, stage, offset=0):
            cols = pl.ds(pl.multiple_of(first * _T, _T), count * _T)
            return pltpu.make_async_copy(w_hbm.bitcast(jnp.uint32).at[:, cols],
                                         stage.at[n % 2, :, _cols(offset, count)],
                                         other_sem.at[n % 2])

        for active, gate, down in ((n < n_gate, _WHOLE, _WHOLE),
                                   (n == n_gate, _GATE_REST, _DOWN_REST)):
            when(active, act, lambda count=len(gate.piece) // 2: [
                columns(w, n * (_UNIT // 2), count, gate_stage, side * _UNIT // 2)
                for side, w in enumerate((w1_hbm, w3_hbm))])
            when(active & (n >= n_wo), act, lambda count=len(down.piece): [
                columns(w2t_hbm, (n - n_wo) * _UNIT, count, back_stage)])
        when(n < n_wo, act, lambda: [
            pltpu.make_async_copy(wot_hbm.bitcast(jnp.uint32).at[n * _UNIT + t],
                                  back_stage.at[n % 2, :, _cols(t)], other_sem.at[n % 2])
            for t in range(_UNIT)])

    def halves_of(x):
        return lambda p: x[p * _T // 2:(p + 1) * _T // 2]

    def combine_qkv(n, w_ref):
        tiles = []
        for pair in range(_UNIT // 2):
            words = qkv_stage[n % 2, pair]
            tiles += [halves_of(pltpu.bitcast(head, jnp.float32))
                      for head in (words << 16, words & jnp.uint32(0xFFFF0000))]
        return _combine(lambda t, p: tiles[t](p), w_ref, _WHOLE)

    def combine_others(n, gate, back):
        gates = [halves_of(_unpack(gate_stage[n % 2, :, _cols(t % 2 * _UNIT // 2 + t // 2)]))
                 for t in range(len(gate[1].piece))]
        backs = [halves_of(_unpack(back_stage[n % 2, :, _cols(t)]))
                 for t in range(len(back[1].piece))]
        return (_combine(lambda t, p: backs[t](p), *back, transposed=True)
                + _combine(lambda t, p: gates[t](p), *gate))

    def x_copy(i):
        return pltpu.make_async_copy(xt_hbm.at[:, part_of(i, _T)], tile_ref.at[i], tile_sem.at[i])

    def out_copy(i):
        return pltpu.make_async_copy(tile_ref.at[i], outt_hbm.at[:, _cols(i)], tile_sem.at[i])

    def transpose_in(i):
        x = tile_ref[i].astype(jnp.float32)
        x = _stack(x, x[_FULL * _T:])
        blocks = [x[b * _T:(b + 1) * _T].T for b in range(_FULL + 1)]
        set_blocks(res_ref, [part_of(i, _T)], blocks)
        normed = _layernorm(
            [_stack(*[x[s - _EARLY:s] for s in range(seg, _T + 1, seg)]) for x in blocks])
        for s in range(_T // seg):
            rows = part_of(i * (_T // seg // 2) + s // 2, _EARLY)
            set_blocks(early_norm_ref, [s % 2, rows],
                       [x[s * _EARLY:(s + 1) * _EARLY] for x in normed])

    def transpose_out(i):
        for b, x in enumerate(blocks_at(res_ref, part_of(i, _T))):
            depth = min(_T, d_model - b * _T)
            tile_ref[i, pl.ds(b * _T, depth), :] = x.T[:depth].astype(tile_ref.dtype)
            yield

    def early_pass(n, weights, first, count, paced=lambda x: x):
        rows = pl.ds(pl.multiple_of(first + _LAG // 2 * _EARLY, _EARLY), count)
        mix = _mixer([blocks_at(early_norm_ref, half, rows) for half in range(2)])
        tiles = yield from _widen(lambda key: paced(mix(key)), 2, weights, _WHOLE)
        for half in range(2):
            at = pl.multiple_of((half * sum(_EARLY_ROWS) + first) // 2, _EARLY // 2)
            early_ref.at[n][pl.ds(at, count // 2), :] = _pack(jnp.concatenate(
                [halves[half] for halves in tiles], axis=1).astype(jnp.bfloat16))

    def early_passes(n, w_ref, chunks, tokens=()):
        total = sum(_EARLY_ROWS[c] for c in chunks) * _count(_WHOLE)
        due = [(total * (k + 1) // (len(tokens) + 1), token) for k, token in enumerate(tokens)]
        done = 0

        def paced(x):
            nonlocal done
            done += x.shape[0]
            while due and due[0][0] <= done:
                x = _stack(x[:-8], jnp.where(always, x[-8:], due.pop(0)[1]))
            return x

        weights = _weights(w_ref)
        for c in chunks:
            _interleave(early_pass(n, weights, sum(_EARLY_ROWS[:c]), _EARLY_ROWS[c], paced))

    def double_step(b):
        step(_ORDER, attend=[b, b + _LAG], feed=[b - 1, b + _LAG - 1],
             finished=jnp.maximum(b - 1 - _T // seg, 0) * seg // _T)

    mem_copy = pltpu.make_async_copy(mem0_hbm, mem0_ref, mem_sem)
    for copy in [mem_copy] + [x_copy(i) for i in range(_FIRST_TILES)]:
        copy.start()
    move_qkv(start, 0, range(_UNIT // 4))
    mem_copy.wait()
    move_qkv(start, 0, range(_UNIT // 4, _UNIT // 2))

    def load_tile(i, _):
        x_copy(i).wait()
        transpose_in(i)
        return i

    always = jax.lax.fori_loop(0, _FIRST_TILES, load_tile, 0) > 0
    mem0 = mem0_ref[...].astype(jnp.float32)
    mem_ref[0] = mem_ref[1] = jnp.concatenate([mem0, mem0[:, _FULL * _T:]], axis=1)
    for i in range(_FIRST_TILES, n_io):
        x_copy(i).start()

    chunks = range(len(_EARLY_ROWS))
    move_qkv(wait, 0)
    move_qkv(start, 1)
    combine_qkv(0, qkv_ref.at[0])
    early_passes(0, qkv_ref.at[0], chunks[:_TILES_ARRIVE])
    for i in range(_FIRST_TILES, n_io):
        x_copy(i).wait()
    move_qkv(start, 2)
    for i in range(_FIRST_TILES, n_io):
        transpose_in(i)
    early_passes(0, qkv_ref.at[0], chunks[_TILES_ARRIVE:_UNIT_ARRIVES])
    move_qkv(wait, 1)
    move_others(start, 0)
    early_passes(0, qkv_ref.at[0], chunks[_UNIT_ARRIVES:], combine_qkv(1, qkv_ref.at[1]))

    @pl.loop(1, n_qkv - 1)
    def _load_units(n):
        both = qkv_ref.at[pl.ds(n, 2)]
        move_qkv(start, n + 2)
        move_qkv(wait, n + 1)
        early_passes(n, both.at[0], chunks[:3], combine_qkv(n + 1, both.at[1]))
        move_others(start, n)
        move_others(wait, n - 1)
        early_passes(n, both.at[0], chunks[3:], combine_others(
            n - 1, (gate_ref.at[n - 1], _WHOLE), (back_ref.at[n - 1], _WHOLE)))

    def filler(first, count):
        return early_pass(n_qkv - 1, _weights(qkv_ref.at[n_qkv - 1]), first, count)

    move_others(wait, n_gate)
    early_passes(n_qkv - 1, qkv_ref.at[n_qkv - 1], chunks[:-_LAG - 2], combine_others(
        n_gate, (gate_rest_ref, _GATE_REST), (down_rest_ref, _DOWN_REST)))
    for s in range(_LAG):
        c = s - _LAG - 2
        step(_ORDER_HEAD, attend=[s], partner=0,
             filler=filler(sum(_EARLY_ROWS[:c]), _EARLY_ROWS[c]))
    step(_ORDER_FFN + " X0", feed=[0, 1], filler=filler(sum(_EARLY_ROWS[:-2]), _EARLY_ROWS[-2]))
    mem_ref[0], mem_ref[1] = mem_ref[1], mem_ref[0]
    step(_ORDER_HEAD, attend=[0, _LAG], filler=filler(sum(_EARLY_ROWS[:-1]), _EARLY_ROWS[-1]))
    pl.loop(1, n_seg - _LAG)(double_step)
    for i in range(n_io - 1):
        out_copy(i).start()
    step(_ORDER_TAIL, attend=[n_seg - 2], feed=[n_seg - 3, n_seg - 1])
    step(_ORDER_LAST, attend=[n_seg - 1], partner=n_seg - 2)
    step(_ORDER_FFN + " T0", feed=[n_seg - 2, n_seg - 1], finished=n_io - 1)
    out_copy(n_io - 1).start()
    for i in range(n_io):
        out_copy(i).wait()


@functools.partial(jax.jit, static_argnames=("A_seg_len",))
def pallas_interleave_layers__memory_aug_recurrent_mem_tr__glu_gated_swiglu__prompt_kernel(
    A_x: jax.Array,
    A_mem0: jax.Array,
    A_Wq: jax.Array,
    A_Wk: jax.Array,
    A_Wv: jax.Array,
    A_Wo: jax.Array,
    A_seg_len: int,
    B_x: jax.Array,
    B_w1: jax.Array,
    B_w3: jax.Array,
    B_w2: jax.Array,
):
    del B_x
    _, n_tok, d_model = A_x.shape
    n_mem = A_mem0.shape[1]
    assert A_x.shape == (1, 2048, 576) and A_seg_len == 32 and n_mem == 8
    assert A_Wq.shape[1:] == (2 * _UNIT, _T) and B_w1.shape[1] == 36 * _T
    width = (_FULL + 1) * _T
    hbm = pl.BlockSpec(memory_space=pltpu.HBM)

    def weights(scheme, *units):
        return pltpu.VMEM((*units, _T // 2, _count(scheme) * _T), jnp.uint32)

    out_t = pl.pallas_call(
        functools.partial(_kernel, seg=A_seg_len),
        out_shape=jax.ShapeDtypeStruct((d_model, n_tok), A_x.dtype),
        in_specs=[hbm] * 9,
        out_specs=hbm,
        scratch_shapes=[
            pltpu.VMEM((n_tok // _T, d_model, _T), A_x.dtype),
            pltpu.VMEM((n_tok, width), jnp.float32),
            pltpu.VMEM((2, A_seg_len, width), jnp.float32),
            pltpu.VMEM((2, n_tok // A_seg_len * _EARLY // 2, width), jnp.float32),
            pltpu.VMEM((6, sum(_EARLY_ROWS), _UNIT * _T), jnp.uint32),
            weights(_WHOLE, 6), weights(_WHOLE, 4), weights(_WHOLE, 4),
            weights(_GATE_REST), weights(_DOWN_REST),
            pltpu.VMEM((2, _UNIT // 2, d_model, _T), jnp.uint32),
            pltpu.VMEM((2, d_model // 2, _UNIT * _T), jnp.uint32),
            pltpu.VMEM((2, d_model // 2, _UNIT * _T), jnp.uint32),
            pltpu.VMEM((2, n_mem, width), jnp.float32),
            pltpu.VMEM((n_mem, d_model), A_mem0.dtype),
            pltpu.SemaphoreType.DMA((2,)),
            pltpu.SemaphoreType.DMA((2,)),
            pltpu.SemaphoreType.DMA((n_tok // _T,)),
            pltpu.SemaphoreType.DMA,
        ],
        compiler_params=pltpu.CompilerParams(vmem_limit_bytes=116 * 1024 * 1024,
                                             disable_bounds_checks=True),
    )(A_x.reshape(n_tok, d_model).T, A_mem0.reshape(n_mem, d_model), A_Wq, A_Wk, A_Wv,
      A_Wo.transpose(0, 2, 1), B_w1, B_w3, B_w2.T)
    return out_t.T.reshape(A_x.shape)
```

```python
import functools
import itertools
import math
from typing import NamedTuple

import jax
import jax.numpy as jnp
import jax.experimental.pallas as pl
import jax.experimental.pallas.tpu as pltpu

_EPS = 1e-05
_MASKED = -1000000000.0
_LOG2E = math.log2(math.e)
_T = 128
_FULL = 4
_UNIT = 16
_LAG = 2
_EARLY = 16
_EARLY_ROWS = (48,) * 9 + (32,) * 2
_FIRST_TILES = 5
_TILES_ARRIVE = 2
_UNIT_ARRIVES = 7
_ORDER = "G0 K0 Q0 V0 K1 Q1+T0 G1 V1 O0 G2 O1 G3+N0 G4 D1 D0 D2 F0"
_AFTER = {"S": (366, 394, 402, 423, 437, 455, 484, 537, 598, 620, 638, 655, 673, 691, 720, 730, 740, 749, 759, 769, 778, 788, 798, 807, 817, 838, 853, 869, 884, 899, 914, 929),
          "A": (729, 747, 765, 782, 800, 818, 840, 854, 865, 875, 886, 897, 907, 918, 929, 939, 956, 963, 970, 978, 985, 1013, 1019, 1020, 1025, 1033, 1034, 1037, 1041, 1048, 1054, 1074)}
_ORDER_HEAD = "Q0 K0 Q1+S8 K1+S8 V0+S16 V1+A16 O0+A16 O1 X0+N0"
_ORDER_TAIL = "G0 G1 G2 G3 G4 Q0 K0 Q1+S8 K1+S8 V0+S8 V1+S8+A16 D0 D1 D2 F0 O0+A16 O1 N0"
_ORDER_LAST = "Q0 K0 Q1+S8 K1+S8 V0+S16 V1+A16 O0+A16 O1 N0"
_ORDER_FFN = "G0 G1 G2 G3 G4 D0 D1 D2 F0"
_LEAD = 0.1


class _Product(NamedTuple):
    rows: tuple
    weights: tuple
    tiles: tuple


class _Scheme(NamedTuple):
    piece: tuple
    helper: tuple
    shared: tuple
    main: tuple


def _pair_up(blocks, left, right, edges):
    products = []
    edges = [(u, blocks[u][i], v, blocks[v][j]) for u, i, v, j in edges]
    assert all(i in blocks[v] and j in blocks[u] for u, i, v, j in edges)

    def add(rows, weights, tiles):
        rows = tuple(sorted(rows, key=lambda term: term[1:]))
        if rows[0][0] < 0:
            rows = tuple((-s, half, i) for s, half, i in rows)
            tiles = tuple((-s, half, t) for s, half, t in tiles)
        products.append(_Product(rows, tuple(weights), tuple(tiles)))

    def unpaired_blocks(t, half):
        mine = [((i, v, j), (j, u, i))[half] for u, i, v, j in edges if (u, v)[half] == t]
        for i in blocks[t]:
            if any(i == j for _, _, j in mine):
                continue
            partners = [(p, j) for own, p, j in mine if own == i]
            if not partners:
                add([(1, 0, i)], [(1, t, i)], [(1, 0, t)])
                add([(1, 1, i)], [(1, t, i)], [(1, 1, t)])
                continue
            add([(1, half, i)], [(1, t, i)] + [(1, t, j) for _, j in partners],
                [(1, half, t), (-1, 1 - half, t)])
            add([(1, 0, i), (1, 1, i)], [(1, t, i)] + [(-1, p, i) for p, _ in partners],
                [(1, 1 - half, t)])

    for t in left:
        unpaired_blocks(t, 0)
        for u, i, v, j in edges:
            if u == t:
                add([(1, 1, i), (-1, 1, j)], [(1, v, i)], [(1, 1, v), (1, 1, u)])
                add([(1, 0, j), (-1, 0, i)], [(1, u, j)], [(1, 0, u), (1, 0, v)])
                add([(1, 0, i), (1, 1, j)], [(1, u, j), (1, v, i)], [(1, 1, u), (1, 0, v)])
    for t in right:
        unpaired_blocks(t, 1)
    return products


def _scheme(n):
    if n == 4:
        piece = [0, 0, 1, 1]
        groups = [([u], [u + 1], [(u, 0, u + 1, 2), (u, 1, u + 1, 3)]) for u in (0, 2)]
    else:
        piece = [2 * (t // 8) + ((t % 4 == t // 8) == (t % 8 >= 4)) for t in range(n)]
        groups = [(range(g, g + 4), range(g + 4, g + 8),
                   [(g + i, i, g + 4 + j, j) for i in range(4) for j in range(4) if i != j])
                  for g in range(0, n, 8)]
    helper = [n + piece[:t].count(piece[t]) for t in range(n)]
    helpers = range(n, max(helper) + 1)
    blocks = [[_FULL + p if i == p // 2 else i for i in range(_FULL)] for p in piece]
    blocks += [range(max(piece) // 2 + 1)] * len(helpers)
    shared = [p for u in helpers[::2] for p in _pair_up(
        blocks, [u], [u + 1], [(u, 0, u + 1, 1)] if len(blocks[u]) == 2 else [])]
    return _Scheme(tuple(piece), tuple(helper), tuple(shared),
                   tuple(p for group in groups for p in _pair_up(blocks, *group)))


_WHOLE, _GATE_REST, _DOWN_REST = _scheme(_UNIT), _scheme(8), _scheme(4)


def _numbered(scheme, n_halves):
    kept = [], []
    for n, (rows, weights, tiles) in enumerate(scheme.shared + scheme.main):
        rows = tuple(term for term in rows if term[1] < n_halves)
        tiles = tuple(term for term in tiles if term[1] < n_halves)
        if rows and tiles:
            kept[n >= len(scheme.shared)].append((n, _Product(rows, weights, tiles)))
    return kept


def _count(scheme, n_halves=2):
    return sum(map(len, _numbered(scheme, n_halves)))


def _plain(block):
    return block if block < _FULL else (block - _FULL) // 2


def _signed_sum(terms):
    (sign, total), *rest = sorted(terms, key=lambda term: -term[0])
    for s, value in rest:
        total = total + value if s == sign else total - value
    return total if sign > 0 else -total


def _accumulate(acc, key, sign, value):
    if key in acc:
        s, total = acc[key]
        if s == sign:
            acc[key] = s, total + value
        else:
            acc[key] = 1, total - value if s > 0 else value - total
    else:
        acc[key] = sign, value


def _interleaved(main, *others):
    due = sorted((main[1] * (_LEAD + (1 - _LEAD) * (k + m / len(others)) / n), m, k)
                 for m, (_, n) in enumerate(others) for k in range(n))
    for done, _ in enumerate(main[0]):
        while due and due[0][0] <= done:
            next(others[due.pop(0)[1]][0])
        yield
    for other, _ in others:
        list(other)


def _dot(a, b, axis=0):
    return jax.lax.dot_general(a, b, (((1,), (axis,)), ((), ())),
                               preferred_element_type=jnp.float32)


def _pack(x):
    return pltpu.bitcast(x, jnp.uint32)


def _unpack(words):
    return pltpu.bitcast(words, jnp.bfloat16)


def _cols(n, width=1):
    return slice(n * _T, (n + width) * _T)


def _stack(*parts):
    return jnp.concatenate(parts, axis=0)


def _splice(low, high):
    lane = jax.lax.broadcasted_iota(jnp.int32, low.shape, 1)
    return jnp.where(lane < _T // 2, low, high)


def _layernorm(blocks):
    def mean(terms):
        total = sum(terms[:-1], 0.5 * terms[-1])
        return jnp.sum(total, axis=-1, keepdims=True) * (1 / ((_FULL + 0.5) * _T))

    center = mean(blocks)
    d = [x - center for x in blocks]
    inv = jax.lax.rsqrt(mean([x * x for x in d]) + _EPS)
    return [x * inv for x in d]


def _mixer(halves, dtype=jnp.float32):
    @functools.cache
    def block(half, i):
        x, rest = halves[half][_plain(i)], halves[half][_FULL]
        if i < _FULL:
            return x
        return _splice(x, rest) if (i - _FULL) % 2 else _splice(rest, x)

    return functools.cache(
        lambda rows: _signed_sum([(s, block(half, i)) for s, half, i in rows]).astype(dtype))


def _weights(w_ref):
    w = _unpack(w_ref[...])
    return functools.cache(lambda n: w[:, _cols(n)])


def _widen(mix, n_halves, weights, scheme):
    acc = {}
    for products in _numbered(scheme, n_halves):
        if acc:
            acc = {(t, half): acc[h, half] for t, h in enumerate(scheme.helper)
                   for half in range(n_halves)}
        for n, (rows, _, tiles) in products:
            value = _dot(mix(rows), weights(n))
            for s, half, t in tiles:
                _accumulate(acc, (t, half), s, value)
            yield
    return [[_signed_sum([acc[t, half]]) for half in range(n_halves)]
            for t in range(len(scheme.piece))]


def _narrow(acc, wide, weights, scheme):
    n_halves = len(wide[0])
    wide = wide + [
        [_signed_sum([(1, x[half]) for x, h in zip(wide, scheme.helper) if h == helper])
         for half in range(n_halves)] for helper in range(len(wide), max(scheme.helper) + 1)]
    by_rows = {}
    for n, product in sum(_numbered(scheme, n_halves)[::-1], []):
        by_rows.setdefault(product.rows, []).append((n, product.tiles))
    for rows in sorted(by_rows, key=lambda rows: sorted({-i for _, _, i in rows})):
        total = {}
        for n, tiles in by_rows[rows]:
            sign = max(s for s, _, _ in tiles)
            lhs = _signed_sum([(s * sign, wide[t][half]) for s, half, t in tiles])
            _accumulate(total, rows, sign, _dot(lhs, weights(n)))
            yield
        for s, half, i in rows:
            _accumulate(acc, (half, i), s * total[rows][0], total[rows][1])


def _narrowed(acc, half):
    blocks = [_signed_sum([acc[half, i]]) for i in range(2 * _FULL)]
    folded = list(zip(blocks[_FULL::2], blocks[_FULL + 1::2]))
    rest = _signed_sum([(1, _splice(low, high)) for low, high in folded])
    rest += jnp.concatenate([rest[:, _T // 2:], rest[:, :_T // 2]], axis=1)
    return ([x + _splice(high, low) for x, (low, high) in zip(blocks, folded)]
            + blocks[len(folded):_FULL] + [rest])


def _combine(part, w_ref, scheme, transposed=False):
    donor = {(h, p): t for t, (h, p) in enumerate(zip(scheme.helper, scheme.piece))}
    products = scheme.shared + scheme.main
    uses = {}
    for n in sorted(range(len(products)), key=lambda n: len(products[n].weights) > 1):
        for s, t, i in products[n].weights:
            uses.setdefault((t, i), []).append((s, n))

    def folded(t, p):
        if t >= len(scheme.piece):
            return part(donor[t, p], p)
        if p == scheme.piece[t]:
            return part(t, 2 * _FULL)
        if (scheme.helper[t], p) in donor:
            return (part(t, p).astype(jnp.float32)
                    - folded(scheme.helper[t], p).astype(jnp.float32))
        return part(t, p)

    acc, missing, stored = {}, [len(product.weights) for product in products], []
    for t, i in sorted(uses, key=lambda source: uses[source][0][1]):
        w = _stack(*[folded(t, 2 * _plain(i) + side) for side in range(2)])
        exact = w.astype(jnp.float32)
        for s, n in uses[t, i]:
            _accumulate(acc, n, s, exact if len(products[n].weights) > 1 else w)
            missing[n] -= 1
            if not missing[n]:
                w_ref[:, _cols(n)] = _pack(_signed_sum([acc.pop(n)]).astype(jnp.bfloat16))
                stored.append(w_ref[:, _cols(n)])
    stored = [functools.reduce(jnp.bitwise_or, stored[n:n + 4]) for n in range(0, len(stored), 4)]
    stored = [pltpu.bitcast(words, jnp.float32) for words in stored]
    tokens = [words[r:r + 8] for r in range(0, _T // 2, 8) for words in stored]
    for n in range(len(products) if transposed else 0):
        w_ref[:, _cols(n)] = words = _pack(_unpack(w_ref[:, _cols(n)]).T)
        tokens.append(pltpu.bitcast(words[-8:], jnp.float32))
    return tokens


def _kernel(xt_hbm, mem0_hbm, wq_hbm, wk_hbm, wv_hbm, wot_hbm, w1_hbm, w3_hbm, w2t_hbm,
            outt_hbm, tile_ref, res_ref, norm_ref, early_norm_ref, early_ref, qkv_ref, gate_ref,
            back_ref, gate_rest_ref, down_rest_ref, qkv_stage, gate_stage, back_stage, mem_ref,
            mem0_ref, qkv_sem, gate_sem, back_sem, tile_sem, mem_sem, *, seg):
    d_model, n_tok = xt_hbm.shape
    n_mem = mem0_hbm.shape[0]
    n_seg = n_tok // seg
    n_io = n_tok // _T
    span = n_mem + seg
    score_scale = wq_hbm.shape[2] ** -0.5 * _LOG2E
    n_qkv, n_gate = early_ref.shape[0], gate_ref.shape[0]
    n_wo = n_qkv // 3

    def blocks_at(ref, *index):
        return [ref[(*index, _cols(i))] for i in range(_FULL + 1)]

    def set_blocks(ref, index, blocks):
        for i, x in enumerate(blocks):
            ref[(*index, _cols(i))] = x

    def part_of(i, size):
        return pl.ds(pl.multiple_of(i * size, size), size)

    def step(order, attend=(), feed=(), partner=None, finished=None, filler=None, after=()):
        n_layers = len(attend)
        operand = jnp.bfloat16 if n_layers == 2 else jnp.float32
        qkv, probs, heads, hidden, mixed, fed = {"Q": [], "K": [], "V": []}, [], [], [], {}, {}
        if attend:
            query, key = (jax.lax.broadcasted_iota(jnp.int32, (span, _T), a) for a in (0, 1))
            own_keys = [(key >= n * span) & (key < (n + 1) * span) for n in range(n_layers)]
            visible = (query < n_mem) | (query >= jnp.where(key < span, key, key - span))
            mem = [blocks_at(mem_ref, n, slice(None)) for n in range(n_layers)]
            h = _layernorm(blocks_at(res_ref, part_of(attend[0], seg)))
            if n_layers == 1:
                attend_mix = _mixer([list(map(_stack, mem[0], h))])
            else:
                ahead = _layernorm(
                    [x[:seg - _EARLY] for x in blocks_at(res_ref, part_of(attend[1], seg))])
                cut = seg - _EARLY // 2
                known = part_of(attend[0] % 2 * (sum(_EARLY_ROWS) // _EARLY) + attend[0] // 2,
                                _EARLY // 2)
                attend_mix = _mixer(
                    [[_stack(m, a[:cut]) for m, a in zip(mem[0], h)],
                     [_stack(m, a[cut:], b) for m, a, b in zip(mem[1], h, ahead)]], operand)
        if feed:
            feed_mix = _mixer([blocks_at(norm_ref, n, slice(None)) for n in range(2)])

        def project(stage, n):
            tiles = yield from _widen(attend_mix, n_layers, _weights(qkv_ref.at[n]), _WHOLE)
            if n_layers == 1:
                qkv[stage] += [halves[0] for halves in tiles]
                return
            moved = n_mem + _EARLY // 2
            early = _unpack(early_ref[n, known, :]).astype(jnp.float32)
            for t, (a, b) in enumerate(tiles):
                x = _stack(a, b[n_mem:moved], b[:n_mem], b[moved:], early[:, _cols(t)])
                if stage == "V":
                    x = _stack(x, jnp.zeros((_T - 2 * span, _T), x.dtype))
                qkv[stage].append(x if stage == "Q" else x.astype(operand))

        def score(count):
            for t in range(len(probs), len(probs) + count):
                s = _dot(qkv["Q"][t], qkv["K"][t], axis=1)
                if n_layers == 2:
                    s = jnp.where(own_keys[1][:, :2 * span], s[span:], s[:span])
                s = jnp.concatenate(
                    [s * score_scale, jnp.zeros((span, _T - s.shape[1]), s.dtype)], axis=1)
                s = jnp.where(visible, s, _MASKED * _LOG2E)
                top = [jnp.max(jnp.where(own, s, -jnp.inf), axis=-1, keepdims=True)
                       for own in own_keys]
                p = jnp.exp2(s - jnp.where(own_keys[-1], top[-1], top[0]))
                p = _stack(*[jnp.where(own, p, 0.0) for own in own_keys])
                probs.append((p.astype(operand), pltpu.reciprocal(
                    jnp.sum(p, axis=-1, keepdims=True), approx=True)))
                yield

        def average(count):
            for t in range(len(heads), len(heads) + count):
                (p, inv), v = probs[t], qkv["V"][t]
                both = _dot(p[:, :v.shape[0]], v) * inv
                heads.append([both[n * span:(n + 1) * span] for n in range(n_layers)])
                yield

        def add_attended():
            x = [] if partner is None else [blocks_at(res_ref, part_of(partner, seg))]
            before = [blocks_at(res_ref, part_of(s, seg)) for s in attend]
            for n, s in enumerate(attend):
                out = _narrowed(mixed, n)
                x.append([a + o[n_mem:] for a, o in zip(before[n], out)])
                set_blocks(res_ref, [part_of(s, seg)], x[-1])
                set_blocks(mem_ref, [n, slice(None)], [o[:n_mem] for o in out])
            for n, blocks in enumerate(x):
                set_blocks(norm_ref, [n, slice(None)], _layernorm(blocks))
                yield

        def gated(w_ref, scheme):
            tiles = yield from _widen(feed_mix, 2, _weights(w_ref), scheme)
            for pair in zip(tiles[::2], tiles[1::2]):
                halved = [(0.5 * gate, up) for gate, up in zip(*pair)]
                hidden.append([(g * jnp.tanh(g) + g) * up for g, up in halved])

        def add_fed():
            before = [blocks_at(res_ref, part_of(s, seg)) for s in feed]
            for n, s in enumerate(feed):
                set_blocks(res_ref, [part_of(s, seg)],
                           [a + o for a, o in zip(before[n], _narrowed(fed, n))])
            yield

        def begin(name):
            stage, number = name[0], int(name[1:])
            if stage in "SA":
                return (score if stage == "S" else average)(number), number
            if stage in "NF":
                return (add_attended if stage == "N" else add_fed)(), 1
            if stage == "T":
                return transpose_out(finished), _FULL + 1
            if stage == "X":
                return filler, _count(_WHOLE)
            if stage in "QKV":
                return project(stage, 3 * number + "QKV".index(stage)), _count(_WHOLE, n_layers)
            if stage == "G":
                unit = ((gate_ref.at[number], _WHOLE) if number < n_gate
                        else (gate_rest_ref, _GATE_REST))
                return gated(*unit), _count(unit[1])
            acc, wide, n = (mixed, heads, number) if stage == "O" else (fed, hidden, n_wo + number)
            w_ref, scheme = (back_ref.at[n], _WHOLE) if n < n_gate else (down_rest_ref, _DOWN_REST)
            wide = wide[number * _UNIT:(number + 1) * _UNIT]
            return _narrow(acc, wide, _weights(w_ref), scheme), _count(scheme, len(wide[0]))

        due = sorted((n, stage) for stage in after for n in after[stage])
        passes = itertools.chain.from_iterable(
            _interleaved(*map(begin, names.split("+"))) for names in order.split())
        for done, _ in enumerate(passes):
            while due and due[0][0] <= done:
                next(begin(due.pop(0)[1] + "1")[0])

    def start_when(condition, copies):
        @pl.when(condition)
        def _():
            for copy in copies():
                copy.start()

    def await_whole(ref, sem):
        pltpu.make_async_copy(ref, ref, sem).wait()

    def request_qkv(n, pairs=range(_UNIT // 2)):
        for which, w in enumerate((wq_hbm, wk_hbm, wv_hbm)):
            start_when((n < n_qkv) & (n % 3 == which), lambda w=w: [
                pltpu.make_async_copy(w.bitcast(jnp.uint32).at[:, n // 3 * (_UNIT // 2) + p, :],
                                      qkv_stage.at[n % 2, p], qkv_sem.at[n % 2]) for p in pairs])

    def column_copy(w_hbm, first, count, stage, sem, offset=0):
        cols = pl.ds(pl.multiple_of(first * _T, _T), count * _T)
        return pltpu.make_async_copy(w_hbm.bitcast(jnp.uint32).at[:, cols],
                                     stage.at[:, _cols(offset, count)], sem)

    def gate_copies(n, scheme):
        return [column_copy(w, n * (_UNIT // 2), len(scheme.piece) // 2, gate_stage.at[n % 2],
                            gate_sem.at[n % 2], side * _UNIT // 2)
                for side, w in enumerate((w1_hbm, w3_hbm))]

    def down_copies(n, scheme):
        return [column_copy(w2t_hbm, (n - n_wo) * _UNIT, len(scheme.piece), back_stage.at[n % 2],
                            back_sem.at[n % 2])]

    def rest_copies():
        return gate_copies(n_gate, _GATE_REST) + down_copies(n_gate, _DOWN_REST)

    def request_others(n):
        start_when(n < n_wo, lambda: [
            pltpu.make_async_copy(wot_hbm.bitcast(jnp.uint32).at[n * _UNIT + t],
                                  back_stage.at[n % 2, :, _cols(t)], back_sem.at[n % 2])
            for t in range(_UNIT)])
        start_when((n >= n_wo) & (n < n_gate), lambda: down_copies(n, _WHOLE))
        start_when(n < n_gate, lambda: gate_copies(n, _WHOLE))
        start_when(n == n_gate, rest_copies)

    def combine_qkv(n, w_ref):
        stage = qkv_stage.at[n % 2]

        def part(t, p):
            words = stage[t // 2, pl.ds(p * _T // 2, _T // 2), :]
            words = words & jnp.uint32(0xFFFF0000) if t % 2 else words << 16
            return pltpu.bitcast(words, jnp.float32)

        return _combine(part, w_ref, _WHOLE)

    def combine_others(n, gate, back):
        gates, backs = gate_stage.at[n % 2], back_stage.at[n % 2]

        def part(stage, column, p):
            return _unpack(stage[pl.ds(p * _T // 4, _T // 4), _cols(column)])

        return (_combine(functools.partial(part, backs), *back, transposed=True)
                + _combine(lambda t, p: part(gates, t % 2 * _UNIT // 2 + t // 2, p), *gate))

    def x_copy(i):
        return pltpu.make_async_copy(xt_hbm.at[:, part_of(i, _T)], tile_ref.at[i], tile_sem.at[i])

    def out_copy(i):
        return pltpu.make_async_copy(tile_ref.at[i], outt_hbm.at[:, _cols(i)], tile_sem.at[i])

    def transpose_in(i):
        x = tile_ref[i].astype(jnp.float32)
        x = _stack(x, x[_FULL * _T:])
        blocks = [x[b * _T:(b + 1) * _T].T for b in range(_FULL + 1)]
        set_blocks(res_ref, [part_of(i, _T)], blocks)
        normed = _layernorm(
            [_stack(*[x[s - _EARLY:s] for s in range(seg, _T + 1, seg)]) for x in blocks])
        for s in range(_T // seg):
            rows = part_of(i * (_T // seg // 2) + s // 2, _EARLY)
            set_blocks(early_norm_ref, [s % 2, rows],
                       [x[s * _EARLY:(s + 1) * _EARLY] for x in normed])

    def transpose_out(i):
        for b, x in enumerate(blocks_at(res_ref, part_of(i, _T))):
            depth = min(_T, d_model - b * _T)
            tile_ref[i, pl.ds(b * _T, depth), :] = x.T[:depth].astype(tile_ref.dtype)
            yield

    def early_pass(n, weights, first, count, paced=lambda x: x):
        rows = pl.ds(pl.multiple_of(first + _LAG // 2 * _EARLY, _EARLY), count)
        mix = _mixer([blocks_at(early_norm_ref, half, rows) for half in range(2)])
        tiles = yield from _widen(lambda key: paced(mix(key)), 2, weights, _WHOLE)
        for half in range(2):
            at = pl.multiple_of((half * sum(_EARLY_ROWS) + first) // 2, _EARLY // 2)
            early_ref.at[n][pl.ds(at, count // 2), :] = _pack(jnp.concatenate(
                [halves[half] for halves in tiles], axis=1).astype(jnp.bfloat16))

    def early_passes(n, w_ref, chunks, tokens=()):
        total = sum(_EARLY_ROWS[c] for c in chunks) * _count(_WHOLE)
        due = [(total * (k + 1) // (len(tokens) + 1), token) for k, token in enumerate(tokens)]
        done = 0

        def paced(x):
            nonlocal done
            done += x.shape[0]
            while due and due[0][0] <= done:
                x = _stack(x[:-8], jnp.where(always, x[-8:], due.pop(0)[1]))
            return x

        weights = _weights(w_ref)
        for c in chunks:
            list(early_pass(n, weights, sum(_EARLY_ROWS[:c]), _EARLY_ROWS[c], paced))

    def double_step(b):
        step(_ORDER, attend=[b, b + _LAG], feed=[b - 1, b + _LAG - 1], after=_AFTER,
             finished=jnp.maximum(b - 1 - _T // seg, 0) * seg // _T)

    mem_copy = pltpu.make_async_copy(mem0_hbm, mem0_ref.at[0], mem_sem)
    for copy in [mem_copy] + [x_copy(i) for i in range(_FIRST_TILES)]:
        copy.start()
    request_qkv(0, range(_UNIT // 4))
    mem_copy.wait()
    request_qkv(0, range(_UNIT // 4, _UNIT // 2))

    def load_tile(i, _):
        x_copy(i).wait()
        transpose_in(i)
        return i

    always = jax.lax.fori_loop(0, _FIRST_TILES, load_tile, 0) > 0
    mem0 = mem0_ref[0].astype(jnp.float32)
    mem_ref[0] = mem_ref[1] = jnp.concatenate([mem0, mem0[:, _FULL * _T:]], axis=1)
    for i in range(_FIRST_TILES, n_io):
        x_copy(i).start()

    chunks = range(len(_EARLY_ROWS))
    await_whole(qkv_stage.at[0], qkv_sem.at[0])
    request_qkv(1)
    combine_qkv(0, qkv_ref.at[0])
    early_passes(0, qkv_ref.at[0], chunks[:_TILES_ARRIVE])
    for i in range(_FIRST_TILES, n_io):
        x_copy(i).wait()
    request_qkv(2)
    for i in range(_FIRST_TILES, n_io):
        transpose_in(i)
    early_passes(0, qkv_ref.at[0], chunks[_TILES_ARRIVE:_UNIT_ARRIVES])
    await_whole(qkv_stage.at[1], qkv_sem.at[1])
    request_others(0)
    early_passes(0, qkv_ref.at[0], chunks[_UNIT_ARRIVES:], combine_qkv(1, qkv_ref.at[1]))

    @pl.loop(1, n_qkv - 1)
    def _load_units(n):
        both = qkv_ref.at[pl.ds(n, 2)]
        request_qkv(n + 2)
        await_whole(qkv_stage.at[(n + 1) % 2], qkv_sem.at[(n + 1) % 2])
        early_passes(n, both.at[0], chunks[:3], combine_qkv(n + 1, both.at[1]))
        request_others(n)
        await_whole(gate_stage.at[(n - 1) % 2], gate_sem.at[(n - 1) % 2])
        await_whole(back_stage.at[(n - 1) % 2], back_sem.at[(n - 1) % 2])
        early_passes(n, both.at[0], chunks[3:], combine_others(
            n - 1, (gate_ref.at[n - 1], _WHOLE), (back_ref.at[n - 1], _WHOLE)))

    def filler(first, count):
        return early_pass(n_qkv - 1, _weights(qkv_ref.at[n_qkv - 1]), first, count)

    for copy in rest_copies():
        copy.wait()
    early_passes(n_qkv - 1, qkv_ref.at[n_qkv - 1], chunks[:-_LAG - 2], combine_others(
        n_gate, (gate_rest_ref, _GATE_REST), (down_rest_ref, _DOWN_REST)))

    @pl.loop(0, _LAG, unroll=True)
    def _first_steps(s):
        step(_ORDER_HEAD, attend=[s], partner=0,
             filler=filler((chunks[-_LAG - 2] + s) * _EARLY_ROWS[0], _EARLY_ROWS[0]))

    step(_ORDER_FFN + " X0", feed=[0, 1], filler=filler(sum(_EARLY_ROWS[:-2]), _EARLY_ROWS[-2]))
    mem_ref[0], mem_ref[1] = mem_ref[1], mem_ref[0]
    step(_ORDER_HEAD, attend=[0, _LAG], filler=filler(sum(_EARLY_ROWS[:-1]), _EARLY_ROWS[-1]))
    pl.loop(1, n_seg - _LAG)(double_step)
    for i in range(n_io - 1):
        out_copy(i).start()
    step(_ORDER_TAIL, attend=[n_seg - 2], feed=[n_seg - 3, n_seg - 1])
    step(_ORDER_LAST, attend=[n_seg - 1], partner=n_seg - 2)
    step(_ORDER_FFN + " T0", feed=[n_seg - 2, n_seg - 1], finished=n_io - 1)
    out_copy(n_io - 1).start()
    for i in range(n_io):
        out_copy(i).wait()


@functools.partial(jax.jit, static_argnames=("A_seg_len",))
def pallas_interleave_layers__memory_aug_recurrent_mem_tr__glu_gated_swiglu__prompt_kernel(
    A_x: jax.Array,
    A_mem0: jax.Array,
    A_Wq: jax.Array,
    A_Wk: jax.Array,
    A_Wv: jax.Array,
    A_Wo: jax.Array,
    A_seg_len: int,
    B_x: jax.Array,
    B_w1: jax.Array,
    B_w3: jax.Array,
    B_w2: jax.Array,
):
    del B_x
    _, n_tok, d_model = A_x.shape
    n_mem = A_mem0.shape[1]
    assert A_x.shape == (1, 2048, 576) and A_seg_len == 32 and n_mem == 8
    assert A_Wq.shape[1:] == (2 * _UNIT, _T) and B_w1.shape[1] == 36 * _T
    width = (_FULL + 1) * _T
    hbm = pl.BlockSpec(memory_space=pltpu.HBM)

    def weights(scheme, *units):
        return pltpu.VMEM((*units, _T // 2, _count(scheme) * _T), jnp.uint32)

    out_t = pl.pallas_call(
        functools.partial(_kernel, seg=A_seg_len),
        out_shape=jax.ShapeDtypeStruct((d_model, n_tok), A_x.dtype),
        in_specs=[hbm] * 9,
        out_specs=hbm,
        scratch_shapes=[
            pltpu.VMEM((n_tok // _T, d_model, _T), A_x.dtype),
            pltpu.VMEM((n_tok, width), jnp.float32),
            pltpu.VMEM((2, A_seg_len, width), jnp.float32),
            pltpu.VMEM((2, n_tok // A_seg_len * _EARLY // 2, width), jnp.float32),
            pltpu.VMEM((6, sum(_EARLY_ROWS), _UNIT * _T), jnp.uint32),
            weights(_WHOLE, 6), weights(_WHOLE, 4), weights(_WHOLE, 4),
            weights(_GATE_REST), weights(_DOWN_REST),
            pltpu.VMEM((2, _UNIT // 2, d_model, _T), jnp.uint32),
            pltpu.VMEM((2, d_model // 2, _UNIT * _T), jnp.uint32),
            pltpu.VMEM((2, d_model // 2, _UNIT * _T), jnp.uint32),
            pltpu.VMEM((2, n_mem, width), jnp.float32),
            pltpu.VMEM((8, n_mem, d_model), A_mem0.dtype),
            pltpu.SemaphoreType.DMA((2,)),
            pltpu.SemaphoreType.DMA((2,)),
            pltpu.SemaphoreType.DMA((2,)),
            pltpu.SemaphoreType.DMA((n_tok // _T,)),
            pltpu.SemaphoreType.DMA,
        ],
        compiler_params=pltpu.CompilerParams(vmem_limit_bytes=116 * 1024 * 1024,
                                             disable_bounds_checks=True),
    )(A_x.reshape(n_tok, d_model).T, A_mem0.reshape(n_mem, d_model), A_Wq, A_Wk, A_Wv,
      A_Wo.transpose(0, 2, 1), B_w1, B_w3, B_w2.T)
    return out_t.T.reshape(A_x.shape)
```

```python
import functools
import itertools
import math
from typing import NamedTuple

import jax
import jax.numpy as jnp
import jax.experimental.pallas as pl
import jax.experimental.pallas.tpu as pltpu

_EPS = 1e-05
_MASKED = -1000000000.0
_LOG2E = math.log2(math.e)
_T = 128
_FULL = 4
_UNIT = 16
_LAG = 2
_EARLY = 16
_EARLY_ROWS = (48,) * 9 + (32,) * 2
_FIRST_TILES = 5
_TILES_ARRIVE = 2
_UNIT_ARRIVES = 7
_ORDER = "G0 K0 Q0 K1 V0 Q1+T0 U0 V1 O0 G1 O1 U1+N0 G2 U2 D0 D1 D2 F0"
_AFTER = {
    "S": (366, 394, 402, 419, 437, 455, 484, 537, 598, 620, 638, 655, 673, 691, 720, 730,
          740, 749, 759, 769, 778, 788, 798, 807, 817, 838, 853, 869, 884, 899, 914, 929),
    "A": (729, 747, 765, 782, 800, 818, 840, 854, 865, 875, 886, 897, 907, 918, 929, 939,
          955, 963, 970, 978, 985, 1013, 1019, 1019, 1025, 1033, 1034, 1037, 1041, 1047, 1054, 1074)}
_ORDER_HEAD = "Q0 K0 Q1+S8 K1+S8 V0+S16 V1+A16 O0+A16 O1 X0+N0"
_ORDER_TAIL = "G0 U0 G1 U1 G2 U2 Q0 K0 Q1+S8 K1+S8 V0+S8 V1+S8+A16 D0 D1 D2 F0 O0+A16 O1 N0"
_ORDER_LAST = "Q0 K0 Q1+S8 K1+S8 V0+S16 V1+A16 O0+A16 O1 N0"
_ORDER_FFN = "G0 U0 G1 U1 G2 U2 D0 D1 D2 F0"
_LEAD = 0.1


class _Product(NamedTuple):
    rows: tuple
    weights: tuple
    tiles: tuple


class _Scheme(NamedTuple):
    piece: tuple
    helper: tuple
    shared: tuple
    main: tuple


def _pair_up(blocks, left, right, edges):
    products = []
    edges = [(u, blocks[u][i], v, blocks[v][j]) for u, i, v, j in edges]
    assert all(i in blocks[v] and j in blocks[u] for u, i, v, j in edges)

    def add(rows, weights, tiles):
        rows = tuple(sorted(rows, key=lambda term: term[1:]))
        if rows[0][0] < 0:
            rows = tuple((-s, half, i) for s, half, i in rows)
            tiles = tuple((-s, half, t) for s, half, t in tiles)
        products.append(_Product(rows, tuple(weights), tuple(tiles)))

    def unpaired_blocks(t, half):
        mine = [((i, v, j), (j, u, i))[half] for u, i, v, j in edges if (u, v)[half] == t]
        for i in blocks[t]:
            if any(i == j for _, _, j in mine):
                continue
            partners = [(p, j) for own, p, j in mine if own == i]
            if not partners:
                add([(1, 0, i)], [(1, t, i)], [(1, 0, t)])
                add([(1, 1, i)], [(1, t, i)], [(1, 1, t)])
                continue
            add([(1, half, i)], [(1, t, i)] + [(1, t, j) for _, j in partners],
                [(1, half, t), (-1, 1 - half, t)])
            add([(1, 0, i), (1, 1, i)], [(1, t, i)] + [(-1, p, i) for p, _ in partners],
                [(1, 1 - half, t)])

    for t in left:
        unpaired_blocks(t, 0)
        for u, i, v, j in edges:
            if u == t:
                add([(1, 1, i), (-1, 1, j)], [(1, v, i)], [(1, 1, v), (1, 1, u)])
                add([(1, 0, j), (-1, 0, i)], [(1, u, j)], [(1, 0, u), (1, 0, v)])
                add([(1, 0, i), (1, 1, j)], [(1, u, j), (1, v, i)], [(1, 1, u), (1, 0, v)])
    for t in right:
        unpaired_blocks(t, 1)
    return products


def _scheme(n):
    if n == 4:
        piece = [0, 0, 1, 1]
        groups = [([u], [u + 1], [(u, 0, u + 1, 2), (u, 1, u + 1, 3)]) for u in (0, 2)]
    else:
        piece = [2 * (t // 8) + ((t % 4 == t // 8) == (t % 8 >= 4)) for t in range(n)]
        groups = [(range(g, g + 4), range(g + 4, g + 8),
                   [(g + i, i, g + 4 + j, j) for i in range(4) for j in range(4) if i != j])
                  for g in range(0, n, 8)]
    helper = [n + piece[:t].count(piece[t]) for t in range(n)]
    helpers = range(n, max(helper) + 1)
    blocks = [[_FULL + p if i == p // 2 else i for i in range(_FULL)] for p in piece]
    blocks += [range(max(piece) // 2 + 1)] * len(helpers)
    shared = [p for u in helpers[::2] for p in _pair_up(
        blocks, [u], [u + 1], [(u, 0, u + 1, 1)] if len(blocks[u]) == 2 else [])]
    return _Scheme(tuple(piece), tuple(helper), tuple(shared),
                   tuple(p for group in groups for p in _pair_up(blocks, *group)))


_WHOLE, _REST = _scheme(_UNIT), _scheme(4)


def _numbered(scheme, n_halves):
    kept = [], []
    for n, (rows, weights, tiles) in enumerate(scheme.shared + scheme.main):
        rows = tuple(term for term in rows if term[1] < n_halves)
        tiles = tuple(term for term in tiles if term[1] < n_halves)
        if rows and tiles:
            kept[n >= len(scheme.shared)].append((n, _Product(rows, weights, tiles)))
    return kept


def _count(scheme, n_halves=2):
    return sum(map(len, _numbered(scheme, n_halves)))


def _plain(block):
    return block if block < _FULL else (block - _FULL) // 2


def _signed_sum(terms):
    (sign, total), *rest = sorted(terms, key=lambda term: -term[0])
    for s, value in rest:
        total = total + value if s == sign else total - value
    return total if sign > 0 else -total


def _accumulate(acc, key, sign, value):
    if key in acc:
        s, total = acc[key]
        if s == sign:
            acc[key] = s, total + value
        else:
            acc[key] = 1, total - value if s > 0 else value - total
    else:
        acc[key] = sign, value


def _interleaved(main, *others):
    due = sorted((main[1] * (_LEAD + (1 - _LEAD) * (k + m / len(others)) / n), m, k)
                 for m, (_, n) in enumerate(others) for k in range(n))
    for done, _ in enumerate(main[0]):
        while due and due[0][0] <= done:
            next(others[due.pop(0)[1]][0])
        yield
    for other, _ in others:
        list(other)


def _dot(a, b, axis=0):
    return jax.lax.dot_general(a, b, (((1,), (axis,)), ((), ())),
                               preferred_element_type=jnp.float32)


def _pack(x):
    return pltpu.bitcast(x, jnp.uint32)


def _unpack(words):
    return pltpu.bitcast(words, jnp.bfloat16)


def _cols(n, width=1):
    return slice(n * _T, (n + width) * _T)


def _stack(*parts):
    return jnp.concatenate(parts, axis=0)


def _splice(low, high):
    lane = jax.lax.broadcasted_iota(jnp.int32, low.shape, 1)
    return jnp.where(lane < _T // 2, low, high)


def _inverse(x):
    r = pltpu.reciprocal(x, approx=True)
    return r * (2.0 - x * r)


def _layernorm(blocks):
    def mean(terms):
        total = sum(terms[:-1], 0.5 * terms[-1])
        return jnp.sum(total, axis=-1, keepdims=True) * (1 / ((_FULL + 0.5) * _T))

    center = mean(blocks)
    d = [x - center for x in blocks]
    inv = jax.lax.rsqrt(mean([x * x for x in d]) + _EPS)
    return [x * inv for x in d]


def _mixer(halves, dtype=jnp.float32):
    @functools.cache
    def block(half, i):
        x, rest = halves[half][_plain(i)], halves[half][_FULL]
        if i < _FULL:
            return x
        return _splice(x, rest) if (i - _FULL) % 2 else _splice(rest, x)

    return functools.cache(
        lambda rows: _signed_sum([(s, block(half, i)) for s, half, i in rows]).astype(dtype))


def _weights(w_ref):
    w = _unpack(w_ref[...])
    return functools.cache(lambda n: w[:, _cols(n)])


def _widen(mix, n_halves, weights, scheme):
    acc = {}
    for products in _numbered(scheme, n_halves):
        if acc:
            acc = {(t, half): acc[h, half] for t, h in enumerate(scheme.helper)
                   for half in range(n_halves)}
        for n, (rows, _, tiles) in products:
            value = _dot(mix(rows), weights(n))
            for s, half, t in tiles:
                _accumulate(acc, (t, half), s, value)
            yield
    return [[_signed_sum([acc[t, half]]) for half in range(n_halves)]
            for t in range(len(scheme.piece))]


def _narrow(acc, wide, weights, scheme):
    n_halves = len(wide[0])
    wide = wide + [
        [_signed_sum([(1, x[half]) for x, h in zip(wide, scheme.helper) if h == helper])
         for half in range(n_halves)] for helper in range(len(wide), max(scheme.helper) + 1)]
    by_rows = {}
    for n, product in sum(_numbered(scheme, n_halves)[::-1], []):
        by_rows.setdefault(product.rows, []).append((n, product.tiles))
    for rows in sorted(by_rows, key=lambda rows: sorted({-i for _, _, i in rows})):
        total = {}
        for n, tiles in by_rows[rows]:
            sign = max(s for s, _, _ in tiles)
            lhs = _signed_sum([(s * sign, wide[t][half]) for s, half, t in tiles])
            _accumulate(total, rows, sign, _dot(lhs, weights(n)))
            yield
        for s, half, i in rows:
            _accumulate(acc, (half, i), s * total[rows][0], total[rows][1])


def _narrowed(acc, half):
    blocks = [_signed_sum([acc[half, i]]) for i in range(2 * _FULL)]
    folded = list(zip(blocks[_FULL::2], blocks[_FULL + 1::2]))
    rest = _signed_sum([(1, _splice(low, high)) for low, high in folded])
    rest += jnp.concatenate([rest[:, _T // 2:], rest[:, :_T // 2]], axis=1)
    return ([x + _splice(high, low) for x, (low, high) in zip(blocks, folded)]
            + blocks[len(folded):_FULL] + [rest])


def _combine(part, w_ref, scheme, transposed=False):
    donor = {(h, p): t for t, (h, p) in enumerate(zip(scheme.helper, scheme.piece))}
    products = scheme.shared + scheme.main
    uses = {}
    for n in sorted(range(len(products)), key=lambda n: len(products[n].weights) > 1):
        for s, t, i in products[n].weights:
            uses.setdefault((t, i), []).append((s, n))

    def folded(t, p):
        if t >= len(scheme.piece):
            return part(donor[t, p], p)
        if p == scheme.piece[t]:
            return part(t, 2 * _FULL)
        if (scheme.helper[t], p) in donor:
            return (part(t, p).astype(jnp.float32)
                    - folded(scheme.helper[t], p).astype(jnp.float32))
        return part(t, p)

    acc, missing, stored = {}, [len(product.weights) for product in products], []
    for t, i in sorted(uses, key=lambda source: uses[source][0][1]):
        w = _stack(*[folded(t, 2 * _plain(i) + side) for side in range(2)])
        exact = w.astype(jnp.float32)
        for s, n in uses[t, i]:
            _accumulate(acc, n, s, exact if len(products[n].weights) > 1 else w)
            missing[n] -= 1
            if not missing[n]:
                w_ref[:, _cols(n)] = _pack(_signed_sum([acc.pop(n)]).astype(jnp.bfloat16))
                stored.append(w_ref[:, _cols(n)])
    stored = [functools.reduce(jnp.bitwise_or, stored[n:n + 4]) for n in range(0, len(stored), 4)]
    stored = [pltpu.bitcast(words, jnp.float32) for words in stored]
    tokens = [words[r:r + 8] for r in range(0, _T // 2, 8) for words in stored]
    for n in range(len(products) if transposed else 0):
        w_ref[:, _cols(n)] = words = _pack(_unpack(w_ref[:, _cols(n)]).T)
        tokens.append(pltpu.bitcast(words[-8:], jnp.float32))
    return tokens


def _kernel(xt_hbm, mem0_hbm, wq_hbm, wk_hbm, wv_hbm, wot_hbm, w1_hbm, w3_hbm, w2t_hbm,
            outt_hbm, tile_ref, res_ref, norm_ref, early_norm_ref, early_ref, qkv_ref, gate_ref,
            back_ref, rest_ref, qkv_stage, gate_stage, back_stage, mem_ref,
            mem0_ref, qkv_sem, gate_sem, back_sem, tile_sem, mem_sem, *, seg):
    d_model, n_tok = xt_hbm.shape
    n_mem = mem0_hbm.shape[0]
    n_seg = n_tok // seg
    n_io = n_tok // _T
    span = n_mem + seg
    score_scale = wq_hbm.shape[2] ** -0.5 * _LOG2E
    n_qkv, n_gate = early_ref.shape[0], gate_ref.shape[0]
    n_wo = n_qkv // 3

    def blocks_at(ref, *index):
        return [ref[(*index, _cols(i))] for i in range(_FULL + 1)]

    def set_blocks(ref, index, blocks):
        for i, x in enumerate(blocks):
            ref[(*index, _cols(i))] = x

    def part_of(i, size):
        return pl.ds(pl.multiple_of(i * size, size), size)

    def step(order, attend=(), feed=(), partner=None, finished=None, filler=None, after=()):
        n_layers = len(attend)
        operand = jnp.bfloat16 if n_layers == 2 else jnp.float32
        qkv, probs, heads, mixed = {"Q": [], "K": [], "V": []}, [], [], {}
        gates, hidden, fed = [], [], {}
        if attend:
            query, key = (jax.lax.broadcasted_iota(jnp.int32, (span, _T), a) for a in (0, 1))
            own_keys = [(key >= n * span) & (key < (n + 1) * span) for n in range(n_layers)]
            visible = (query < n_mem) | (query >= jnp.where(key < span, key, key - span))
            mem = [blocks_at(mem_ref, n, slice(None)) for n in range(n_layers)]
            h = _layernorm(blocks_at(res_ref, part_of(attend[0], seg)))
            if n_layers == 1:
                attend_mix = _mixer([list(map(_stack, mem[0], h))])
            else:
                ahead = _layernorm(
                    [x[:seg - _EARLY] for x in blocks_at(res_ref, part_of(attend[1], seg))])
                cut = seg - _EARLY // 2
                known = part_of(attend[0] % 2 * (sum(_EARLY_ROWS) // _EARLY) + attend[0] // 2,
                                _EARLY // 2)
                attend_mix = _mixer(
                    [[_stack(m, a[:cut]) for m, a in zip(mem[0], h)],
                     [_stack(m, a[cut:], b) for m, a, b in zip(mem[1], h, ahead)]], operand)
        if feed:
            feed_mix = _mixer([blocks_at(norm_ref, n, slice(None)) for n in range(2)])

        def project(stage, n):
            tiles = yield from _widen(attend_mix, n_layers, _weights(qkv_ref.at[n]), _WHOLE)
            if n_layers == 1:
                qkv[stage] += [halves[0] for halves in tiles]
                return
            moved = n_mem + _EARLY // 2
            early = _unpack(early_ref[n, known, :]).astype(jnp.float32)
            for t, (a, b) in enumerate(tiles):
                x = _stack(a, b[n_mem:moved], b[:n_mem], b[moved:], early[:, _cols(t)])
                if stage == "V":
                    x = _stack(x, jnp.zeros((_T - 2 * span, _T), x.dtype))
                qkv[stage].append(x if stage == "Q" else x.astype(operand))

        def score(count):
            for t in range(len(probs), len(probs) + count):
                s = _dot(qkv["Q"][t], qkv["K"][t], axis=1)
                if n_layers == 2:
                    s = jnp.where(own_keys[1][:, :2 * span], s[span:], s[:span])
                s = jnp.concatenate(
                    [s * score_scale, jnp.zeros((span, _T - s.shape[1]), s.dtype)], axis=1)
                s = jnp.where(visible, s, _MASKED * _LOG2E)
                top = [jnp.max(jnp.where(own, s, -jnp.inf), axis=-1, keepdims=True)
                       for own in own_keys]
                p = jnp.exp2(s - jnp.where(own_keys[-1], top[-1], top[0]))
                p = _stack(*[jnp.where(own, p, 0.0) for own in own_keys])
                probs.append((p.astype(operand), _inverse(jnp.sum(p, axis=-1, keepdims=True))))
                yield

        def average(count):
            for t in range(len(heads), len(heads) + count):
                (p, inv), v = probs[t], qkv["V"][t]
                both = _dot(p[:, :v.shape[0]], v) * inv
                heads.append([both[n * span:(n + 1) * span] for n in range(n_layers)])
                yield

        def add_attended():
            x = [] if partner is None else [blocks_at(res_ref, part_of(partner, seg))]
            before = [blocks_at(res_ref, part_of(s, seg)) for s in attend]
            for n, s in enumerate(attend):
                out = _narrowed(mixed, n)
                x.append([a + o[n_mem:] for a, o in zip(before[n], out)])
                set_blocks(res_ref, [part_of(s, seg)], x[-1])
                set_blocks(mem_ref, [n, slice(None)], [o[:n_mem] for o in out])
            for n, blocks in enumerate(x):
                set_blocks(norm_ref, [n, slice(None)], _layernorm(blocks))
                yield

        def gate(w_ref, scheme):
            for halves in (yield from _widen(feed_mix, 2, _weights(w_ref), scheme)):
                gates.append([g * jnp.tanh(g) + g for g in [0.5 * x for x in halves]])

        def up(w_ref, scheme):
            for halves in (yield from _widen(feed_mix, 2, _weights(w_ref), scheme)):
                hidden.append([g * x for g, x in zip(gates[len(hidden)], halves)])

        def add_fed():
            before = [blocks_at(res_ref, part_of(s, seg)) for s in feed]
            for n, s in enumerate(feed):
                set_blocks(res_ref, [part_of(s, seg)],
                           [a + o for a, o in zip(before[n], _narrowed(fed, n))])
            yield

        def begin(name):
            stage, number = name[0], int(name[1:])
            if stage in "SA":
                return (score if stage == "S" else average)(number), number
            if stage in "NF":
                return (add_attended if stage == "N" else add_fed)(), 1
            if stage == "T":
                return transpose_out(finished), _FULL + 1
            if stage == "X":
                return filler, _count(_WHOLE)
            if stage in "QKV":
                return project(stage, 3 * number + "QKV".index(stage)), _count(_WHOLE, n_layers)
            ref, n = {"G": (gate_ref, 2 * number), "U": (gate_ref, 2 * number + 1),
                      "O": (back_ref, number), "D": (back_ref, n_wo + number)}[stage]
            w_ref, scheme = ((ref.at[n], _WHOLE) if n < n_gate
                             else (rest_ref.at["GUD".index(stage)], _REST))
            if stage in "GU":
                return (gate if stage == "G" else up)(w_ref, scheme), _count(scheme)
            acc, wide = (mixed, heads) if stage == "O" else (fed, hidden)
            wide = wide[number * _UNIT:(number + 1) * _UNIT]
            return _narrow(acc, wide, _weights(w_ref), scheme), _count(scheme, len(wide[0]))

        due = sorted((n, stage) for stage in after for n in after[stage])
        passes = itertools.chain.from_iterable(
            _interleaved(*map(begin, names.split("+"))) for names in order.split())
        for done, _ in enumerate(passes):
            while due and due[0][0] <= done:
                next(begin(due.pop(0)[1] + "1")[0])

    def start_when(condition, copies):
        @pl.when(condition)
        def _():
            for copy in copies():
                copy.start()

    def await_whole(ref, sem):
        pltpu.make_async_copy(ref, ref, sem).wait()

    def request_qkv(n, pairs=range(_UNIT // 2)):
        for which, w in enumerate((wq_hbm, wk_hbm, wv_hbm)):
            start_when((n < n_qkv) & (n % 3 == which), lambda w=w: [
                pltpu.make_async_copy(w.bitcast(jnp.uint32).at[:, n // 3 * (_UNIT // 2) + p, :],
                                      qkv_stage.at[n % 2, p], qkv_sem.at[n % 2]) for p in pairs])

    def request_others(n):
        def columns(w_hbm, unit, stage, sem):
            return [pltpu.make_async_copy(
                w_hbm.bitcast(jnp.uint32).at[:, part_of(unit, _UNIT * _T)],
                stage.at[n % 2], sem.at[n % 2])]

        start_when(n < n_wo, lambda: [
            pltpu.make_async_copy(wot_hbm.bitcast(jnp.uint32).at[n * _UNIT + t],
                                  back_stage.at[n % 2, :, _cols(t)], back_sem.at[n % 2])
            for t in range(_UNIT)])
        start_when((n >= n_wo) & (n < n_gate),
                   lambda: columns(w2t_hbm, n - n_wo, back_stage, back_sem))
        for side, w in enumerate((w1_hbm, w3_hbm)):
            start_when((n < n_gate) & (n % 2 == side),
                       lambda w=w: columns(w, n // 2, gate_stage, gate_sem))
        start_when(n == n_gate, rest_copies)

    def rest_copies():
        count = len(_REST.piece)
        return [pltpu.make_async_copy(
            w.bitcast(jnp.uint32).at[:, _cols(n_gate // 2 * _UNIT, count)],
            gate_stage.at[n_gate % 2, :, _cols(i * count, count)], gate_sem.at[n_gate % 2])
                for i, w in enumerate((w1_hbm, w3_hbm, w2t_hbm))]

    def combine_qkv(n, w_ref):
        stage = qkv_stage.at[n % 2]

        def part(t, p):
            words = stage[t // 2, pl.ds(p * _T // 2, _T // 2), :]
            words = words & jnp.uint32(0xFFFF0000) if t % 2 else words << 16
            return pltpu.bitcast(words, jnp.float32)

        return _combine(part, w_ref, _WHOLE)

    def combine_columns(stage, w_ref, scheme, first=0, transposed=False):
        return _combine(lambda t, p: _unpack(stage[pl.ds(p * _T // 4, _T // 4), _cols(first + t)]),
                        w_ref, scheme, transposed)

    def x_copy(i):
        return pltpu.make_async_copy(xt_hbm.at[:, part_of(i, _T)], tile_ref.at[i], tile_sem.at[i])

    def out_copy(i):
        return pltpu.make_async_copy(tile_ref.at[i], outt_hbm.at[:, _cols(i)], tile_sem.at[i])

    def transpose_in(i):
        x = tile_ref[i].astype(jnp.float32)
        x = _stack(x, x[_FULL * _T:])
        blocks = [x[b * _T:(b + 1) * _T].T for b in range(_FULL + 1)]
        set_blocks(res_ref, [part_of(i, _T)], blocks)
        normed = _layernorm(
            [_stack(*[x[s - _EARLY:s] for s in range(seg, _T + 1, seg)]) for x in blocks])
        for s in range(_T // seg):
            rows = part_of(i * (_T // seg // 2) + s // 2, _EARLY)
            set_blocks(early_norm_ref, [s % 2, rows],
                       [x[s * _EARLY:(s + 1) * _EARLY] for x in normed])

    def transpose_out(i):
        for b, x in enumerate(blocks_at(res_ref, part_of(i, _T))):
            depth = min(_T, d_model - b * _T)
            tile_ref[i, pl.ds(b * _T, depth), :] = x.T[:depth].astype(tile_ref.dtype)
            yield

    def early_pass(n, weights, first, count, paced=lambda x: x):
        rows = pl.ds(pl.multiple_of(first + _LAG // 2 * _EARLY, _EARLY), count)
        mix = _mixer([blocks_at(early_norm_ref, half, rows) for half in range(2)])
        tiles = yield from _widen(lambda key: paced(mix(key)), 2, weights, _WHOLE)
        for half in range(2):
            at = pl.multiple_of((half * sum(_EARLY_ROWS) + first) // 2, _EARLY // 2)
            early_ref.at[n][pl.ds(at, count // 2), :] = _pack(jnp.concatenate(
                [halves[half] for halves in tiles], axis=1).astype(jnp.bfloat16))

    def early_passes(n, w_ref, chunks, tokens=()):
        total = sum(_EARLY_ROWS[c] for c in chunks) * _count(_WHOLE)
        due = [(total * (k + 1) // (len(tokens) + 1), token) for k, token in enumerate(tokens)]
        done = 0

        def paced(x):
            nonlocal done
            done += x.shape[0]
            while due and due[0][0] <= done:
                x = _stack(x[:-8], jnp.where(always, x[-8:], due.pop(0)[1]))
            return x

        weights = _weights(w_ref)
        for c in chunks:
            list(early_pass(n, weights, sum(_EARLY_ROWS[:c]), _EARLY_ROWS[c], paced))

    def double_step(b):
        step(_ORDER, attend=[b, b + _LAG], feed=[b - 1, b + _LAG - 1], after=_AFTER,
             finished=jnp.maximum(b - 1 - _T // seg, 0) * seg // _T)

    mem_copy = pltpu.make_async_copy(mem0_hbm, mem0_ref.at[0], mem_sem)
    for copy in [mem_copy] + [x_copy(i) for i in range(_FIRST_TILES)]:
        copy.start()
    request_qkv(0, range(_UNIT // 4))
    mem_copy.wait()
    request_qkv(0, range(_UNIT // 4, _UNIT // 2))

    def load_tile(i, _):
        x_copy(i).wait()
        transpose_in(i)
        return i

    always = jax.lax.fori_loop(0, _FIRST_TILES, load_tile, 0) > 0
    mem0 = mem0_ref[0].astype(jnp.float32)
    mem_ref[0] = mem_ref[1] = jnp.concatenate([mem0, mem0[:, _FULL * _T:]], axis=1)
    for i in range(_FIRST_TILES, n_io):
        x_copy(i).start()

    chunks = range(len(_EARLY_ROWS))
    await_whole(qkv_stage.at[0], qkv_sem.at[0])
    request_qkv(1)
    combine_qkv(0, qkv_ref.at[0])
    early_passes(0, qkv_ref.at[0], chunks[:_TILES_ARRIVE])
    for i in range(_FIRST_TILES, n_io):
        x_copy(i).wait()
    request_qkv(2)
    for i in range(_FIRST_TILES, n_io):
        transpose_in(i)
    early_passes(0, qkv_ref.at[0], chunks[_TILES_ARRIVE:_UNIT_ARRIVES])
    await_whole(qkv_stage.at[1], qkv_sem.at[1])
    request_others(0)
    early_passes(0, qkv_ref.at[0], chunks[_UNIT_ARRIVES:], combine_qkv(1, qkv_ref.at[1]))

    @pl.loop(1, n_qkv - 1)
    def _load_units(n):
        both = qkv_ref.at[pl.ds(n, 2)]
        request_qkv(n + 2)
        await_whole(qkv_stage.at[(n + 1) % 2], qkv_sem.at[(n + 1) % 2])
        early_passes(n, both.at[0], chunks[:3], combine_qkv(n + 1, both.at[1]))
        request_others(n)
        await_whole(gate_stage.at[(n - 1) % 2], gate_sem.at[(n - 1) % 2])
        await_whole(back_stage.at[(n - 1) % 2], back_sem.at[(n - 1) % 2])
        early_passes(
            n, both.at[0], chunks[3:],
            combine_columns(back_stage.at[(n - 1) % 2], back_ref.at[n - 1], _WHOLE, transposed=True)
            + combine_columns(gate_stage.at[(n - 1) % 2], gate_ref.at[n - 1], _WHOLE))

    def filler(first, count):
        return early_pass(n_qkv - 1, _weights(qkv_ref.at[n_qkv - 1]), first, count)

    for copy in rest_copies():
        copy.wait()
    early_passes(n_qkv - 1, qkv_ref.at[n_qkv - 1], chunks[:-_LAG - 2], sum([
        combine_columns(gate_stage.at[n_gate % 2], rest_ref.at[i], _REST, i * len(_REST.piece),
                        transposed=i == 2) for i in (2, 1, 0)], []))

    @pl.loop(0, _LAG, unroll=True)
    def _first_steps(s):
        step(_ORDER_HEAD, attend=[s], partner=0,
             filler=filler((chunks[-_LAG - 2] + s) * _EARLY_ROWS[0], _EARLY_ROWS[0]))

    step(_ORDER_FFN + " X0", feed=[0, 1], filler=filler(sum(_EARLY_ROWS[:-2]), _EARLY_ROWS[-2]))
    mem_ref[0], mem_ref[1] = mem_ref[1], mem_ref[0]
    step(_ORDER_HEAD, attend=[0, _LAG], filler=filler(sum(_EARLY_ROWS[:-1]), _EARLY_ROWS[-1]))
    pl.loop(1, n_seg - _LAG)(double_step)
    for i in range(n_io - 1):
        out_copy(i).start()
    step(_ORDER_TAIL, attend=[n_seg - 2], feed=[n_seg - 3, n_seg - 1])
    step(_ORDER_LAST, attend=[n_seg - 1], partner=n_seg - 2)
    step(_ORDER_FFN + " T0", feed=[n_seg - 2, n_seg - 1], finished=n_io - 1)
    out_copy(n_io - 1).start()
    for i in range(n_io):
        out_copy(i).wait()


@functools.partial(jax.jit, static_argnames=("A_seg_len",))
def pallas_interleave_layers__memory_aug_recurrent_mem_tr__glu_gated_swiglu__prompt_kernel(
    A_x: jax.Array,
    A_mem0: jax.Array,
    A_Wq: jax.Array,
    A_Wk: jax.Array,
    A_Wv: jax.Array,
    A_Wo: jax.Array,
    A_seg_len: int,
    B_x: jax.Array,
    B_w1: jax.Array,
    B_w3: jax.Array,
    B_w2: jax.Array,
):
    del B_x
    _, n_tok, d_model = A_x.shape
    n_mem = A_mem0.shape[1]
    assert A_x.shape == (1, 2048, 576) and A_seg_len == 32 and n_mem == 8
    assert A_Wq.shape[1:] == (2 * _UNIT, _T) and B_w1.shape[1] == 36 * _T
    width = (_FULL + 1) * _T
    hbm = pl.BlockSpec(memory_space=pltpu.HBM)

    def weights(scheme, units):
        return pltpu.VMEM((units, _T // 2, _count(scheme) * _T), jnp.uint32)

    out_t = pl.pallas_call(
        functools.partial(_kernel, seg=A_seg_len),
        out_shape=jax.ShapeDtypeStruct((d_model, n_tok), A_x.dtype),
        in_specs=[hbm] * 9,
        out_specs=hbm,
        scratch_shapes=[
            pltpu.VMEM((n_tok // _T, d_model, _T), A_x.dtype),
            pltpu.VMEM((n_tok, width), jnp.float32),
            pltpu.VMEM((2, A_seg_len, width), jnp.float32),
            pltpu.VMEM((2, n_tok // A_seg_len * _EARLY // 2, width), jnp.float32),
            pltpu.VMEM((6, sum(_EARLY_ROWS), _UNIT * _T), jnp.uint32),
            weights(_WHOLE, 6), weights(_WHOLE, 4), weights(_WHOLE, 4), weights(_REST, 3),
            pltpu.VMEM((2, _UNIT // 2, d_model, _T), jnp.uint32),
            pltpu.VMEM((2, d_model // 2, _UNIT * _T), jnp.uint32),
            pltpu.VMEM((2, d_model // 2, _UNIT * _T), jnp.uint32),
            pltpu.VMEM((2, n_mem, width), jnp.float32),
            pltpu.VMEM((8, n_mem, d_model), A_mem0.dtype),
            pltpu.SemaphoreType.DMA((2,)),
            pltpu.SemaphoreType.DMA((2,)),
            pltpu.SemaphoreType.DMA((2,)),
            pltpu.SemaphoreType.DMA((n_tok // _T,)),
            pltpu.SemaphoreType.DMA,
        ],
        compiler_params=pltpu.CompilerParams(vmem_limit_bytes=116 * 1024 * 1024,
                                             disable_bounds_checks=True),
    )(A_x.reshape(n_tok, d_model).T, A_mem0.reshape(n_mem, d_model), A_Wq, A_Wk, A_Wv,
      A_Wo.transpose(0, 2, 1), B_w1, B_w3, B_w2.T)
    return out_t.T.reshape(A_x.shape)
```

```python
import functools
import itertools
import math
from typing import NamedTuple

import jax
import jax.numpy as jnp
import jax.experimental.pallas as pl
import jax.experimental.pallas.tpu as pltpu
import numpy as np

_EPS = 1e-05
_MASKED = -1000000000.0
_LOG2E = math.log2(math.e)
_T = 128
_FULL = 4
_PIECES = ((0, 1), (2, 3), (4, 5), (6, 7), (8, 1), (0, 8))
_UNIT = 16
_LAG = 2
_EARLY = 16
_EARLY_ROWS = (48,) * 9 + (32,) * 2
_FIRST_TILES = 5
_TILES_ARRIVE = 2
_UNIT_ARRIVES = 7
_ORDER = "G0 Q0 K0 K1 V0 Q1+T0 U0 V1 O0 G1 O1 G2 U1+N0 U2 D0 D1 D2 F0"
_AFTER = {
    "S": (363, 391, 399, 439, 453, 472, 500, 541, 549, 617, 633,
          651, 667, 685, 714, 724, 734, 743, 753, 762, 771, 781,
          791, 800, 811, 831, 846, 862, 877, 891, 906, 921),
    "A": (723, 741, 759, 775, 793, 801, 823, 847, 858, 868, 878,
          889, 899, 910, 921, 931, 947, 955, 962, 970, 980, 1004,
          1006, 1010, 1014, 1024, 1025, 1028, 1032, 1038, 1044, 1065)}
_ORDER_HEAD = "Q0 K0 Q1+S8 K1+S8 V0+S16 V1+A16 O0+A16 O1 X0+N0"
_ORDER_TAIL = "G0 U0 G1 U1 G2 U2 Q0 K0 Q1+S8 K1+S8 V0+S8 V1+S8+A16 D0 D1 D2 F0 O0+A16 O1 N0"
_ORDER_LAST = "Q0 K0 Q1+S8 K1+S8 V0+S16 V1+A16 O0+A16 O1 N0"
_ORDER_FFN = "G0 U0 G1 U1 G2 U2 D0 D1 D2 F0"
_RANK = (5, 4, 3, 2, 0, 1)
_LEAD = 0.1


class _Product(NamedTuple):
    rows: tuple
    weights: tuple
    tiles: tuple


class _Scheme(NamedTuple):
    n_tiles: int
    helpers: dict
    parts: dict
    shared: tuple
    main: tuple


def _scheme(n_tiles, helpers, homes, edges):
    def added_to(t):
        return helpers.get(t, ((1, t),))

    def product(rows, weights, tiles):
        rows = tuple(sorted(rows, key=lambda term: term[1:]))
        if rows[0][0] < 0:
            rows = tuple((-s, half, i) for s, half, i in rows)
            tiles = tuple((-s, half, t) for s, half, t in tiles)
        return _Product(rows, tuple(weights), tuple(tiles))

    surplus = {home: [] for home in homes}
    for u, i, v, j in edges:
        for side, (t, own, partner, paired) in enumerate(((u, i, v, j), (v, j, u, i))):
            for s, owner in ((1, t),) if (side, t, own) in surplus else added_to(t):
                surplus[side, owner, own].append(((s, t, paired), (-s, partner, own)))
    products = []
    for t in (*helpers, *range(n_tiles)):
        for (side, owner, i), terms in surplus.items():
            if owner == t and terms:
                products += [
                    product([(1, side, i)], [(1, t, i)] + [term[0] for term in terms],
                            [(1, side, t), (-1, 1 - side, t)]),
                    product([(1, 0, i), (1, 1, i)], [(1, t, i)] + [term[1] for term in terms],
                            [(1, 1 - side, t)])]
            elif owner == t:
                products += [product([(1, half, i)], [(1, t, i)], [(1, half, t)])
                             for half in range(2)]
        for u, i, v, j in edges:
            if u == t:
                products += [
                    product([(1, 1, i), (-1, 1, j)], [(1, v, i)], [(1, 1, v), (1, 1, u)]),
                    product([(1, 0, j), (-1, 0, i)], [(1, u, j)], [(1, 0, u), (1, 0, v)]),
                    product([(1, 0, i), (1, 1, j)], [(1, u, j), (1, v, i)], [(1, 1, u), (1, 0, v)])]
    parts = {(t, i): [None, None] for p in products for _, t, i in p.weights}
    for piece in range(2 * _FULL + 1):
        holders = [(t, i) for t, i in parts if piece in _PIECES[i]]
        adds = np.zeros((n_tiles, len(holders)), int)
        for n, (t, _) in enumerate(holders):
            for s, owner in added_to(t):
                adds[owner, n] = s
        inverse = np.rint(np.linalg.inv(adds)).astype(int)
        assert (adds @ inverse == np.eye(n_tiles)).all() and abs(inverse).max() == 1
        for (t, i), row in zip(holders, inverse.tolist()):
            parts[t, i][_PIECES[i].index(piece)] = [(s, given) for given, s in enumerate(row) if s]
    shared = [p for p in products if p.tiles[0][2] in helpers]
    return _Scheme(n_tiles, helpers, parts, tuple(shared), tuple(products[len(shared):]))


def _whole_scheme():
    helpers = {16 + side * 4 + i: ((1, side * 4 + i), (-1 if i == 2 else 1, 8 + side * 4 + i))
               for side in range(2) for i in range(4)}
    helpers[16] += (1, 9), (1, 14)
    helpers[20] += (1, 10), (1, 15)
    homes = [(t // 4 % 2, t, t % 4 or _FULL + t // 8) for t in range(_UNIT)]
    edges = [(8 * g + i, i or _FULL + g, 8 * g + 4 + j, j or _FULL + g)
             for g in range(2) for i in range(4) for j in range(4)
             if i != j and not (g and 0 < i < j)]
    edges += [(16 + i, i, 20 + j, j) for i in range(4) for j in range(4) if (i == 0) != (j == 0)]
    return _scheme(_UNIT, helpers, homes + [(0, 16, 0), (1, 20, 0)], edges)


_WHOLE = _whole_scheme()
_REST = _scheme(
    4, {4: ((1, 0), (1, 1)), 5: ((1, 2), (1, 3))},
    [(0, 0, 1), (1, 3, 2), (0, 2, 3), (1, 2, _FULL), (0, 1, _FULL + 1), (1, 1, 3), (0, 4, 0),
     (0, 5, 0)],
    [(0, 1, 3, 2), (0, 1, 2, _FULL), (0, 1, 1, 3), (2, 3, 3, 2), (1, _FULL + 1, 3, 2)])


def _numbered(scheme, n_halves):
    kept = [], []
    for n, (rows, weights, tiles) in enumerate(scheme.shared + scheme.main):
        rows = tuple(term for term in rows if term[1] < n_halves)
        tiles = tuple(term for term in tiles if term[1] < n_halves)
        if rows and tiles:
            kept[n >= len(scheme.shared)].append((n, _Product(rows, weights, tiles)))
    return kept


def _count(scheme, n_halves=2):
    return sum(map(len, _numbered(scheme, n_halves)))


def _signed_sum(terms):
    (sign, total), *rest = sorted(terms, key=lambda term: -term[0])
    for s, value in rest:
        total = total + value if s == sign else total - value
    return total if sign > 0 else -total


def _accumulate(acc, key, sign, value):
    if key in acc:
        s, total = acc[key]
        if s == sign:
            acc[key] = s, total + value
        else:
            acc[key] = 1, total - value if s > 0 else value - total
    else:
        acc[key] = sign, value


def _interleaved(main, *others):
    due = sorted((main[1] * (_LEAD + (1 - _LEAD) * (k + m / len(others)) / n), m, k)
                 for m, (_, n) in enumerate(others) for k in range(n))
    for done, _ in enumerate(main[0]):
        while due and due[0][0] <= done:
            next(others[due.pop(0)[1]][0])
        yield
    for other, _ in others:
        list(other)


def _dot(a, b, axis=0):
    return jax.lax.dot_general(a, b, (((1,), (axis,)), ((), ())),
                               preferred_element_type=jnp.float32)


def _pack(x):
    return pltpu.bitcast(x, jnp.uint32)


def _unpack(words):
    return pltpu.bitcast(words, jnp.bfloat16)


def _cols(n, width=1):
    return slice(n * _T, (n + width) * _T)


def _stack(*parts):
    return jnp.concatenate(parts, axis=0)


def _splice(low, high):
    lane = jax.lax.broadcasted_iota(jnp.int32, low.shape, 1)
    return jnp.where(lane < _T // 2, low, high)


def _inverse(x):
    r = pltpu.reciprocal(x, approx=True)
    return r * (2.0 - x * r)


def _layernorm(blocks):
    def mean(terms):
        total = sum(terms[:-1], 0.5 * terms[-1])
        return jnp.sum(total, axis=-1, keepdims=True) * (1 / ((_FULL + 0.5) * _T))

    center = mean(blocks)
    d = [x - center for x in blocks]
    inv = jax.lax.rsqrt(mean([x * x for x in d]) + _EPS)
    return [x * inv for x in d]


def _mixer(halves, dtype=jnp.float32):
    halves = [[*full, _splice(rest, full[0]), _splice(full[0], rest)] for *full, rest in halves]
    return functools.cache(
        lambda rows: _signed_sum([(s, halves[half][i]) for s, half, i in rows]).astype(dtype))


def _weights(w_ref):
    w = _unpack(w_ref[...])
    return functools.cache(lambda n: w[:, _cols(n)])


def _widen(mix, n_halves, weights, scheme):
    acc = {}
    for products in _numbered(scheme, n_halves):
        for (helper, half), (sign, value) in list(acc.items()):
            for s, t in scheme.helpers[helper]:
                _accumulate(acc, (t, half), s * sign, value)
        for n, (rows, _, tiles) in products:
            value = _dot(mix(rows), weights(n))
            for s, half, t in tiles:
                _accumulate(acc, (t, half), s, value)
            yield
    return [[_signed_sum([acc[t, half]]) for half in range(n_halves)]
            for t in range(scheme.n_tiles)]


def _narrow(acc, wide, weights, scheme):
    n_halves = len(wide[0])
    wide = wide + [[_signed_sum([(s, wide[t][half]) for s, t in added]) for half in range(n_halves)]
                   for added in scheme.helpers.values()]
    by_rows = {}
    for n, product in sum(_numbered(scheme, n_halves)[::-1], []):
        by_rows.setdefault(product.rows, []).append((n, product.tiles))
    for rows in sorted(by_rows, key=lambda rows: sorted({_RANK[i] for _, _, i in rows})):
        total = {}
        for n, tiles in by_rows[rows]:
            sign = max(s for s, _, _ in tiles)
            lhs = _signed_sum([(s * sign, wide[t][half]) for s, half, t in tiles])
            _accumulate(total, rows, sign, _dot(lhs, weights(n)))
            yield
        for s, half, i in rows:
            _accumulate(acc, (half, i), s * total[rows][0], total[rows][1])


def _narrowed(acc, half):
    first, *others, low, high = [_signed_sum([acc[half, i]]) for i in range(len(_PIECES))]
    rest = _splice(low, high)
    rest += jnp.concatenate([rest[:, _T // 2:], rest[:, :_T // 2]], axis=1)
    return [first + _splice(high, low), *others, rest]


def _combine(part, w_ref, scheme, transposed=False):
    products = scheme.shared + scheme.main
    uses = {}
    for n in sorted(range(len(products)), key=lambda n: len(products[n].weights) > 1):
        for s, t, i in products[n].weights:
            uses.setdefault((t, i), []).append((s, n))

    def gathered(terms, piece):
        if len(terms) == 1 and terms[0][0] > 0:
            return part(terms[0][1], piece)
        return _signed_sum([(s, part(t, piece).astype(jnp.float32)) for s, t in terms])

    acc, missing, stored = {}, [len(product.weights) for product in products], []
    for t, i in sorted(uses, key=lambda source: uses[source][0][1]):
        w = _stack(*map(gathered, scheme.parts[t, i], _PIECES[i]))
        exact = w.astype(jnp.float32)
        for s, n in uses[t, i]:
            _accumulate(acc, n, s, exact if len(products[n].weights) > 1 else w)
            missing[n] -= 1
            if not missing[n]:
                w_ref[:, _cols(n)] = _pack(_signed_sum([acc.pop(n)]).astype(jnp.bfloat16))
                stored.append(w_ref[:, _cols(n)])
    stored = [functools.reduce(jnp.bitwise_or, stored[n:n + 4]) for n in range(0, len(stored), 4)]
    stored = [pltpu.bitcast(words, jnp.float32) for words in stored]
    tokens = [words[r:r + 8] for r in range(0, _T // 2, 8) for words in stored]
    for n in range(len(products) if transposed else 0):
        w_ref[:, _cols(n)] = words = _pack(_unpack(w_ref[:, _cols(n)]).T)
        tokens.append(pltpu.bitcast(words[-8:], jnp.float32))
    return tokens


def _kernel(xt_hbm, mem0_hbm, wq_hbm, wk_hbm, wv_hbm, wot_hbm, w1_hbm, w3_hbm, w2t_hbm,
            outt_hbm, tile_ref, res_ref, norm_ref, early_norm_ref, early_ref, qkv_ref, gate_ref,
            back_ref, rest_ref, qkv_stage, gate_stage, back_stage, mem_ref,
            mem0_ref, qkv_sem, gate_sem, back_sem, tile_sem, mem_sem, *, seg):
    d_model, n_tok = xt_hbm.shape
    n_mem = mem0_hbm.shape[0]
    n_seg = n_tok // seg
    n_io = n_tok // _T
    span = n_mem + seg
    score_scale = wq_hbm.shape[2] ** -0.5 * _LOG2E
    n_qkv, n_gate = early_ref.shape[0], gate_ref.shape[0]
    n_wo = n_qkv // 3

    def blocks_at(ref, *index):
        return [ref[(*index, _cols(i))] for i in range(_FULL + 1)]

    def set_blocks(ref, index, blocks):
        for i, x in enumerate(blocks):
            ref[(*index, _cols(i))] = x

    def part_of(i, size):
        return pl.ds(pl.multiple_of(i * size, size), size)

    def step(order, attend=(), feed=(), partner=None, finished=None, filler=None, after=()):
        n_layers = len(attend)
        operand = jnp.bfloat16 if n_layers == 2 else jnp.float32
        qkv, probs, heads, mixed = {"Q": [], "K": [], "V": []}, [], [], {}
        gates, hidden, fed = [], [], {}
        if attend:
            query, key = (jax.lax.broadcasted_iota(jnp.int32, (span, _T), a) for a in (0, 1))
            own_keys = [(key >= n * span) & (key < (n + 1) * span) for n in range(n_layers)]
            visible = (query < n_mem) | (query >= jnp.where(key < span, key, key - span))
            mem = [blocks_at(mem_ref, n, slice(None)) for n in range(n_layers)]
            h = _layernorm(blocks_at(res_ref, part_of(attend[0], seg)))
            if n_layers == 1:
                attend_mix = _mixer([list(map(_stack, mem[0], h))])
            else:
                ahead = _layernorm(
                    [x[:seg - _EARLY] for x in blocks_at(res_ref, part_of(attend[1], seg))])
                cut = seg - _EARLY // 2
                known = part_of(attend[0] % 2 * (sum(_EARLY_ROWS) // _EARLY) + attend[0] // 2,
                                _EARLY // 2)
                attend_mix = _mixer(
                    [[_stack(m, a[:cut]) for m, a in zip(mem[0], h)],
                     [_stack(m, a[cut:], b) for m, a, b in zip(mem[1], h, ahead)]], operand)
        if feed:
            feed_mix = _mixer([blocks_at(norm_ref, n, slice(None)) for n in range(2)])

        def project(stage, n):
            tiles = yield from _widen(attend_mix, n_layers, _weights(qkv_ref.at[n]), _WHOLE)
            if n_layers == 1:
                qkv[stage] += [halves[0] for halves in tiles]
                return
            moved = n_mem + _EARLY // 2
            early = _unpack(early_ref[n, known, :]).astype(jnp.float32)
            for t, (a, b) in enumerate(tiles):
                x = _stack(a, b[n_mem:moved], b[:n_mem], b[moved:], early[:, _cols(t)])
                if stage == "V":
                    x = _stack(x, jnp.zeros((_T - 2 * span, _T), x.dtype))
                qkv[stage].append(x if stage == "Q" else x.astype(operand))

        def score(count):
            for t in range(len(probs), len(probs) + count):
                s = _dot(qkv["Q"][t], qkv["K"][t], axis=1)
                if n_layers == 2:
                    s = jnp.where(own_keys[1][:, :2 * span], s[span:], s[:span])
                s = jnp.concatenate(
                    [s * score_scale, jnp.zeros((span, _T - s.shape[1]), s.dtype)], axis=1)
                s = jnp.where(visible, s, _MASKED * _LOG2E)
                top = [jnp.max(jnp.where(own, s, -jnp.inf), axis=-1, keepdims=True)
                       for own in own_keys]
                p = jnp.exp2(s - jnp.where(own_keys[-1], top[-1], top[0]))
                p = _stack(*[jnp.where(own, p, 0.0) for own in own_keys])
                probs.append((p.astype(operand), _inverse(jnp.sum(p, axis=-1, keepdims=True))))
                yield

        def average(count):
            for t in range(len(heads), len(heads) + count):
                (p, inv), v = probs[t], qkv["V"][t]
                both = _dot(p[:, :v.shape[0]], v) * inv
                heads.append([both[n * span:(n + 1) * span] for n in range(n_layers)])
                yield

        def add_attended():
            x = [] if partner is None else [blocks_at(res_ref, part_of(partner, seg))]
            before = [blocks_at(res_ref, part_of(s, seg)) for s in attend]
            for n, s in enumerate(attend):
                out = _narrowed(mixed, n)
                x.append([a + o[n_mem:] for a, o in zip(before[n], out)])
                set_blocks(res_ref, [part_of(s, seg)], x[-1])
                set_blocks(mem_ref, [n, slice(None)], [o[:n_mem] for o in out])
            for n, blocks in enumerate(x):
                set_blocks(norm_ref, [n, slice(None)], _layernorm(blocks))
                yield

        def gate(w_ref, scheme):
            for halves in (yield from _widen(feed_mix, 2, _weights(w_ref), scheme)):
                gates.append([g * jnp.tanh(g) + g for g in [0.5 * x for x in halves]])

        def up(w_ref, scheme):
            for halves in (yield from _widen(feed_mix, 2, _weights(w_ref), scheme)):
                hidden.append([g * x for g, x in zip(gates[len(hidden)], halves)])

        def add_fed():
            before = [blocks_at(res_ref, part_of(s, seg)) for s in feed]
            for n, s in enumerate(feed):
                set_blocks(res_ref, [part_of(s, seg)],
                           [a + o for a, o in zip(before[n], _narrowed(fed, n))])
            yield

        def begin(name):
            stage, number = name[0], int(name[1:])
            if stage in "SA":
                return (score if stage == "S" else average)(number), number
            if stage in "NF":
                return (add_attended if stage == "N" else add_fed)(), 1
            if stage == "T":
                return transpose_out(finished), _FULL + 1
            if stage == "X":
                return filler, _count(_WHOLE)
            if stage in "QKV":
                return project(stage, 3 * number + "QKV".index(stage)), _count(_WHOLE, n_layers)
            ref, n = {"G": (gate_ref, 2 * number), "U": (gate_ref, 2 * number + 1),
                      "O": (back_ref, number), "D": (back_ref, n_wo + number)}[stage]
            w_ref, scheme = ((ref.at[n], _WHOLE) if n < n_gate
                             else (rest_ref.at["GUD".index(stage)], _REST))
            if stage in "GU":
                return (gate if stage == "G" else up)(w_ref, scheme), _count(scheme)
            acc, wide = (mixed, heads) if stage == "O" else (fed, hidden)
            wide = wide[number * _UNIT:(number + 1) * _UNIT]
            return _narrow(acc, wide, _weights(w_ref), scheme), _count(scheme, len(wide[0]))

        due = sorted((n, stage) for stage in after for n in after[stage])
        passes = itertools.chain.from_iterable(
            _interleaved(*map(begin, names.split("+"))) for names in order.split())
        for done, _ in enumerate(passes):
            while due and due[0][0] <= done:
                next(begin(due.pop(0)[1] + "1")[0])

    def start_when(condition, copies):
        @pl.when(condition)
        def _():
            for copy in copies():
                copy.start()

    def await_whole(ref, sem):
        pltpu.make_async_copy(ref, ref, sem).wait()

    def request_qkv(n, pairs=range(_UNIT // 2)):
        for which, w in enumerate((wq_hbm, wk_hbm, wv_hbm)):
            start_when((n < n_qkv) & (n % 3 == which), lambda w=w: [
                pltpu.make_async_copy(w.bitcast(jnp.uint32).at[:, n // 3 * (_UNIT // 2) + p, :],
                                      qkv_stage.at[n % 2, p], qkv_sem.at[n % 2]) for p in pairs])

    def request_others(n):
        def columns(w_hbm, unit, stage, sem):
            return [pltpu.make_async_copy(
                w_hbm.bitcast(jnp.uint32).at[:, part_of(unit, _UNIT * _T)],
                stage.at[n % 2], sem.at[n % 2])]

        start_when(n < n_wo, lambda: [
            pltpu.make_async_copy(wot_hbm.bitcast(jnp.uint32).at[n * _UNIT + t],
                                  back_stage.at[n % 2, :, _cols(t)], back_sem.at[n % 2])
            for t in range(_UNIT)])
        start_when((n >= n_wo) & (n < n_gate),
                   lambda: columns(w2t_hbm, n - n_wo, back_stage, back_sem))
        for side, w in enumerate((w1_hbm, w3_hbm)):
            start_when((n < n_gate) & (n % 2 == side),
                       lambda w=w: columns(w, n // 2, gate_stage, gate_sem))
        start_when(n == n_gate, rest_copies)

    def rest_copies():
        count = _REST.n_tiles
        return [pltpu.make_async_copy(
            w.bitcast(jnp.uint32).at[:, _cols(n_gate // 2 * _UNIT, count)],
            gate_stage.at[n_gate % 2, :, _cols(i * count, count)], gate_sem.at[n_gate % 2])
                for i, w in enumerate((w1_hbm, w3_hbm, w2t_hbm))]

    def combine_qkv(n, w_ref):
        stage = qkv_stage.at[n % 2]

        def part(t, p):
            words = stage[t // 2, pl.ds(p * _T // 2, _T // 2), :]
            words = words & jnp.uint32(0xFFFF0000) if t % 2 else words << 16
            return pltpu.bitcast(words, jnp.float32)

        return _combine(part, w_ref, _WHOLE)

    def combine_columns(stage, w_ref, scheme, first=0, transposed=False):
        return _combine(lambda t, p: _unpack(stage[pl.ds(p * _T // 4, _T // 4), _cols(first + t)]),
                        w_ref, scheme, transposed)

    def x_copy(i):
        return pltpu.make_async_copy(xt_hbm.at[:, part_of(i, _T)], tile_ref.at[i], tile_sem.at[i])

    def out_copy(i):
        return pltpu.make_async_copy(tile_ref.at[i], outt_hbm.at[:, _cols(i)], tile_sem.at[i])

    def transpose_in(i):
        x = tile_ref[i].astype(jnp.float32)
        x = _stack(x, x[_FULL * _T:])
        blocks = [x[b * _T:(b + 1) * _T].T for b in range(_FULL + 1)]
        set_blocks(res_ref, [part_of(i, _T)], blocks)
        normed = _layernorm(
            [_stack(*[x[s - _EARLY:s] for s in range(seg, _T + 1, seg)]) for x in blocks])
        for s in range(_T // seg):
            rows = part_of(i * (_T // seg // 2) + s // 2, _EARLY)
            set_blocks(early_norm_ref, [s % 2, rows],
                       [x[s * _EARLY:(s + 1) * _EARLY] for x in normed])

    def transpose_out(i):
        for b, x in enumerate(blocks_at(res_ref, part_of(i, _T))):
            depth = min(_T, d_model - b * _T)
            tile_ref[i, pl.ds(b * _T, depth), :] = x.T[:depth].astype(tile_ref.dtype)
            yield

    def early_pass(n, weights, first, count, paced=lambda x: x):
        rows = pl.ds(pl.multiple_of(first + _LAG // 2 * _EARLY, _EARLY), count)
        mix = _mixer([blocks_at(early_norm_ref, half, rows) for half in range(2)])
        tiles = yield from _widen(lambda key: paced(mix(key)), 2, weights, _WHOLE)
        for half in range(2):
            at = pl.multiple_of((half * sum(_EARLY_ROWS) + first) // 2, _EARLY // 2)
            early_ref.at[n][pl.ds(at, count // 2), :] = _pack(jnp.concatenate(
                [halves[half] for halves in tiles], axis=1).astype(jnp.bfloat16))

    def early_passes(n, w_ref, chunks, tokens=()):
        total = sum(_EARLY_ROWS[c] for c in chunks) * _count(_WHOLE)
        due = [(total * (k + 1) // (len(tokens) + 1), token) for k, token in enumerate(tokens)]
        done = 0

        def paced(x):
            nonlocal done
            done += x.shape[0]
            while due and due[0][0] <= done:
                x = _stack(x[:-8], jnp.where(always, x[-8:], due.pop(0)[1]))
            return x

        weights = _weights(w_ref)
        for c in chunks:
            list(early_pass(n, weights, sum(_EARLY_ROWS[:c]), _EARLY_ROWS[c], paced))

    def double_step(b):
        step(_ORDER, attend=[b, b + _LAG], feed=[b - 1, b + _LAG - 1], after=_AFTER,
             finished=jnp.maximum(b - 1 - _T // seg, 0) * seg // _T)

    mem_copy = pltpu.make_async_copy(mem0_hbm, mem0_ref.at[0], mem_sem)
    for copy in [mem_copy] + [x_copy(i) for i in range(_FIRST_TILES)]:
        copy.start()
    request_qkv(0, range(_UNIT // 4))
    mem_copy.wait()
    request_qkv(0, range(_UNIT // 4, _UNIT // 2))

    def load_tile(i, _):
        x_copy(i).wait()
        transpose_in(i)
        return i

    always = jax.lax.fori_loop(0, _FIRST_TILES, load_tile, 0) > 0
    mem0 = mem0_ref[0].astype(jnp.float32)
    mem_ref[0] = mem_ref[1] = jnp.concatenate([mem0, mem0[:, _FULL * _T:]], axis=1)
    for i in range(_FIRST_TILES, n_io):
        x_copy(i).start()

    chunks = range(len(_EARLY_ROWS))
    await_whole(qkv_stage.at[0], qkv_sem.at[0])
    request_qkv(1)
    combine_qkv(0, qkv_ref.at[0])
    early_passes(0, qkv_ref.at[0], chunks[:_TILES_ARRIVE])
    for i in range(_FIRST_TILES, n_io):
        x_copy(i).wait()
    request_qkv(2)
    for i in range(_FIRST_TILES, n_io):
        transpose_in(i)
    early_passes(0, qkv_ref.at[0], chunks[_TILES_ARRIVE:_UNIT_ARRIVES])
    await_whole(qkv_stage.at[1], qkv_sem.at[1])
    request_others(0)
    early_passes(0, qkv_ref.at[0], chunks[_UNIT_ARRIVES:], combine_qkv(1, qkv_ref.at[1]))

    @pl.loop(1, n_qkv - 1)
    def _load_units(n):
        both = qkv_ref.at[pl.ds(n, 2)]
        request_qkv(n + 2)
        await_whole(qkv_stage.at[(n + 1) % 2], qkv_sem.at[(n + 1) % 2])
        early_passes(n, both.at[0], chunks[:3], combine_qkv(n + 1, both.at[1]))
        request_others(n)
        await_whole(gate_stage.at[(n - 1) % 2], gate_sem.at[(n - 1) % 2])
        await_whole(back_stage.at[(n - 1) % 2], back_sem.at[(n - 1) % 2])
        early_passes(
            n, both.at[0], chunks[3:],
            combine_columns(back_stage.at[(n - 1) % 2], back_ref.at[n - 1], _WHOLE, transposed=True)
            + combine_columns(gate_stage.at[(n - 1) % 2], gate_ref.at[n - 1], _WHOLE))

    def filler(first, count):
        return early_pass(n_qkv - 1, _weights(qkv_ref.at[n_qkv - 1]), first, count)

    for copy in rest_copies():
        copy.wait()
    early_passes(n_qkv - 1, qkv_ref.at[n_qkv - 1], chunks[:-_LAG - 2], sum([
        combine_columns(gate_stage.at[n_gate % 2], rest_ref.at[i], _REST, i * _REST.n_tiles,
                        transposed=i == 2) for i in (2, 1, 0)], []))

    @pl.loop(0, _LAG, unroll=True)
    def _first_steps(s):
        step(_ORDER_HEAD, attend=[s], partner=0,
             filler=filler((chunks[-_LAG - 2] + s) * _EARLY_ROWS[0], _EARLY_ROWS[0]))

    step(_ORDER_FFN + " X0", feed=[0, 1], filler=filler(sum(_EARLY_ROWS[:-2]), _EARLY_ROWS[-2]))
    mem_ref[0], mem_ref[1] = mem_ref[1], mem_ref[0]
    step(_ORDER_HEAD, attend=[0, _LAG], filler=filler(sum(_EARLY_ROWS[:-1]), _EARLY_ROWS[-1]))
    pl.loop(1, n_seg - _LAG)(double_step)
    for i in range(n_io - 1):
        out_copy(i).start()
    step(_ORDER_TAIL, attend=[n_seg - 2], feed=[n_seg - 3, n_seg - 1])
    step(_ORDER_LAST, attend=[n_seg - 1], partner=n_seg - 2)
    step(_ORDER_FFN + " T0", feed=[n_seg - 2, n_seg - 1], finished=n_io - 1)
    out_copy(n_io - 1).start()
    for i in range(n_io):
        out_copy(i).wait()


@functools.partial(jax.jit, static_argnames=("A_seg_len",))
def pallas_interleave_layers__memory_aug_recurrent_mem_tr__glu_gated_swiglu__prompt_kernel(
    A_x: jax.Array,
    A_mem0: jax.Array,
    A_Wq: jax.Array,
    A_Wk: jax.Array,
    A_Wv: jax.Array,
    A_Wo: jax.Array,
    A_seg_len: int,
    B_x: jax.Array,
    B_w1: jax.Array,
    B_w3: jax.Array,
    B_w2: jax.Array,
):
    del B_x
    _, n_tok, d_model = A_x.shape
    n_mem = A_mem0.shape[1]
    assert A_x.shape == (1, 2048, 576) and A_seg_len == 32 and n_mem == 8
    assert A_Wq.shape[1:] == (2 * _UNIT, _T) and B_w1.shape[1] == 36 * _T
    width = (_FULL + 1) * _T
    hbm = pl.BlockSpec(memory_space=pltpu.HBM)

    def weights(scheme, units):
        return pltpu.VMEM((units, _T // 2, _count(scheme) * _T), jnp.uint32)

    out_t = pl.pallas_call(
        functools.partial(_kernel, seg=A_seg_len),
        out_shape=jax.ShapeDtypeStruct((d_model, n_tok), A_x.dtype),
        in_specs=[hbm] * 9,
        out_specs=hbm,
        scratch_shapes=[
            pltpu.VMEM((n_tok // _T, d_model, _T), A_x.dtype),
            pltpu.VMEM((n_tok, width), jnp.float32),
            pltpu.VMEM((2, A_seg_len, width), jnp.float32),
            pltpu.VMEM((2, n_tok // A_seg_len * _EARLY // 2, width), jnp.float32),
            pltpu.VMEM((6, sum(_EARLY_ROWS), _UNIT * _T), jnp.uint32),
            weights(_WHOLE, 6), weights(_WHOLE, 4), weights(_WHOLE, 4), weights(_REST, 3),
            pltpu.VMEM((2, _UNIT // 2, d_model, _T), jnp.uint32),
            pltpu.VMEM((2, d_model // 2, _UNIT * _T), jnp.uint32),
            pltpu.VMEM((2, d_model // 2, _UNIT * _T), jnp.uint32),
            pltpu.VMEM((2, n_mem, width), jnp.float32),
            pltpu.VMEM((8, n_mem, d_model), A_mem0.dtype),
            pltpu.SemaphoreType.DMA((2,)),
            pltpu.SemaphoreType.DMA((2,)),
            pltpu.SemaphoreType.DMA((2,)),
            pltpu.SemaphoreType.DMA((n_tok // _T,)),
            pltpu.SemaphoreType.DMA,
        ],
        compiler_params=pltpu.CompilerParams(vmem_limit_bytes=116 * 1024 * 1024,
                                             disable_bounds_checks=True),
    )(A_x.reshape(n_tok, d_model).T, A_mem0.reshape(n_mem, d_model), A_Wq, A_Wk, A_Wv,
      A_Wo.transpose(0, 2, 1), B_w1, B_w3, B_w2.T)
    return out_t.T.reshape(A_x.shape)
```

```python
import functools
import itertools
import math
from typing import NamedTuple

import jax
import jax.numpy as jnp
import jax.experimental.pallas as pl
import jax.experimental.pallas.tpu as pltpu
import numpy as np

_EPS = 1e-05
_MASKED = -1000000000.0
_LOG2E = math.log2(math.e)
_T = 128
_FULL = 4
_PIECES = ((0, 1), (2, 3), (4, 5), (6, 7), (8, 1), (0, 8))
_UNIT = 16
_LAG = 2
_EARLY = 16
_EARLY_ROWS = (48,) * 9 + (32,) * 2
_FIRST_TILES = 5
_TILES_ARRIVE = 2
_UNIT_ARRIVES = 7
_ORDER = "G0 Q0 K0 K1 V0 Q1+T0 U0 V1 O0 G1 O1 G2 U1+N0 U2 D0 D1 D2 F0"
_AFTER = {
    "S": (363, 391, 399, 439, 453, 472, 500, 541, 549, 617, 633,
          651, 667, 685, 714, 724, 734, 743, 753, 762, 771, 781,
          791, 800, 811, 831, 846, 862, 877, 891, 906, 921),
    "A": (723, 741, 759, 775, 793, 801, 823, 847, 858, 868, 878,
          889, 899, 910, 921, 931, 947, 955, 962, 970, 980, 1004,
          1006, 1010, 1014, 1024, 1025, 1028, 1032, 1038, 1044, 1065)}
_ORDER_HEAD = "Q0 K0 Q1+S8 K1+S8 V0+S16 V1+A16 O0+A16 O1 X0+N0"
_ORDER_TAIL = "G0 U0 G1 U1 G2 U2 Q0 K0 Q1+S8 K1+S8 V0+S8 V1+S8+A16 D0 D1 D2 F0 O0+A16 O1 N0"
_ORDER_LAST = "Q0 K0 Q1+S8 K1+S8 V0+S16 V1+A16 O0+A16 O1 N0"
_ORDER_FFN = "G0 U0 G1 U1 G2 U2 D0 D1 D2 F0"
_RANK = (5, 4, 3, 2, 0, 1)
_LEAD = 0.1


class _Product(NamedTuple):
    rows: tuple
    weights: tuple
    tiles: tuple


class _Scheme(NamedTuple):
    n_tiles: int
    helpers: dict
    parts: dict
    shared: tuple
    main: tuple


def _scheme(n_tiles, helpers, homes, edges):
    def added_to(t):
        return helpers.get(t, ((1, t),))

    def product(rows, weights, tiles):
        rows = tuple(sorted(rows, key=lambda term: term[1:]))
        if rows[0][0] < 0:
            rows = tuple((-s, half, i) for s, half, i in rows)
            tiles = tuple((-s, half, t) for s, half, t in tiles)
        return _Product(rows, tuple(weights), tuple(tiles))

    surplus = {home: [] for home in homes}
    for u, i, v, j in edges:
        for side, (t, own, partner, paired) in enumerate(((u, i, v, j), (v, j, u, i))):
            for s, owner in ((1, t),) if (side, t, own) in surplus else added_to(t):
                surplus[side, owner, own].append(((s, t, paired), (-s, partner, own)))
    products = []
    for t in (*helpers, *range(n_tiles)):
        for (side, owner, i), terms in surplus.items():
            if owner == t and terms:
                products += [
                    product([(1, side, i)], [(1, t, i)] + [term[0] for term in terms],
                            [(1, side, t), (-1, 1 - side, t)]),
                    product([(1, 0, i), (1, 1, i)], [(1, t, i)] + [term[1] for term in terms],
                            [(1, 1 - side, t)])]
            elif owner == t:
                products += [product([(1, half, i)], [(1, t, i)], [(1, half, t)])
                             for half in range(2)]
        for u, i, v, j in edges:
            if u == t:
                products += [
                    product([(1, 1, i), (-1, 1, j)], [(1, v, i)], [(1, 1, v), (1, 1, u)]),
                    product([(1, 0, j), (-1, 0, i)], [(1, u, j)], [(1, 0, u), (1, 0, v)]),
                    product([(1, 0, i), (1, 1, j)], [(1, u, j), (1, v, i)], [(1, 1, u), (1, 0, v)])]
    parts = {(t, i): [None, None] for p in products for _, t, i in p.weights}
    for piece in range(2 * _FULL + 1):
        holders = [(t, i) for t, i in parts if piece in _PIECES[i]]
        adds = np.zeros((n_tiles, len(holders)), int)
        for n, (t, _) in enumerate(holders):
            for s, owner in added_to(t):
                adds[owner, n] = s
        inverse = np.rint(np.linalg.inv(adds)).astype(int)
        assert (adds @ inverse == np.eye(n_tiles)).all() and abs(inverse).max() == 1
        for (t, i), row in zip(holders, inverse.tolist()):
            parts[t, i][_PIECES[i].index(piece)] = [(s, given) for given, s in enumerate(row) if s]
    shared = [p for p in products if p.tiles[0][2] in helpers]
    return _Scheme(n_tiles, helpers, parts, tuple(shared), tuple(products[len(shared):]))


def _whole_scheme():
    helpers = {16 + side * 4 + i: ((1, side * 4 + i), (-1 if i == 2 else 1, 8 + side * 4 + i))
               for side in range(2) for i in range(4)}
    helpers[16] += (1, 9), (1, 14)
    helpers[20] += (1, 10), (1, 15)
    homes = [(t // 4 % 2, t, t % 4 or _FULL + t // 8) for t in range(_UNIT)]
    edges = [(8 * g + i, i or _FULL + g, 8 * g + 4 + j, j or _FULL + g)
             for g in range(2) for i in range(4) for j in range(4)
             if i != j and not (g and 0 < i < j)]
    edges += [(16 + i, i, 20 + j, j) for i in range(4) for j in range(4) if (i == 0) != (j == 0)]
    return _scheme(_UNIT, helpers, homes + [(0, 16, 0), (1, 20, 0)], edges)


_WHOLE = _whole_scheme()
_REST = _scheme(
    4, {4: ((1, 0), (1, 1)), 5: ((1, 2), (1, 3))},
    [(0, 0, 1), (1, 3, 2), (0, 2, 3), (1, 2, _FULL), (0, 1, _FULL + 1), (1, 1, 3), (0, 4, 0),
     (0, 5, 0)],
    [(0, 1, 3, 2), (0, 1, 2, _FULL), (0, 1, 1, 3), (2, 3, 3, 2), (1, _FULL + 1, 3, 2)])


def _numbered(scheme, n_halves):
    kept = [], []
    for n, (rows, weights, tiles) in enumerate(scheme.shared + scheme.main):
        rows = tuple(term for term in rows if term[1] < n_halves)
        tiles = tuple(term for term in tiles if term[1] < n_halves)
        if rows and tiles:
            kept[n >= len(scheme.shared)].append((n, _Product(rows, weights, tiles)))
    return kept


def _count(scheme, n_halves=2):
    return sum(map(len, _numbered(scheme, n_halves)))


def _signed_sum(terms):
    (sign, total), *rest = sorted(terms, key=lambda term: -term[0])
    for s, value in rest:
        total = total + value if s == sign else total - value
    return total if sign > 0 else -total


def _accumulate(acc, key, sign, value):
    if key in acc:
        s, total = acc[key]
        if s == sign:
            acc[key] = s, total + value
        else:
            acc[key] = 1, total - value if s > 0 else value - total
    else:
        acc[key] = sign, value


def _interleaved(main, *others):
    due = sorted((main[1] * (_LEAD + (1 - _LEAD) * (k + m / len(others)) / n), m, k)
                 for m, (_, n) in enumerate(others) for k in range(n))
    for done, _ in enumerate(main[0]):
        while due and due[0][0] <= done:
            next(others[due.pop(0)[1]][0])
        yield
    for other, _ in others:
        list(other)


def _dot(a, b, axis=0):
    return jax.lax.dot_general(a, b, (((1,), (axis,)), ((), ())),
                               preferred_element_type=jnp.float32)


def _pack(x):
    return pltpu.bitcast(x, jnp.uint32)


def _unpack(words):
    return pltpu.bitcast(words, jnp.bfloat16)


def _cols(n, width=1):
    return slice(n * _T, (n + width) * _T)


def _stack(*parts):
    return jnp.concatenate(parts, axis=0)


def _splice(low, high):
    lane = jax.lax.broadcasted_iota(jnp.int32, low.shape, 1)
    return jnp.where(lane < _T // 2, low, high)


def _inverse(x):
    r = pltpu.reciprocal(x, approx=True)
    return r * (2.0 - x * r)


def _layernorm(blocks):
    def mean(terms):
        total = sum(terms[:-1], 0.5 * terms[-1])
        return jnp.sum(total, axis=-1, keepdims=True) * (1 / ((_FULL + 0.5) * _T))

    center = mean(blocks)
    d = [x - center for x in blocks]
    inv = jax.lax.rsqrt(mean([x * x for x in d]) + _EPS)
    return [x * inv for x in d]


def _mixer(halves, dtype=jnp.float32):
    halves = [[*full, _splice(rest, full[0]), _splice(full[0], rest)] for *full, rest in halves]
    return functools.cache(
        lambda rows: _signed_sum([(s, halves[half][i]) for s, half, i in rows]).astype(dtype))


def _weights(w_ref):
    w = _unpack(w_ref[...])
    return functools.cache(lambda n: w[:, _cols(n)])


def _widen(mix, n_halves, weights, scheme):
    acc = {}
    for products in _numbered(scheme, n_halves):
        for (helper, half), (sign, value) in list(acc.items()):
            for s, t in scheme.helpers[helper]:
                _accumulate(acc, (t, half), s * sign, value)
        for n, (rows, _, tiles) in products:
            value = _dot(mix(rows), weights(n))
            for s, half, t in tiles:
                _accumulate(acc, (t, half), s, value)
            yield
    return [[_signed_sum([acc[t, half]]) for half in range(n_halves)]
            for t in range(scheme.n_tiles)]


def _narrow(acc, wide, weights, scheme):
    n_halves = len(wide[0])
    wide = wide + [[_signed_sum([(s, wide[t][half]) for s, t in added]) for half in range(n_halves)]
                   for added in scheme.helpers.values()]
    by_rows = {}
    for n, product in sum(_numbered(scheme, n_halves)[::-1], []):
        by_rows.setdefault(product.rows, []).append((n, product.tiles))
    for rows in sorted(by_rows, key=lambda rows: sorted({_RANK[i] for _, _, i in rows})):
        total = {}
        for n, tiles in by_rows[rows]:
            sign = max(s for s, _, _ in tiles)
            lhs = _signed_sum([(s * sign, wide[t][half]) for s, half, t in tiles])
            _accumulate(total, rows, sign, _dot(lhs, weights(n)))
            yield
        for s, half, i in rows:
            _accumulate(acc, (half, i), s * total[rows][0], total[rows][1])


def _narrowed(acc, half):
    first, *others, low, high = [_signed_sum([acc[half, i]]) for i in range(len(_PIECES))]
    rest = _splice(low, high)
    rest += jnp.concatenate([rest[:, _T // 2:], rest[:, :_T // 2]], axis=1)
    return [first + _splice(high, low), *others, rest]


def _combine(part, w_ref, scheme):
    products = scheme.shared + scheme.main
    uses = {}
    for n in sorted(range(len(products)), key=lambda n: len(products[n].weights) > 1):
        for s, t, i in products[n].weights:
            uses.setdefault((t, i), []).append((s, n))

    def gathered(terms, piece):
        if len(terms) == 1 and terms[0][0] > 0:
            return part(terms[0][1], piece)
        return _signed_sum([(s, part(t, piece).astype(jnp.float32)) for s, t in terms])

    acc, missing, stored = {}, [len(product.weights) for product in products], []
    for t, i in sorted(uses, key=lambda source: uses[source][0][1]):
        w = _stack(*map(gathered, scheme.parts[t, i], _PIECES[i]))
        exact = w.astype(jnp.float32)
        for s, n in uses[t, i]:
            _accumulate(acc, n, s, exact if len(products[n].weights) > 1 else w)
            missing[n] -= 1
            if not missing[n]:
                w_ref[:, _cols(n)] = _pack(_signed_sum([acc.pop(n)]).astype(jnp.bfloat16))
                stored.append(w_ref[:, _cols(n)])
    stored = [functools.reduce(jnp.bitwise_or, stored[n:n + 4]) for n in range(0, len(stored), 4)]
    stored = [pltpu.bitcast(words, jnp.float32) for words in stored]
    return [words[r:r + 8] for r in range(0, _T // 2, 8) for words in stored]


def _transpose(w_ref):
    tokens = []
    for n in range(w_ref.shape[1] // _T):
        w_ref[:, _cols(n)] = words = _pack(_unpack(w_ref[:, _cols(n)]).T)
        tokens.append(pltpu.bitcast(words[-8:], jnp.float32))
    return tokens


def _kernel(xt_hbm, mem0_hbm, wq_hbm, wk_hbm, wv_hbm, wot_hbm, w1_hbm, w3_hbm, w2t_hbm,
            outt_hbm, tile_ref, res_ref, norm_ref, early_norm_ref, early_ref, qkv_ref, gate_ref,
            back_ref, rest_ref, qkv_stage, gate_stage, back_stage, mem_ref,
            mem0_ref, qkv_sem, gate_sem, back_sem, tile_sem, mem_sem, *, seg):
    d_model, n_tok = xt_hbm.shape
    n_mem = mem0_hbm.shape[0]
    n_seg = n_tok // seg
    n_io = n_tok // _T
    span = n_mem + seg
    score_scale = wq_hbm.shape[2] ** -0.5 * _LOG2E
    n_qkv, n_gate = early_ref.shape[0], gate_ref.shape[0]
    n_wo = n_qkv // 3

    def blocks_at(ref, *index):
        return [ref[(*index, _cols(i))] for i in range(_FULL + 1)]

    def set_blocks(ref, index, blocks):
        for i, x in enumerate(blocks):
            ref[(*index, _cols(i))] = x

    def part_of(i, size):
        return pl.ds(pl.multiple_of(i * size, size), size)

    def step(order, attend=(), feed=(), partner=None, finished=None, filler=None, after=()):
        n_layers = len(attend)
        operand = jnp.bfloat16 if n_layers == 2 else jnp.float32
        qkv, probs, heads, mixed = {"Q": [], "K": [], "V": []}, [], [], {}
        gates, hidden, fed = [], [], {}
        if attend:
            query, key = (jax.lax.broadcasted_iota(jnp.int32, (span, _T), a) for a in (0, 1))
            own_keys = [(key >= n * span) & (key < (n + 1) * span) for n in range(n_layers)]
            visible = (query < n_mem) | (query >= jnp.where(key < span, key, key - span))
            mem = [blocks_at(mem_ref, n, slice(None)) for n in range(n_layers)]
            h = _layernorm(blocks_at(res_ref, part_of(attend[0], seg)))
            if n_layers == 1:
                attend_mix = _mixer([list(map(_stack, mem[0], h))])
            else:
                ahead = _layernorm(
                    [x[:seg - _EARLY] for x in blocks_at(res_ref, part_of(attend[1], seg))])
                cut = seg - _EARLY // 2
                known = part_of(attend[0] % 2 * (sum(_EARLY_ROWS) // _EARLY) + attend[0] // 2,
                                _EARLY // 2)
                attend_mix = _mixer(
                    [[_stack(m, a[:cut]) for m, a in zip(mem[0], h)],
                     [_stack(m, a[cut:], b) for m, a, b in zip(mem[1], h, ahead)]], operand)
        if feed:
            feed_mix = _mixer([blocks_at(norm_ref, n, slice(None)) for n in range(2)])

        def project(stage, n):
            tiles = yield from _widen(attend_mix, n_layers, _weights(qkv_ref.at[n]), _WHOLE)
            if n_layers == 1:
                qkv[stage] += [halves[0] for halves in tiles]
                return
            moved = n_mem + _EARLY // 2
            early = _unpack(early_ref[n, known, :]).astype(jnp.float32)
            for t, (a, b) in enumerate(tiles):
                x = _stack(a, b[n_mem:moved], b[:n_mem], b[moved:], early[:, _cols(t)])
                if stage == "V":
                    x = _stack(x, jnp.zeros((_T - 2 * span, _T), x.dtype))
                qkv[stage].append(x if stage == "Q" else x.astype(operand))

        def score(count):
            for t in range(len(probs), len(probs) + count):
                s = _dot(qkv["Q"][t], qkv["K"][t], axis=1)
                if n_layers == 2:
                    s = jnp.where(own_keys[1][:, :2 * span], s[span:], s[:span])
                s = jnp.concatenate(
                    [s * score_scale, jnp.zeros((span, _T - s.shape[1]), s.dtype)], axis=1)
                s = jnp.where(visible, s, _MASKED * _LOG2E)
                top = [jnp.max(jnp.where(own, s, -jnp.inf), axis=-1, keepdims=True)
                       for own in own_keys]
                p = jnp.exp2(s - jnp.where(own_keys[-1], top[-1], top[0]))
                p = _stack(*[jnp.where(own, p, 0.0) for own in own_keys])
                probs.append((p.astype(operand), _inverse(jnp.sum(p, axis=-1, keepdims=True))))
                yield

        def average(count):
            for t in range(len(heads), len(heads) + count):
                (p, inv), v = probs[t], qkv["V"][t]
                both = _dot(p[:, :v.shape[0]], v) * inv
                heads.append([both[n * span:(n + 1) * span] for n in range(n_layers)])
                yield

        def add_attended():
            x = [] if partner is None else [blocks_at(res_ref, part_of(partner, seg))]
            before = [blocks_at(res_ref, part_of(s, seg)) for s in attend]
            for n, s in enumerate(attend):
                out = _narrowed(mixed, n)
                x.append([a + o[n_mem:] for a, o in zip(before[n], out)])
                set_blocks(res_ref, [part_of(s, seg)], x[-1])
                set_blocks(mem_ref, [n, slice(None)], [o[:n_mem] for o in out])
            for n, blocks in enumerate(x):
                set_blocks(norm_ref, [n, slice(None)], _layernorm(blocks))
                yield

        def gate(w_ref, scheme):
            for halves in (yield from _widen(feed_mix, 2, _weights(w_ref), scheme)):
                gates.append([g * jnp.tanh(g) + g for g in [0.5 * x for x in halves]])

        def up(w_ref, scheme):
            for halves in (yield from _widen(feed_mix, 2, _weights(w_ref), scheme)):
                hidden.append([g * x for g, x in zip(gates[len(hidden)], halves)])

        def add_fed():
            before = [blocks_at(res_ref, part_of(s, seg)) for s in feed]
            for n, s in enumerate(feed):
                set_blocks(res_ref, [part_of(s, seg)],
                           [a + o for a, o in zip(before[n], _narrowed(fed, n))])
            yield

        def begin(name):
            stage, number = name[0], int(name[1:])
            if stage in "SA":
                return (score if stage == "S" else average)(number), number
            if stage in "NF":
                return (add_attended if stage == "N" else add_fed)(), 1
            if stage == "T":
                return transpose_out(finished), _FULL + 1
            if stage == "X":
                return filler, _count(_WHOLE)
            if stage in "QKV":
                return project(stage, 3 * number + "QKV".index(stage)), _count(_WHOLE, n_layers)
            ref, n = {"G": (gate_ref, 2 * number), "U": (gate_ref, 2 * number + 1),
                      "O": (back_ref, number), "D": (back_ref, n_wo + number)}[stage]
            w_ref, scheme = ((ref.at[n], _WHOLE) if n < n_gate
                             else (rest_ref.at["GUD".index(stage)], _REST))
            if stage in "GU":
                return (gate if stage == "G" else up)(w_ref, scheme), _count(scheme)
            acc, wide = (mixed, heads) if stage == "O" else (fed, hidden)
            wide = wide[number * _UNIT:(number + 1) * _UNIT]
            return _narrow(acc, wide, _weights(w_ref), scheme), _count(scheme, len(wide[0]))

        due = sorted((n, stage) for stage in after for n in after[stage])
        passes = itertools.chain.from_iterable(
            _interleaved(*map(begin, names.split("+"))) for names in order.split())
        for done, _ in enumerate(passes):
            while due and due[0][0] <= done:
                next(begin(due.pop(0)[1] + "1")[0])

    def start_when(condition, copies):
        @pl.when(condition)
        def _():
            for copy in copies():
                copy.start()

    def await_whole(ref, sem):
        pltpu.make_async_copy(ref, ref, sem).wait()

    def request_qkv(n, pairs=range(_UNIT // 2)):
        for which, w in enumerate((wq_hbm, wk_hbm, wv_hbm)):
            start_when((n < n_qkv) & (n % 3 == which), lambda w=w: [
                pltpu.make_async_copy(w.bitcast(jnp.uint32).at[:, n // 3 * (_UNIT // 2) + p, :],
                                      qkv_stage.at[n % 2, p], qkv_sem.at[n % 2]) for p in pairs])

    def request_others(n):
        def columns(w_hbm, unit, stage, sem):
            return [pltpu.make_async_copy(
                w_hbm.bitcast(jnp.uint32).at[:, part_of(unit, _UNIT * _T)],
                stage.at[n % 2], sem.at[n % 2])]

        start_when(n < n_wo, lambda: [
            pltpu.make_async_copy(wot_hbm.bitcast(jnp.uint32).at[n * _UNIT + t],
                                  back_stage.at[n % 2, :, _cols(t)], back_sem.at[n % 2])
            for t in range(_UNIT)])
        start_when((n >= n_wo) & (n < n_gate),
                   lambda: columns(w2t_hbm, n - n_wo, back_stage, back_sem))
        for side, w in enumerate((w1_hbm, w3_hbm)):
            start_when((n < n_gate) & (n % 2 == side),
                       lambda w=w: columns(w, n // 2, gate_stage, gate_sem))
        start_when(n == n_gate, rest_copies)

    def rest_copies():
        count = _REST.n_tiles
        return [pltpu.make_async_copy(
            w.bitcast(jnp.uint32).at[:, _cols(n_gate // 2 * _UNIT, count)],
            gate_stage.at[n_gate % 2, :, _cols(i * count, count)], gate_sem.at[n_gate % 2])
                for i, w in enumerate((w1_hbm, w3_hbm, w2t_hbm))]

    def combine_qkv(n, w_ref):
        stage = qkv_stage.at[n % 2]

        def part(t, p):
            words = stage[t // 2, pl.ds(p * _T // 2, _T // 2), :]
            words = words & jnp.uint32(0xFFFF0000) if t % 2 else words << 16
            return pltpu.bitcast(words, jnp.float32)

        return _combine(part, w_ref, _WHOLE)

    def combine_columns(stage, w_ref, scheme):
        return _combine(lambda t, p: _unpack(stage[pl.ds(p * _T // 4, _T // 4), _cols(t)]),
                        w_ref, scheme)

    def x_copy(i):
        return pltpu.make_async_copy(xt_hbm.at[:, part_of(i, _T)], tile_ref.at[i], tile_sem.at[i])

    def out_copy(i):
        return pltpu.make_async_copy(tile_ref.at[i], outt_hbm.at[:, _cols(i)], tile_sem.at[i])

    def transpose_in(i):
        x = tile_ref[i].astype(jnp.float32)
        x = _stack(x, x[_FULL * _T:])
        blocks = [x[b * _T:(b + 1) * _T].T for b in range(_FULL + 1)]
        set_blocks(res_ref, [part_of(i, _T)], blocks)
        normed = _layernorm(
            [_stack(*[x[s - _EARLY:s] for s in range(seg, _T + 1, seg)]) for x in blocks])
        for s in range(_T // seg):
            rows = part_of(i * (_T // seg // 2) + s // 2, _EARLY)
            set_blocks(early_norm_ref, [s % 2, rows],
                       [x[s * _EARLY:(s + 1) * _EARLY] for x in normed])

    def transpose_out(i):
        for b, x in enumerate(blocks_at(res_ref, part_of(i, _T))):
            depth = min(_T, d_model - b * _T)
            tile_ref[i, pl.ds(b * _T, depth), :] = x.T[:depth].astype(tile_ref.dtype)
            yield

    def early_passes(n, w_ref, chunks, *work):
        total = sum(count for _, count in chunks) * _count(_WHOLE)
        due = sorted(((total * (k + 1) // (len(tokens) + 1), token) for tokens in work
                      for k, token in enumerate(tokens)), key=lambda item: item[0])
        done = 0

        def paced(x):
            nonlocal done
            done += x.shape[0]
            while due and due[0][0] <= done:
                x = _stack(x[:-8], jnp.where(always, x[-8:], due.pop(0)[1]))
            return x

        weights = _weights(w_ref)
        for first, count in chunks:
            rows = pl.ds(pl.multiple_of(first + _LAG // 2 * _EARLY, _EARLY), count)
            mix = _mixer([blocks_at(early_norm_ref, half, rows) for half in range(2)])
            tiles = yield from _widen(lambda key, mix=mix: paced(mix(key)), 2, weights, _WHOLE)
            for half in range(2):
                at = pl.multiple_of((half * sum(_EARLY_ROWS) + first) // 2, _EARLY // 2)
                early_ref.at[n][pl.ds(at, count // 2), :] = _pack(jnp.concatenate(
                    [halves[half] for halves in tiles], axis=1).astype(jnp.bfloat16))

    def double_step(b):
        step(_ORDER, attend=[b, b + _LAG], feed=[b - 1, b + _LAG - 1], after=_AFTER,
             finished=jnp.maximum(b - 1 - _T // seg, 0) * seg // _T)

    mem_copy = pltpu.make_async_copy(mem0_hbm, mem0_ref.at[0], mem_sem)
    for copy in [mem_copy] + [x_copy(i) for i in range(_FIRST_TILES)]:
        copy.start()
    request_qkv(0, range(_UNIT // 4))
    mem_copy.wait()
    request_qkv(0, range(_UNIT // 4, _UNIT // 2))

    def load_tile(i, _):
        x_copy(i).wait()
        transpose_in(i)
        return i

    always = jax.lax.fori_loop(0, _FIRST_TILES, load_tile, 0) > 0
    mem0 = mem0_ref[0].astype(jnp.float32)
    mem_ref[0] = mem_ref[1] = jnp.concatenate([mem0, mem0[:, _FULL * _T:]], axis=1)
    for i in range(_FIRST_TILES, n_io):
        x_copy(i).start()

    chunks = list(zip(itertools.accumulate((0,) + _EARLY_ROWS), _EARLY_ROWS))
    await_whole(qkv_stage.at[0], qkv_sem.at[0])
    request_qkv(1)
    combine_qkv(0, qkv_ref.at[0])
    list(early_passes(0, qkv_ref.at[0], chunks[:_TILES_ARRIVE]))
    for i in range(_FIRST_TILES, n_io):
        x_copy(i).wait()
    request_qkv(2)
    for i in range(_FIRST_TILES, n_io):
        transpose_in(i)
    list(early_passes(0, qkv_ref.at[0], chunks[_TILES_ARRIVE:_UNIT_ARRIVES]))
    await_whole(qkv_stage.at[1], qkv_sem.at[1])
    request_others(0)
    list(early_passes(0, qkv_ref.at[0], chunks[_UNIT_ARRIVES:], combine_qkv(1, qkv_ref.at[1])))

    @pl.loop(1, n_qkv - 1)
    def _load_units(n):
        both = qkv_ref.at[pl.ds(n, 2)]
        request_qkv(n + 2)
        await_whole(qkv_stage.at[(n + 1) % 2], qkv_sem.at[(n + 1) % 2])
        list(early_passes(n, both.at[0], chunks[:4], combine_qkv(n + 1, both.at[1])))
        request_others(n)
        await_whole(gate_stage.at[(n - 1) % 2], gate_sem.at[(n - 1) % 2])
        await_whole(back_stage.at[(n - 1) % 2], back_sem.at[(n - 1) % 2])
        list(early_passes(
            n, both.at[0], chunks[4:],
            combine_columns(back_stage.at[(n - 1) % 2], back_ref.at[n - 1], _WHOLE)
            + combine_columns(gate_stage.at[(n - 1) % 2], gate_ref.at[n - 1], _WHOLE)))

    def combine_rest(i):
        stage = gate_stage.at[n_gate % 2, :, part_of(i, _REST.n_tiles * _T)]
        return combine_columns(stage, rest_ref.at[i], _REST)

    last_unit = functools.partial(early_passes, n_qkv - 1, qkv_ref.at[n_qkv - 1])
    for copy in rest_copies():
        copy.wait()
    postponed = _count(_WHOLE) // 3 * _T
    list(last_unit(chunks[:-_LAG - 2], combine_rest(2) + combine_rest(1) + combine_rest(0), sum(
        [_transpose(back_ref.at[n, :, postponed * (n // n_wo):]) for n in range(n_gate)]
        + [_transpose(rest_ref.at[2])], [])))

    @pl.loop(0, _LAG, unroll=True)
    def _first_steps(s):
        def filler(first, count):
            yield from last_unit([(first + s * count, count)],
                                 _transpose(back_ref.at[n_wo + s, :, :postponed]))

        step(_ORDER_HEAD, attend=[s], partner=0, filler=filler(*chunks[-_LAG - 2]))

    step(_ORDER_FFN + " X0", feed=[0, 1], filler=last_unit(chunks[-2:-1]))
    mem_ref[0], mem_ref[1] = mem_ref[1], mem_ref[0]
    step(_ORDER_HEAD, attend=[0, _LAG], filler=last_unit(chunks[-1:]))
    pl.loop(1, n_seg - _LAG)(double_step)
    for i in range(n_io - 1):
        out_copy(i).start()
    step(_ORDER_TAIL, attend=[n_seg - 2], feed=[n_seg - 3, n_seg - 1])
    step(_ORDER_LAST, attend=[n_seg - 1], partner=n_seg - 2)
    step(_ORDER_FFN + " T0", feed=[n_seg - 2, n_seg - 1], finished=n_io - 1)
    out_copy(n_io - 1).start()
    for i in range(n_io):
        out_copy(i).wait()


@functools.partial(jax.jit, static_argnames=("A_seg_len",))
def pallas_interleave_layers__memory_aug_recurrent_mem_tr__glu_gated_swiglu__prompt_kernel(
    A_x: jax.Array,
    A_mem0: jax.Array,
    A_Wq: jax.Array,
    A_Wk: jax.Array,
    A_Wv: jax.Array,
    A_Wo: jax.Array,
    A_seg_len: int,
    B_x: jax.Array,
    B_w1: jax.Array,
    B_w3: jax.Array,
    B_w2: jax.Array,
):
    del B_x
    _, n_tok, d_model = A_x.shape
    n_mem = A_mem0.shape[1]
    assert A_x.shape == (1, 2048, 576) and A_seg_len == 32 and n_mem == 8
    assert A_Wq.shape[1:] == (2 * _UNIT, _T) and B_w1.shape[1] == 36 * _T
    width = (_FULL + 1) * _T
    hbm = pl.BlockSpec(memory_space=pltpu.HBM)

    def weights(scheme, units):
        return pltpu.VMEM((units, _T // 2, _count(scheme) * _T), jnp.uint32)

    out_t = pl.pallas_call(
        functools.partial(_kernel, seg=A_seg_len),
        out_shape=jax.ShapeDtypeStruct((d_model, n_tok), A_x.dtype),
        in_specs=[hbm] * 9,
        out_specs=hbm,
        scratch_shapes=[
            pltpu.VMEM((n_tok // _T, d_model, _T), A_x.dtype),
            pltpu.VMEM((n_tok, width), jnp.float32),
            pltpu.VMEM((2, A_seg_len, width), jnp.float32),
            pltpu.VMEM((2, n_tok // A_seg_len * _EARLY // 2, width), jnp.float32),
            pltpu.VMEM((6, sum(_EARLY_ROWS), _UNIT * _T), jnp.uint32),
            weights(_WHOLE, 6), weights(_WHOLE, 4), weights(_WHOLE, 4), weights(_REST, 3),
            pltpu.VMEM((2, _UNIT // 2, d_model, _T), jnp.uint32),
            pltpu.VMEM((2, d_model // 2, _UNIT * _T), jnp.uint32),
            pltpu.VMEM((2, d_model // 2, _UNIT * _T), jnp.uint32),
            pltpu.VMEM((2, n_mem, width), jnp.float32),
            pltpu.VMEM((8, n_mem, d_model), A_mem0.dtype),
            pltpu.SemaphoreType.DMA((2,)),
            pltpu.SemaphoreType.DMA((2,)),
            pltpu.SemaphoreType.DMA((2,)),
            pltpu.SemaphoreType.DMA((n_tok // _T,)),
            pltpu.SemaphoreType.DMA,
        ],
        compiler_params=pltpu.CompilerParams(vmem_limit_bytes=116 * 1024 * 1024,
                                             disable_bounds_checks=True),
    )(A_x.reshape(n_tok, d_model).T, A_mem0.reshape(n_mem, d_model), A_Wq, A_Wk, A_Wv,
      A_Wo.transpose(0, 2, 1), B_w1, B_w3, B_w2.T)
    return out_t.T.reshape(A_x.shape)
```
